```python
import jax
import jax.numpy as jnp

def _softmax(x, axis=-1):
    return jax.nn.softmax(x, axis=axis)

def _gelu(x):
    return jax.nn.gelu(x, approximate=True)

def _silu(x):
    return jax.nn.silu(x)

def _sigmoid(x):
    return jax.nn.sigmoid(x)

def _layernorm(x, axis=-1, eps=1e-05):
    m = jnp.mean(x, axis=axis, keepdims=True)
    v = jnp.var(x, axis=axis, keepdims=True)
    return (x - m) / jnp.sqrt(v + eps)

def _scatter_add(tgt, idx, src, axis=0):
    return tgt.at[idx].add(src)

def _segment_sum(src, seg, n):
    return jax.ops.segment_sum(src, seg, n)

class _Rng:

    def __init__(self, key):
        self._k = key

    def _next(self):
        self._k, sub = jax.random.split(self._k)
        return sub

    def normal(self, shape):
        return jax.random.normal(self._next(), shape, dtype=jnp.bfloat16)

    def randint(self, lo, hi, shape):
        return jax.random.randint(self._next(), shape, lo, hi, dtype=jnp.int32)

    def uniform(self, shape, lo=0.0, hi=1.0):
        return jax.random.uniform(self._next(), shape, jnp.bfloat16, lo, hi)

    def permutation(self, n):
        return jax.random.permutation(self._next(), n)
kernel_name = 'adaLN_cond__spectral_gfnet__mixer_token_mlp__prompt'

def setup_inputs():
    _rng = _Rng(jax.random.key(int.from_bytes(__import__("os").urandom(4), "little")))
    _w = lambda a: (lambda t: t.astype(jnp.bfloat16) if jnp.issubdtype(t.dtype, jnp.floating) else t)(jnp.asarray(a))

    def _A_setup():
        B, S, D = (1, 2048, 576)
        Df = D // 2 + 1
        return {'x': _w((lambda *s: _rng.normal(s) * 0.05)(B, S, D)), 'w_r': _w((lambda *s: _rng.normal(s) * 0.05)(S, Df) * 0.02), 'w_i': _w((lambda *s: _rng.normal(s) * 0.05)(S, Df) * 0.02)}
    _A_in = _A_setup()

    def _B_setup():
        B, S, D, F = (1, 2048, 576, 4608)
        return {'x': _w((lambda *s: _rng.normal(s) * 0.05)(B, S, D)), 'w1': _w((lambda *s: _rng.normal(s) * 0.05)(S, F) * S ** (-0.5)), 'b1': _w((lambda *s: _rng.normal(s) * 0.05)(F) * 0.02), 'w2': _w((lambda *s: _rng.normal(s) * 0.05)(F, S) * F ** (-0.5)), 'b2': _w((lambda *s: _rng.normal(s) * 0.05)(S) * 0.02)}
    _B_in = _B_setup()
    return {'A_x': _A_in['x'], 'A_w_r': _A_in['w_r'], 'A_w_i': _A_in['w_i'], 'B_x': _B_in['x'], 'B_w1': _B_in['w1'], 'B_b1': _B_in['b1'], 'B_w2': _B_in['w2'], 'B_b2': _B_in['b2'], 'c': _w((lambda *s: _rng.normal(s) * 0.05)(1, 576)), 'w_mod': _w((lambda *s: _rng.normal(s) * 0.05)(576, 6 * 576) * 576 ** (-0.5))}

def reference(A_x, A_w_r, A_w_i, B_x, B_w1, B_b1, B_w2, B_b2, c, w_mod):

    def _A_ref(x, w_r, w_i):
        B, S, D = x.shape
        X = (lambda x, axes=(-2, -1): jnp.fft.rfft2(x.astype(jnp.float32), axes=axes))(x, axes=(-2, -1))
        W = w_r + 1j * w_i
        X = X * W
        y = (lambda x, s, axes=(-2, -1): jnp.fft.irfft2(x, s=s, axes=axes).astype(jnp.bfloat16))(X, (S, D), axes=(-2, -1))
        return y

    def _B_ref(x, w1, b1, w2, b2):
        B, S, D = x.shape
        h = _layernorm(x, axis=-1)
        u = jnp.einsum('bsd,sf->bdf', h, w1) + b1
        u = _gelu(u)
        y = jnp.einsum('bdf,fs->bds', u, w2) + b2
        return (lambda x, *d: x.transpose(*d))(y, 0, 2, 1)
    x = A_x
    mod = (_silu(c) @ w_mod).reshape(c.shape[0], 6, 1, -1)
    sa, ca, ga, sb, cb, gb = (mod[:, 0].copy(), mod[:, 1].copy(), mod[:, 2].copy(), mod[:, 3].copy(), mod[:, 4].copy(), mod[:, 5].copy())
    h = _layernorm(x, axis=-1) * (1 + ca) + sa
    x = x + ga * _A_ref(h, A_w_r, A_w_i)
    h = _layernorm(x, axis=-1) * (1 + cb) + sb
    x = x + gb * _B_ref(h, B_w1, B_b1, B_w2, B_b2)
    return x
```

```python
import functools
import math

import jax
import jax.numpy as jnp
import numpy as np
from jax import lax
import jax.experimental.pallas as pl
import jax.experimental.pallas.tpu as pltpu

S, D, F = 2048, 576, 4608
DF = D // 2 + 1
KR = 296
NB = S // 128
XC = 4
XW = S // XC
FC = 512
SC = 512
EPS = 1e-5

f32 = jnp.float32
bf16 = jnp.bfloat16
_NN = (((1,), (0,)), ((), ()))
_NT = (((1,), (1,)), ((), ()))


def _dot(a, b, dims=_NN):
    return lax.dot_general(a, b, dims, preferred_element_type=f32)


@functools.lru_cache(maxsize=None)
def _tables():
    r = np.arange(64)
    kk = np.arange(32)
    th = lambda k: 2 * np.pi * np.outer(k, r) / D
    fwd = []
    for q in range(1, 5):
        a, b = th(q + 9 * kk), th(9 - q + 9 * kk)
        fwd.append(np.block([[np.cos(a), np.sin(a)], [-np.sin(a), np.cos(a)],
                             [np.cos(b), -np.sin(b)], [-np.sin(b), -np.cos(b)]]))
    l0 = np.concatenate(
        [np.cos(th(9 * kk)), -np.sin(th(9 * kk)), np.cos(th(np.array([D // 2])))], 0)
    cw = np.full((65, 1), 2.0)
    cw[0] = cw[64] = 1.0
    l0f = np.zeros((80, 128))
    l0f[:65, :64] = l0
    l0i = np.zeros((64, 128))
    l0i[:, :65] = (l0 * cw).T
    dmat = np.concatenate(fwd + [l0f] + [2 * m.T for m in fwd] + [l0i], 0)

    n2 = np.arange(128)
    a16 = np.arange(16)
    tw = lambda m: np.exp(-2j * np.pi * np.outer(m, n2) / S)
    e, r1, r2 = tw(n2), tw(127 * a16), tw(127 * a16 + 128)
    t1, t2 = np.concatenate([r2, r1], 0), np.concatenate([r1, r1], 0)
    smat = np.concatenate([e.real, e.imag, t1.real, t1.imag, t2.real, t2.imag], 0)
    return dmat.astype(np.float32), smat.astype(np.float32)


_DF_OFF = 0
_D0F_OFF = 512
_DI_OFF = 592
_D0I_OFF = 1104
_DROWS = 1168
_SROWS = 384


_S3 = math.sqrt(3.0) / 2
_C1, _S1 = math.cos(2 * math.pi / 9), math.sin(2 * math.pi / 9)
_C2, _S2 = math.cos(4 * math.pi / 9), math.sin(4 * math.pi / 9)


def _radix9_fwd(a):
    b0, br, bd = [], [], []
    for j in range(3):
        t = a[3 + j] + a[6 + j]
        b0.append(a[j] + t)
        br.append(a[j] - 0.5 * t)
        bd.append(a[3 + j] - a[6 + j])
    t = b0[1] + b0[2]
    y0 = b0[0] + t
    y3 = (b0[0] - 0.5 * t, _S3 * (b0[2] - b0[1]))
    c0r, c0i = br[0], -_S3 * bd[0]
    c1r = _C1 * br[1] - (_S3 * _S1) * bd[1]
    c1i = -_S1 * br[1] - (_S3 * _C1) * bd[1]
    c2r = _C2 * br[2] - (_S3 * _S2) * bd[2]
    c2i = -_S2 * br[2] - (_S3 * _C2) * bd[2]
    tr, ti = c1r + c2r, c1i + c2i
    y1 = (c0r + tr, c0i + ti)
    ur, ui = c0r - 0.5 * tr, c0i - 0.5 * ti
    nvr, vi = _S3 * (c2r - c1r), _S3 * (c1i - c2i)
    y4 = (ur + vi, ui + nvr)
    y2 = (ur - vi, nvr - ui)
    return y0, {1: y1, 2: y2, 3: y3, 4: y4}


def _radix9_inv(p0, p):
    (p1r, p1i), (p2r, p2i), (p3r, p3i), (p4r, p4i) = p[1], p[2], p[3], p[4]
    ur, ui = p4r + p2r, p4i - p2i
    vi, nvr = _S3 * (p4r - p2r), _S3 * (p4i + p2i)
    c0r, c0i = p1r + ur, p1i + ui
    tr, ti = p1r - 0.5 * ur, p1i - 0.5 * ui
    c1r, c1i, c2r, c2i = tr - nvr, ti + vi, tr + nvr, ti - vi
    br = [c0r, _C1 * c1r - _S1 * c1i, _C2 * c2r - _S2 * c2i]
    nbd = [_S3 * c0i,
           (_S3 * _S1) * c1r + (_S3 * _C1) * c1i,
           (_S3 * _S2) * c2r + (_S3 * _C2) * c2i]
    ny3 = _S3 * p3i
    t = p0 - 0.5 * p3r
    b0 = [p0 + p3r, t - ny3, t + ny3]
    y = [None] * 9
    for j in range(3):
        t = b0[j] - 0.5 * br[j]
        y[j] = b0[j] + br[j]
        y[3 + j] = t - nbd[j]
        y[6 + j] = t + nbd[j]
    return y


def _sadd(a, b):
    if a[1] == b[1]:
        return (a[0] + b[0], a[1])
    return (b[0] - a[0], False) if a[1] else (a[0] - b[0], False)


def _sneg(a):
    return (a[0], not a[1])


def _radix4(x, inverse):
    add = lambda u, v: (_sadd(u[0], v[0]), _sadd(u[1], v[1]))
    sub = lambda u, v: (_sadd(u[0], _sneg(v[0])), _sadd(u[1], _sneg(v[1])))
    s02, d02, s13, d13 = add(x[0], x[2]), sub(x[0], x[2]), add(x[1], x[3]), sub(x[1], x[3])
    rot = (d13[1], _sneg(d13[0]))
    y1, y3 = add(d02, rot), sub(d02, rot)
    if inverse:
        y1, y3 = y3, y1
    return [add(s02, s13), y1, sub(s02, s13), y3]


def _twiddle16(z, e):
    e %= 16
    re, im = z
    if e == 0:
        return z
    if e == 4:
        return (im, _sneg(re))
    if e == 12:
        return (_sneg(im), re)
    c, s = math.cos(math.pi * e / 8), math.sin(math.pi * e / 8)
    scale = lambda v, w: (v[0] * (-w if v[1] else w), False)
    if e % 4 == 2:
        sc, ss = (1 if c > 0 else -1), (1 if s > 0 else -1)
        flip = lambda v, sg: v if sg > 0 else _sneg(v)
        return (scale(_sadd(flip(re, sc), flip(im, ss)), abs(c)),
                scale(_sadd(flip(im, sc), flip(re, -ss)), abs(c)))
    return (_sadd(scale(re, c), scale(im, s)), _sadd(scale(im, c), scale(re, -s)))


def _radix16(load, store, inverse):
    sgn = -1 if inverse else 1
    t = []
    for b in range(4):
        x = []
        for a in range(4):
            re, im = load(4 * a + b)
            x.append(((re, False), (im, False)))
        y = _radix4(x, inverse)
        t.append([_twiddle16(y[p0], sgn * b * p0) for p0 in range(4)])
    for p0 in range(4):
        y = _radix4([t[b][p0] for b in range(4)], inverse)
        for p1 in range(4):
            (re, nr), (im, ni) = y[p1]
            store(p0 + 4 * p1, -re if nr else re, -im if ni else im)


class _Stats:
    def __init__(self):
        self.s = [None, None]
        self.q = [None, None]
        self.n = 0

    def add(self, v):
        i = self.n % 2
        self.n += 1
        self.s[i] = v if self.s[i] is None else self.s[i] + v
        self.q[i] = v * v if self.q[i] is None else self.q[i] + v * v

    def scale_shift(self):
        mean = jnp.sum(self.s[0] + self.s[1], axis=0, keepdims=True) * (1.0 / D)
        msq = jnp.sum(self.q[0] + self.q[1], axis=0, keepdims=True) * (1.0 / D)
        r = lax.rsqrt(jnp.maximum(msq - mean * mean, 0.0) + EPS)
        return (jnp.broadcast_to(r, (8, 128)), jnp.broadcast_to(-mean * r, (8, 128)))


def _kernel(x_hbm, wr_hbm, wi_hbm, w1_hbm, b1_hbm, w2_hbm, b2_hbm, c_hbm, wm_hbm,
            dm_hbm, sm_hbm, o_hbm,
            x_v, w_v, wm_v, c_v, b1_v, b2_v, dm_v, sm_v, mod_v, g_tab, y_v,
            xd_v, v_v, u_v, z_v, wp_v, p_v, x1_v, t_v, h2_v, w1_v, w2_v, act_v,
            bias1_v, bias2_v, o_v, sem_in, sem_w1, sem_w2, sem_out):
    n1, n2 = F // FC, S // SC
    bpc = XW // 128

    def copy_in(i, src, dst):
        return pltpu.make_async_copy(src, dst, sem_in.at[i])

    def wm_copy(i, lo, hi):
        return copy_in(i, wm_hbm.at[:, lo:hi], wm_v.at[:, lo:hi])

    cp_sm = copy_in(0, sm_hbm, sm_v)
    cp_c = copy_in(1, c_hbm, c_v)
    cp_wm = [wm_copy(2, 0, 1152), wm_copy(3, 1152, 2944), wm_copy(4, 2944, 6 * D)]
    cp_dm = copy_in(5, dm_hbm, dm_v)
    cp_w = [copy_in(6, wr_hbm, w_v.at[0]), copy_in(7, wi_hbm, w_v.at[1])]
    cp_b = [copy_in(8, b1_hbm, b1_v), copy_in(9, b2_hbm, b2_v)]
    cp_x = [copy_in(10 + i, x_hbm.at[:, i * XW:(i + 1) * XW], x_v.at[i]) for i in range(XC)]
    cp_w1 = [pltpu.make_async_copy(w1_hbm.at[:, j * FC:(j + 1) * FC], w1_v.at[j], sem_w1.at[j])
             for j in range(n1)]
    cp_w2 = [pltpu.make_async_copy(w2_hbm.at[:, j * SC:(j + 1) * SC], w2_v.at[j], sem_w2.at[j])
             for j in range(n2)]

    for cp in [cp_sm, cp_c, cp_wm[0], cp_dm] + cp_x:
        cp.start()

    cp_sm.wait()
    for cp in cp_w + [cp_wm[1]]:
        cp.start()
    for p in range(NB):
        for i in range(8):
            off = (256 if i == 0 else 320) + 16 - p
            hr, hi = sm_v[off:off + 16, :], sm_v[off + 32:off + 48, :]
            er, ei = sm_v[16 * i:16 * i + 16, :], sm_v[128 + 16 * i:144 + 16 * i, :]
            cr = er * hr - ei * hi
            ci = er * hi + ei * hr
            for t, m in enumerate((cr, ci - cr, cr + ci)):
                g_tab[p, t, 16 * i:16 * i + 16, :] = m.astype(bf16)

    def modulation(lo, hi):
        cv = c_v[...].astype(f32)
        sc = jnp.broadcast_to(cv * jax.nn.sigmoid(cv), (8, D))
        m = _dot(sc, wm_v[:, lo:hi])
        for t in range((hi - lo) // 128):
            row = jnp.broadcast_to(m[0:1, 128 * t:128 * (t + 1)], (128, 128))
            mod_v[lo + 128 * t:lo + 128 * (t + 1), :] = row.T

    def mod_tile(i, row):
        return mod_v[i * D + row:i * D + row + 8, :]

    cp_c.wait()
    cp_wm[0].wait()
    modulation(0, 1152)
    cp_dm.wait()

    def load_x(xr, i, r):
        v = xr[r:r + 16, 128 * i:128 * (i + 1)].astype(f32)
        return v[:8], v[8:]

    def phase1(ch, carry):
        pltpu.make_async_copy(x_v.at[ch], x_v.at[ch], sem_in.at[10 + ch]).wait()
        xr = x_v.at[ch]
        for i in range(bpc):
            st = _Stats()
            for r in range(0, D, 16):
                for v in load_x(xr, i, r):
                    st.add(v)
            rs, sh = st.scale_shift()
            for t in range(0, 64, 16):
                tiles = [load_x(xr, i, 64 * j + t) for j in range(9)]
                for hf in range(2):
                    r = t + 8 * hf
                    a = [(tiles[j][hf] * rs + sh) * (1.0 + mod_tile(1, 64 * j + r))
                         + mod_tile(0, 64 * j + r) for j in range(9)]
                    y0, y = _radix9_fwd(a)
                    y_v[i, 512 + r:520 + r, :] = y0
                    for q in range(1, 5):
                        y_v[i, 128 * (q - 1) + r:128 * (q - 1) + r + 8, :] = y[q][0]
                        y_v[i, 128 * (q - 1) + 64 + r:128 * (q - 1) + 72 + r, :] = y[q][1]
            blk = ch * bpc + i
            for q in range(1, 5):
                o = _dot(dm_v[_DF_OFF + 128 * (q - 1):_DF_OFF + 128 * q, :],
                         y_v[i, 128 * (q - 1):128 * q, :])
                xd_v[blk, 0, pl.ds(q, 32, stride=9), :] = o[0:32]
                xd_v[blk, 1, pl.ds(q, 32, stride=9), :] = o[32:64]
                xd_v[blk, 0, pl.ds(9 - q, 32, stride=9), :] = o[64:96]
                xd_v[blk, 1, pl.ds(9 - q, 32, stride=9), :] = o[96:128]
            o = _dot(dm_v[_D0F_OFF:_D0F_OFF + 80, 0:64], y_v[i, 512:576, :])
            xd_v[blk, 0, pl.ds(0, 32, stride=9), :] = o[0:32]
            xd_v[blk, 1, pl.ds(0, 32, stride=9), :] = o[32:64]
            xd_v[blk, 0, 288:296, :] = o[64:72]
            xd_v[blk, 1, 288:296, :] = jnp.zeros((8, 128), f32)
        return carry

    lax.fori_loop(0, XC, phase1, None)

    for cp in cp_w1[:2]:
        cp.start()

    lane = lax.broadcasted_iota(jnp.int32, (8, 128), 1)

    def shuffle(v):
        v = [v[0]] + [pltpu.roll(v[a], a, 1) for a in range(15, 0, -1)]
        for t in range(4):
            m = ((lane >> t) & 1) == 1
            v = [jnp.where(m, v[(p - (1 << t)) % NB], v[p]) for p in range(NB)]
        return v

    for pln in range(2):
        cp_w[pln].wait()

        def w_step(t, carry, pln=pln):
            r = pl.multiple_of(t * 16, 16)
            v = [pltpu.bitcast(w_v[pln, pl.ds(r, 16), 128 * a:128 * (a + 1)], jnp.int32)
                 for a in range(NB)]
            for p, w in enumerate(shuffle(v)):
                wp_v[pln, p, pl.ds(r, 16), :] = pltpu.bitcast(w, bf16).astype(f32)
            return carry

        lax.fori_loop(0, 18, w_step, None)
        v = [jnp.broadcast_to(w_v[pln, 288:289, 128 * a:128 * (a + 1)].astype(f32), (8, 128))
             for a in range(NB)]
        for p, w in enumerate(shuffle(v)):
            wp_v[pln, p, 288:296, :] = w

    for cp in cp_w1[2:] + cp_b + [cp_wm[2]] + cp_w2:
        cp.start()

    for g in range(4):
        r0, n = 72 * g, (80 if g == 3 else 72)
        for r in range(r0, r0 + n, 8):
            def store_v(p, re, im, r=r):
                v_v[p, 0, r:r + 8, :] = re
                v_v[p, 1, r:r + 8, :] = im
            _radix16(lambda b, r=r: (xd_v[b, 0, r:r + 8, :], xd_v[b, 1, r:r + 8, :]),
                     store_v, False)
        rows = slice(r0, r0 + n)
        for p in range(NB):
            a, b = v_v[p, 0, rows, :], v_v[p, 1, rows, :]
            m1, m2, m3 = g_tab[p, 0], g_tab[p, 1], g_tab[p, 2]
            k1 = _dot(a + b, m1, _NT)
            xr = k1 - _dot(b, m3, _NT)
            xi = k1 + _dot(a, m2, _NT)
            wr, wi = wp_v[0, p, rows, :], wp_v[1, p, rows, :]
            zr, zi = xr * wr - xi * wi, xr * wi + xi * wr
            k1 = _dot(zr + zi, m1)
            u_v[p, 0, rows, :] = k1 + _dot(zi, m2)
            u_v[p, 1, rows, :] = k1 - _dot(zr, m3)
        for q in range(9 + (g == 3)):
            src = pl.ds(r0 + q, 8, stride=9) if q < 9 else pl.ds(288, 8)
            dst = 32 * q + 8 * g if q < 9 else 288

            def store_z(b, re, im, dst=dst):
                z_v[b, 0, dst:dst + 8, :] = re
                z_v[b, 1, dst:dst + 8, :] = im
            _radix16(lambda p, src=src: (u_v[p, 0, src, :], u_v[p, 1, src, :]), store_z, True)

    cp_wm[1].wait()
    modulation(1152, 2944)

    def phase3(ch, carry):
        xr = x_v.at[ch]
        for i in range(bpc):
            blk = ch * bpc + i
            lanes = slice(128 * i, 128 * (i + 1))
            for q in range(1, 5):
                rhs = jnp.concatenate(
                    [z_v[blk, pln, 32 * k:32 * k + 32, :] for k in (q, 9 - q) for pln in (0, 1)], 0)
                p_v[i, 128 * (q - 1):128 * q, :] = _dot(
                    dm_v[_DI_OFF + 128 * (q - 1):_DI_OFF + 128 * q, :], rhs)
            rhs = jnp.concatenate(
                [z_v[blk, 0, 0:32, :], z_v[blk, 1, 0:32, :], z_v[blk, 0, 288:296, :]], 0)
            p_v[i, 512:576, :] = _dot(dm_v[_D0I_OFF:_D0I_OFF + 64, 0:72], rhs)

            st = _Stats()
            for t in range(0, 64, 16):
                tiles = [load_x(xr, i, 64 * j + t) for j in range(9)]
                for hf in range(2):
                    r = t + 8 * hf
                    y = _radix9_inv(
                        p_v[i, 512 + r:520 + r, :],
                        {q: (p_v[i, 128 * (q - 1) + r:128 * (q - 1) + r + 8, :],
                             p_v[i, 128 * (q - 1) + 64 + r:128 * (q - 1) + 72 + r, :])
                         for q in range(1, 5)})
                    for j in range(9):
                        row = 64 * j + r
                        x1 = tiles[j][hf] + (mod_tile(2, row) * (1.0 / (S * D))) * y[j]
                        st.add(x1)
                        x1_v[ch, row:row + 8, lanes] = x1
            rs, sh = st.scale_shift()
            st = _Stats()
            for row in range(0, D, 8):
                t = (x1_v[ch, row:row + 8, lanes] * rs + sh) * (1.0 + mod_tile(4, row)) \
                    + mod_tile(3, row)
                st.add(t)
                t_v[i, row:row + 8, :] = t
            rs, sh = st.scale_shift()
            for row in range(0, D, 8):
                h2_v[ch, row:row + 8, lanes] = t_v[i, row:row + 8, :] * rs + sh
        return carry

    lax.fori_loop(0, XC, phase3, None)

    for cp in cp_b + [cp_wm[2]]:
        cp.wait()
    modulation(2944, 6 * D)
    for src, dst, w in ((b1_v, bias1_v, FC), (b2_v, bias2_v, SC)):
        bv = src[...].astype(f32)
        for t in range(src.shape[0]):
            j, o = divmod(128 * t, w)
            dst[j, :, o:o + 128] = jnp.broadcast_to(bv[t:t + 1, :], (8, 128))

    def mlp1(j, carry):
        pltpu.make_async_copy(w1_v.at[j], w1_v.at[j], sem_w1.at[j]).wait()
        u = None
        for k in range(XC):
            part = _dot(h2_v[k], w1_v[j, k * XW:(k + 1) * XW, :])
            u = part if u is None else u + part
        u = u + bias1_v[j, 0:1, :]
        k0 = math.sqrt(2.0 / math.pi)
        th = jnp.tanh(u * (k0 + (k0 * 0.044715) * (u * u)))
        hu = 0.5 * u
        act_v[j] = (hu + hu * th).astype(bf16)
        return carry

    lax.fori_loop(0, n1, mlp1, None)

    def out_copy(j):
        return pltpu.make_async_copy(
            o_v.at[j], o_hbm.at[:, pl.ds(pl.multiple_of(j * SC, SC), SC)], sem_out.at[j])

    def mlp2(j, carry):
        pltpu.make_async_copy(w2_v.at[j], w2_v.at[j], sem_w2.at[j]).wait()
        y = None
        for k in range(n1):
            part = _dot(act_v[k], w2_v[j, k * FC:(k + 1) * FC, :])
            y = part if y is None else y + part
        y = y + bias2_v[j, 0:1, :]
        gb = mod_v[5 * D:6 * D, :]
        for i in range(SC // 128):
            lanes = slice(128 * i, 128 * (i + 1))
            o_v[j, :, lanes] = (x1_v[j, :, lanes] + gb * y[:, lanes]).astype(bf16)
        out_copy(j).start()
        return carry

    lax.fori_loop(0, n2, mlp2, None)
    for j in range(n2):
        out_copy(j).wait()


@jax.jit
def pallas_adaLN_cond__spectral_gfnet__mixer_token_mlp__prompt_kernel(
    A_x: jax.Array,
    A_w_r: jax.Array,
    A_w_i: jax.Array,
    B_x: jax.Array,
    B_w1: jax.Array,
    B_b1: jax.Array,
    B_w2: jax.Array,
    B_b2: jax.Array,
    c: jax.Array,
    w_mod: jax.Array,
):
    del B_x
    assert A_x.shape == (1, S, D) and SC == XW
    dmat, smat = _tables()
    n1, n2 = F // FC, S // SC
    vmem = pltpu.VMEM
    spectrum = vmem((NB, 2, KR, 128), f32)
    out_t = pl.pallas_call(
        _kernel,
        in_specs=[pl.BlockSpec(memory_space=pltpu.HBM)] * 11,
        out_specs=pl.BlockSpec(memory_space=pltpu.HBM),
        out_shape=jax.ShapeDtypeStruct((D, S), bf16),
        scratch_shapes=[
            vmem((XC, D, XW), bf16),
            vmem((2, DF, S), bf16),
            vmem((D, 6 * D), bf16),
            vmem((1, D), bf16),
            vmem((F // 128, 128), bf16),
            vmem((S // 128, 128), bf16),
            vmem((_DROWS, 128), bf16),
            vmem((_SROWS, 128), f32),
            vmem((6 * D, 128), f32),
            vmem((NB, 3, 128, 128), bf16),
            vmem((XW // 128, D, 128), f32),
            spectrum, spectrum, spectrum, spectrum,
            vmem((2, NB, KR, 128), f32),
            vmem((XW // 128, D, 128), f32),
            vmem((XC, D, XW), f32),
            vmem((XW // 128, D, 128), f32),
            vmem((XC, D, XW), f32),
            vmem((n1, S, FC), bf16),
            vmem((n2, F, SC), bf16),
            vmem((n1, D, FC), bf16),
            vmem((n1, 8, FC), f32),
            vmem((n2, 8, SC), f32),
            vmem((n2, D, SC), bf16),
            pltpu.SemaphoreType.DMA((10 + XC,)),
            pltpu.SemaphoreType.DMA((n1,)),
            pltpu.SemaphoreType.DMA((n2,)),
            pltpu.SemaphoreType.DMA((n2,)),
        ],
        compiler_params=pltpu.CompilerParams(vmem_limit_bytes=116 * 1024 * 1024),
    )(
        A_x.reshape(S, D).T, A_w_r.T, A_w_i.T, B_w1, B_b1.reshape(F // 128, 128),
        B_w2, B_b2.reshape(S // 128, 128), c, w_mod,
        jnp.asarray(dmat, dtype=bf16), jnp.asarray(smat),
    )
    return out_t.T.reshape(1, S, D)
```

```python
import functools
import math

import jax
import jax.numpy as jnp
import numpy as np
from jax import lax
import jax.experimental.pallas as pl
import jax.experimental.pallas.tpu as pltpu

S, D, F = 2048, 576, 4608
DF = D // 2 + 1
KR = 296
NB = S // 128
HD = D // 2
FC = 512
SC = 512
EPS = 1e-5

f32 = jnp.float32
bf16 = jnp.bfloat16
_NN = (((1,), (0,)), ((), ()))
_NT = (((1,), (1,)), ((), ()))


def _dot(a, b, dims=_NN):
    return lax.dot_general(a, b, dims, preferred_element_type=f32)


@functools.lru_cache(maxsize=None)
def _tables():
    r = np.arange(64)
    kk = np.arange(32)
    th = lambda k: 2 * np.pi * np.outer(k, r) / D

    def weave(re, im):
        n = re.shape[1]
        return np.stack([re.reshape(4, 8, n), im.reshape(4, 8, n)], 1).reshape(64, n)

    fwd = []
    for q in range(1, 5):
        a, b = th(q + 9 * kk), th(9 - q + 9 * kk)
        fwd.append(np.concatenate([
            weave(np.block([np.cos(a), np.sin(a)]), np.block([-np.sin(a), np.cos(a)])),
            weave(np.block([np.cos(b), -np.sin(b)]), np.block([-np.sin(b), -np.cos(b)]))], 0))
    l0 = np.concatenate(
        [weave(np.cos(th(9 * kk)), -np.sin(th(9 * kk))), np.cos(th(np.array([D // 2])))], 0)
    cw = np.full((65, 1), 2.0)
    cw[0] = cw[64] = 1.0
    l0f = np.zeros((80, 128))
    l0f[:65, :64] = l0
    l0i = np.zeros((64, 128))
    l0i[:, :65] = (l0 * cw).T
    dmat = np.concatenate(fwd + [l0f] + [2 * m.T for m in fwd] + [l0i], 0)

    n2 = np.arange(128)
    a16 = np.arange(16)
    tw = lambda m: np.exp(-2j * np.pi * np.outer(m, n2) / S)
    e, r1, r2 = tw(n2), tw(127 * a16), tw(127 * a16 + 128)
    t1, t2 = np.concatenate([r2, r1], 0), np.concatenate([r1, r1], 0)
    smat = np.concatenate([e.real, e.imag, t1.real, t1.imag, t2.real, t2.imag], 0)
    return dmat.astype(np.float32), smat.astype(np.float32)


_DF_OFF = 0
_D0F_OFF = 512
_DI_OFF = 592
_D0I_OFF = 1104
_DROWS = 1168
_SROWS = 384

_S3 = math.sqrt(3.0) / 2
_C1, _S1 = math.cos(2 * math.pi / 9), math.sin(2 * math.pi / 9)
_C2, _S2 = math.cos(4 * math.pi / 9), math.sin(4 * math.pi / 9)


def _radix9_fwd(a):
    b0, br, bd = [], [], []
    for j in range(3):
        t = a[3 + j] + a[6 + j]
        b0.append(a[j] + t)
        br.append(a[j] - 0.5 * t)
        bd.append(a[3 + j] - a[6 + j])
    t = b0[1] + b0[2]
    y0 = b0[0] + t
    y3 = (b0[0] - 0.5 * t, _S3 * (b0[2] - b0[1]))
    c0r, c0i = br[0], -_S3 * bd[0]
    c1r = _C1 * br[1] - (_S3 * _S1) * bd[1]
    c1i = -_S1 * br[1] - (_S3 * _C1) * bd[1]
    c2r = _C2 * br[2] - (_S3 * _S2) * bd[2]
    c2i = -_S2 * br[2] - (_S3 * _C2) * bd[2]
    tr, ti = c1r + c2r, c1i + c2i
    y1 = (c0r + tr, c0i + ti)
    ur, ui = c0r - 0.5 * tr, c0i - 0.5 * ti
    nvr, vi = _S3 * (c2r - c1r), _S3 * (c1i - c2i)
    y4 = (ur + vi, ui + nvr)
    y2 = (ur - vi, nvr - ui)
    return y0, {1: y1, 2: y2, 3: y3, 4: y4}


def _radix9_inv(p0, p):
    (p1r, p1i), (p2r, p2i), (p3r, p3i), (p4r, p4i) = p[1], p[2], p[3], p[4]
    ur, ui = p4r + p2r, p4i - p2i
    vi, nvr = _S3 * (p4r - p2r), _S3 * (p4i + p2i)
    c0r, c0i = p1r + ur, p1i + ui
    tr, ti = p1r - 0.5 * ur, p1i - 0.5 * ui
    c1r, c1i, c2r, c2i = tr - nvr, ti + vi, tr + nvr, ti - vi
    br = [c0r, _C1 * c1r - _S1 * c1i, _C2 * c2r - _S2 * c2i]
    nbd = [_S3 * c0i,
           (_S3 * _S1) * c1r + (_S3 * _C1) * c1i,
           (_S3 * _S2) * c2r + (_S3 * _C2) * c2i]
    ny3 = _S3 * p3i
    t = p0 - 0.5 * p3r
    b0 = [p0 + p3r, t - ny3, t + ny3]
    y = [None] * 9
    for j in range(3):
        t = b0[j] - 0.5 * br[j]
        y[j] = b0[j] + br[j]
        y[3 + j] = t - nbd[j]
        y[6 + j] = t + nbd[j]
    return y


def _radix4(x, inverse):
    (ar, ai), (br, bi), (cr, ci), (dr, di) = x
    sr, si, er, ei = ar + cr, ai + ci, ar - cr, ai - ci
    tr, ti, fr, fi = br + dr, bi + di, br - dr, bi - di
    y1, y3 = (er + fi, ei - fr), (er - fi, ei + fr)
    if inverse:
        y1, y3 = y3, y1
    return [(sr + tr, si + ti), y1, (sr - tr, si - ti), y3]


def _twiddle16(z, e):
    e %= 16
    re, im = z
    if e == 0:
        return z
    if e == 4:
        return (im, -re)
    if e == 12:
        return (-im, re)
    c, s = math.cos(math.pi * e / 8), math.sin(math.pi * e / 8)
    if e % 4 == 2:
        if (c > 0) == (s > 0):
            return (c * (re + im), c * (im - re))
        return (c * (re - im), c * (im + re))
    return (c * re + s * im, c * im - s * re)


class _Stats:
    def __init__(self):
        self.s = [None, None]
        self.q = [None, None]
        self.n = 0

    def add(self, v):
        i = self.n % 2
        self.n += 1
        self.s[i] = v if self.s[i] is None else self.s[i] + v
        self.q[i] = v * v if self.q[i] is None else self.q[i] + v * v

    def scale_shift(self):
        mean = jnp.sum(self.s[0] + self.s[1], axis=0, keepdims=True) * (1.0 / D)
        msq = jnp.sum(self.q[0] + self.q[1], axis=0, keepdims=True) * (1.0 / D)
        r = lax.rsqrt(jnp.maximum(msq - mean * mean, 0.0) + EPS)
        return (jnp.broadcast_to(r, (8, 128)), jnp.broadcast_to(-mean * r, (8, 128)))


def _strassen_lhs(a11, a12, a21, a22):
    return [a11 + a22, a21 + a22, a11, a22, a11 + a12, a21 - a11, a12 - a22]


def _strassen_rhs(i, b11, b12, b21, b22):
    up = lambda b: b().astype(f32)
    return (lambda: up(b11) + up(b22), b11, lambda: up(b12) - up(b22),
            lambda: up(b21) - up(b11), b22, lambda: up(b11) + up(b12),
            lambda: up(b21) + up(b22))[i]()


def _strassen_out(m):
    return (m[0] + m[3] - m[4] + m[6], m[2] + m[4], m[1] + m[3], m[0] - m[1] + m[2] + m[5])


def _gelu(u):
    k0 = math.sqrt(2.0 / math.pi)
    th = jnp.tanh(u * (k0 + (k0 * 0.044715) * (u * u)))
    hu = 0.5 * u
    return hu + hu * th


def _kernel(x_hbm, wr_hbm, wi_hbm, w1_hbm, b1_hbm, w2_hbm, b2_hbm, c_hbm, wm_hbm,
            dm_hbm, sm_hbm, o_hbm,
            x_v, w_v, wn_v, wm_v, c_v, b1_v, b2_v, dm_v, sm_v, mod_v, g_tab, y_v,
            xd_v, v_v, u_v, z_v, wp_v, p_v, x1_v, t_v, h2_v, w1_v, w2_v, act_v,
            bias1_v, bias2_v, o_v, sem_in, sem_x, sem_w, sem_w1, sem_w2, sem_out):
    n1, n2 = F // FC, S // SC

    def copy_in(i, src, dst):
        return pltpu.make_async_copy(src, dst, sem_in.at[i])

    def wm_copy(i, lo, hi):
        return copy_in(i, wm_hbm.at[:, lo:hi], wm_v.at[:, lo:hi])

    cp_sm = copy_in(0, sm_hbm, sm_v)
    cp_c = copy_in(1, c_hbm, c_v)
    cp_wm = [wm_copy(2, 0, 1152), wm_copy(3, 1152, 2944), wm_copy(4, 2944, 6 * D)]
    cp_dm = copy_in(5, dm_hbm, dm_v)
    cp_b = [copy_in(6, b1_hbm, b1_v), copy_in(7, b2_hbm, b2_v)]
    cp_x = [pltpu.make_async_copy(x_hbm.at[:, 128 * (4 * a + b):128 * (4 * a + b + 1)],
                                  x_v.at[b, a], sem_x.at[b])
            for b in range(4) for a in range(4)]
    w_rows = (0, 80, 144, 224, 288)
    cp_w = [[pltpu.make_async_copy(src.at[w_rows[g]:w_rows[g + 1], :],
                                   w_v.at[pln, w_rows[g]:w_rows[g + 1], :], sem_w.at[2 * g + pln])
             for pln, src in enumerate((wr_hbm, wi_hbm))] for g in range(4)]
    cp_wn = [pltpu.make_async_copy(src.at[288:DF, :], wn_v.at[pln], sem_w.at[8 + pln])
             for pln, src in enumerate((wr_hbm, wi_hbm))]

    def w1_copy(j):
        return pltpu.make_async_copy(
            w1_hbm.at[:, pl.ds(pl.multiple_of(j * FC, FC), FC)], w1_v.at[j], sem_w1.at[j])

    def w2_copy(j):
        return pltpu.make_async_copy(
            w2_hbm.at[:, pl.ds(pl.multiple_of(j * SC, SC), SC)], w2_v.at[j], sem_w2.at[j])

    for cp in ([cp_sm, cp_c, cp_wm[0], cp_dm] + cp_x + sum(cp_w, []) + cp_wn
               + [cp_wm[1]] + cp_b + [cp_wm[2]]):
        cp.start()

    cp_sm.wait()
    for p in range(NB):
        for i in range(8):
            off = (256 if i == 0 else 320) + 16 - p
            hr, hi = sm_v[off:off + 16, :], sm_v[off + 32:off + 48, :]
            er, ei = sm_v[16 * i:16 * i + 16, :], sm_v[128 + 16 * i:144 + 16 * i, :]
            cr = er * hr - ei * hi
            ci = er * hi + ei * hr
            for t, m in enumerate((cr, ci - cr, cr + ci)):
                g_tab[p, t, 8 * i:8 * i + 8, :] = pltpu.bitcast(m.astype(bf16), jnp.int32)

    def modulation(lo, hi):
        cv = c_v[...].astype(f32)
        sc = jnp.broadcast_to(cv * jax.nn.sigmoid(cv), (8, D))
        m = _dot(sc, wm_v[:, lo:hi])
        col = lo + lax.broadcasted_iota(jnp.int32, m.shape, 1)
        which = lambda i: (col >= i * D) & (col < (i + 1) * D)
        m = jnp.where(which(1) | which(4), 1.0 + m, m)
        m = jnp.where(which(2), m * (1.0 / (S * D)), m)
        for t in range((hi - lo) // 128):
            row = jnp.broadcast_to(m[0:1, 128 * t:128 * (t + 1)], (128, 128))
            mod_v[lo + 128 * t:lo + 128 * (t + 1), :] = row.T

    def mod_tile(i, row):
        return mod_v[i * D + row:i * D + row + 8, :]

    cp_c.wait()
    cp_wm[0].wait()
    modulation(0, 1152)
    cp_dm.wait()

    def load_x(b, a, r):
        v = x_v[b, a, r:r + 16, :].astype(f32)
        return v[:8], v[8:]

    def phase1(b, carry):
        pltpu.make_async_copy(x_v.at[b], x_v.at[b], sem_x.at[b]).wait()
        for a in range(4):
            lanes = slice(128 * a, 128 * (a + 1))
            st = _Stats()
            for r in range(0, D, 16):
                for v in load_x(b, a, r):
                    st.add(v)
            rs, sh = st.scale_shift()
            for t in range(0, 64, 16):
                tiles = [load_x(b, a, 64 * j + t) for j in range(9)]
                for hf in range(2):
                    r = t + 8 * hf
                    h = [(tiles[j][hf] * rs + sh) * mod_tile(1, 64 * j + r)
                         + mod_tile(0, 64 * j + r) for j in range(9)]
                    y0, y = _radix9_fwd(h)
                    y_v[512 + r:520 + r, lanes] = y0
                    for q in range(1, 5):
                        y_v[128 * (q - 1) + r:128 * (q - 1) + r + 8, lanes] = y[q][0]
                        y_v[128 * (q - 1) + 64 + r:128 * (q - 1) + 72 + r, lanes] = y[q][1]

        def scatter(o, base, k0):
            for g in range(4):
                r = base + 16 * g
                t = _radix4([(o[r:r + 8, 128 * a:128 * (a + 1)],
                              o[r + 8:r + 16, 128 * a:128 * (a + 1)]) for a in range(4)], False)
                rows = pl.ds(72 * g + k0, 8, stride=9)
                for p0 in range(4):
                    xd_v[b, p0, 0, rows, :] = t[p0][0]
                    xd_v[b, p0, 1, rows, :] = t[p0][1]

        for q in range(1, 5):
            o = _dot(dm_v[_DF_OFF + 128 * (q - 1):_DF_OFF + 128 * q, :],
                     y_v[128 * (q - 1):128 * q, :])
            scatter(o, 0, q)
            scatter(o, 64, 9 - q)
        o = _dot(dm_v[_D0F_OFF:_D0F_OFF + 80, 0:64], y_v[512:576, :])
        scatter(o, 0, 0)
        n = [o[64:72, 128 * a:128 * (a + 1)] for a in range(4)]
        s02, d02, s13, d13 = n[0] + n[2], n[0] - n[2], n[1] + n[3], n[1] - n[3]
        zero = jnp.zeros((8, 128), f32)
        for p0, (re, im) in enumerate(((s02 + s13, zero), (d02, -d13), (s02 - s13, zero), (d02, d13))):
            xd_v[b, p0, 0, 288:296, :] = re
            xd_v[b, p0, 1, 288:296, :] = im
        return carry

    lax.fori_loop(0, 4, phase1, None)

    def start_w1(j, carry):
        w1_copy(j).start()
        return carry

    def start_w2(j, carry):
        w2_copy(j).start()
        return carry

    lax.fori_loop(0, n1, start_w1, None)
    lax.fori_loop(0, n2, start_w2, None)

    lane = lax.broadcasted_iota(jnp.int32, (8, 128), 1)
    lane_bit = [((lane >> t) & 1) == 1 for t in range(4)]

    def shuffle(v):
        v = [v[0]] + [pltpu.roll(v[a], a, 1) for a in range(15, 0, -1)]
        for t in range(4):
            v = [jnp.where(lane_bit[t], v[(p - (1 << t)) % NB], v[p]) for p in range(NB)]
        return v

    def w_unit(pln, r):
        v = [pltpu.bitcast(w_v[pln, r:r + 16, 128 * a:128 * (a + 1)], jnp.int32)
             for a in range(NB)]
        for p, w in enumerate(shuffle(v)):
            wp_v[pln, p, r:r + 16, :] = pltpu.bitcast(w, bf16).astype(f32)

    def w_last(pln):
        v = [jnp.broadcast_to(wn_v[pln, :, 128 * a:128 * (a + 1)].astype(f32), (8, 128))
             for a in range(NB)]
        for p, w in enumerate(shuffle(v)):
            wp_v[pln, p, 288:296, :] = w

    def w_jobs(g):
        jobs = [functools.partial(w_unit, pln, r)
                for r in range(w_rows[g], w_rows[g + 1], 16) for pln in range(2)]
        if g == 3:
            jobs += [functools.partial(w_last, pln) for pln in range(2)]
        return jobs

    def w_wait(g):
        for cp in cp_w[g] + (cp_wn if g == 3 else []):
            cp.wait()

    units = [(g, p0) for g in range(4) for p0 in range(4)]
    span = lambda g: (72 * g, 80 if g == 3 else 72)

    def stage_r(g, p0):
        r0, n = span(g)
        for r in range(r0, r0 + n, 8):
            x = [_twiddle16((xd_v[b, p0, 0, r:r + 8, :], xd_v[b, p0, 1, r:r + 8, :]), b * p0)
                 for b in range(4)]
            for p1, (re, im) in enumerate(_radix4(x, False)):
                v_v[p0 + 4 * p1, 0, r:r + 8, :] = re
                v_v[p0 + 4 * p1, 1, r:r + 8, :] = im

    def stage_q(g, p0):
        r0, _ = span(g)
        for q in range(9 + (g == 3)):
            src = pl.ds(r0 + q, 8, stride=9) if q < 9 else pl.ds(288, 8)
            dst = 32 * q + 8 * g if q < 9 else 288
            x = [(u_v[p0 + 4 * p1, 0, src, :], u_v[p0 + 4 * p1, 1, src, :]) for p1 in range(4)]
            for b, z in enumerate(_radix4(x, True)):
                re, im = _twiddle16(z, -b * p0)
                z_v[b, p0, 0, dst:dst + 8, :] = re
                z_v[b, p0, 1, dst:dst + 8, :] = im

    gmat = lambda p, t: pltpu.bitcast(g_tab[p, t], bf16)

    stage_r(*units[0])
    w_wait(0)
    for job in w_jobs(0):
        job()
    jobs = []
    for i, (g, p0) in enumerate(units):
        r0, n = span(g)
        rows = slice(r0, r0 + n)
        ps = [p0 + 4 * p1 for p1 in range(4)]
        spec = []
        for p in ps:
            a, b = v_v[p, 0, rows, :], v_v[p, 1, rows, :]
            k1 = _dot(a + b, gmat(p, 0), _NT)
            spec.append((k1 - _dot(b, gmat(p, 2), _NT), k1 + _dot(a, gmat(p, 1), _NT)))
        if i + 1 < len(units):
            stage_r(*units[i + 1])
        for p, (xr, xi) in zip(ps, spec):
            wr, wi = wp_v[0, p, rows, :], wp_v[1, p, rows, :]
            zr, zi = xr * wr - xi * wi, xr * wi + xi * wr
            k1 = _dot(zr + zi, gmat(p, 0))
            u_v[p, 0, rows, :] = k1 + _dot(zi, gmat(p, 1))
            u_v[p, 1, rows, :] = k1 - _dot(zr, gmat(p, 2))
        if i > 0:
            stage_q(*units[i - 1])
        if p0 == 0 and g < 3:
            w_wait(g + 1)
            jobs = w_jobs(g + 1)
        if p0 > 0:
            take = -(-len(jobs) // (4 - p0))
            for job in jobs[:take]:
                job()
            jobs = jobs[take:]
    stage_q(*units[-1])

    cp_wm[1].wait()
    modulation(1152, 2944)

    def phase3(b, carry):
        def gather(r):
            t = _radix4([(z_v[b, p0, 0, r:r + 8, :], z_v[b, p0, 1, r:r + 8, :])
                         for p0 in range(4)], True)
            return [jnp.concatenate([t[a][pln] for a in range(4)], 1) for pln in range(2)]

        for q in range(1, 5):
            rhs = jnp.concatenate(
                sum((gather(32 * k + 8 * g) for k in (q, 9 - q) for g in range(4)), []), 0)
            p_v[128 * (q - 1):128 * q, :] = _dot(
                dm_v[_DI_OFF + 128 * (q - 1):_DI_OFF + 128 * q, :], rhs)
        rhs = jnp.concatenate(sum((gather(8 * g) for g in range(4)), []) + gather(288)[:1], 0)
        p_v[512:576, :] = _dot(dm_v[_D0I_OFF:_D0I_OFF + 64, 0:72], rhs)

        norm = []
        for a in range(4):
            lanes = slice(128 * a, 128 * (a + 1))
            st = _Stats()
            for t in range(0, 64, 16):
                tiles = [load_x(b, a, 64 * j + t) for j in range(9)]
                for hf in range(2):
                    r = t + 8 * hf
                    y = _radix9_inv(
                        p_v[512 + r:520 + r, lanes],
                        {q: (p_v[128 * (q - 1) + r:128 * (q - 1) + r + 8, lanes],
                             p_v[128 * (q - 1) + 64 + r:128 * (q - 1) + 72 + r, lanes])
                         for q in range(1, 5)})
                    for j in range(9):
                        row = 64 * j + r
                        x1 = tiles[j][hf] + mod_tile(2, row) * y[j]
                        st.add(x1)
                        x1_v[a, b, row:row + 8, :] = x1
            rs, sh = st.scale_shift()
            st = _Stats()
            for row in range(0, D, 8):
                t = (x1_v[a, b, row:row + 8, :] * rs + sh) * mod_tile(4, row) + mod_tile(3, row)
                st.add(t)
                t_v[a, row:row + 8, :] = t
            norm.append(st.scale_shift())
        for a in range(2):
            for row in range(0, HD, 8):
                h = lambda k, r: t_v[k, r:r + 8, :] * norm[k][0] + norm[k][1]
                ops = _strassen_lhs(h(a, row), h(a + 2, row), h(a, HD + row), h(a + 2, HD + row))
                for i, v in enumerate(ops):
                    h2_v[i, a, b, row:row + 8, :] = v
        return carry

    lax.fori_loop(0, 4, phase3, None)

    for cp in cp_b + [cp_wm[2]]:
        cp.wait()
    modulation(2944, 6 * D)
    for src, dst, w in ((b1_v, bias1_v, FC), (b2_v, bias2_v, SC)):
        bv = src[...].astype(f32)
        for t in range(src.shape[0]):
            j, o = divmod(128 * t, w)
            dst[j, :, o:o + 128] = jnp.broadcast_to(bv[t:t + 1, :], (8, 128))

    fh, sh_ = FC // 2, SC // 2

    def mlp1(j, carry):
        w1_copy(j).wait()
        top, bot, lo, hi = slice(0, S // 2), slice(S // 2, S), slice(0, fh), slice(fh, FC)
        quad = [lambda r=r, c=c: w1_v[j, r, c] for r in (top, bot) for c in (lo, hi)]
        m = []
        for i in range(7):
            lhs = jnp.concatenate([h2_v[i, a, b] for a in range(2) for b in range(4)], 1)
            m.append(_dot(lhs, _strassen_rhs(i, *quad)))
        u = _strassen_out(m)
        act = [_gelu(v + bias1_v[j, 0:1, c]) for v, c in zip(u, (lo, hi, lo, hi))]
        for i, v in enumerate(_strassen_lhs(*act)):
            act_v[i, j] = v
        return carry

    lax.fori_loop(0, n1, mlp1, None)

    def out_copy(j):
        return pltpu.make_async_copy(
            o_v.at[j], o_hbm.at[:, pl.ds(pl.multiple_of(j * SC, SC), SC)], sem_out.at[j])

    def mlp2(j, carry):
        w2_copy(j).wait()
        lo, hi = slice(0, sh_), slice(sh_, SC)
        m = []
        for i in range(7):
            acc = None
            for k in range(n1):
                top, bot = slice(k * FC, k * FC + fh), slice(k * FC + fh, (k + 1) * FC)
                quad = [lambda r=r, c=c: w2_v[j, r, c] for r in (top, bot) for c in (lo, hi)]
                part = _dot(act_v[i, k], _strassen_rhs(i, *quad))
                acc = part if acc is None else acc + part
            m.append(acc)
        for y, rows, c0 in zip(_strassen_out(m), (0, 0, HD, HD), (0, sh_, 0, sh_)):
            gb = mod_v[5 * D + rows:5 * D + rows + HD, :]
            for i in range(sh_ // 128):
                col = c0 + 128 * i
                yb = y[:, 128 * i:128 * (i + 1)] + bias2_v[j, 0:1, col:col + 128]
                o_v[j, rows:rows + HD, col:col + 128] = (
                    x1_v[j, col // 128, rows:rows + HD, :] + gb * yb).astype(bf16)
        out_copy(j).start()
        return carry

    lax.fori_loop(0, n2, mlp2, None)
    for j in range(n2):
        out_copy(j).wait()


@jax.jit
def pallas_adaLN_cond__spectral_gfnet__mixer_token_mlp__prompt_kernel(
    A_x, A_w_r, A_w_i, B_x, B_w1, B_b1, B_w2, B_b2, c, w_mod,
):
    del B_x
    assert A_x.shape == (1, S, D) and SC == 512
    dmat, smat = _tables()
    n1, n2 = F // FC, S // SC
    vmem = pltpu.VMEM
    out_t = pl.pallas_call(
        _kernel,
        in_specs=[pl.BlockSpec(memory_space=pltpu.HBM)] * 11,
        out_specs=pl.BlockSpec(memory_space=pltpu.HBM),
        out_shape=jax.ShapeDtypeStruct((D, S), bf16),
        scratch_shapes=[
            vmem((4, 4, D, 128), bf16),
            vmem((2, 288, S), bf16),
            vmem((2, 1, S), bf16),
            vmem((D, 6 * D), bf16),
            vmem((1, D), bf16),
            vmem((F // 128, 128), bf16),
            vmem((S // 128, 128), bf16),
            vmem((_DROWS, 128), bf16),
            vmem((_SROWS, 128), f32),
            vmem((6 * D, 128), f32),
            vmem((NB, 3, 64, 128), jnp.int32),
            vmem((D, 512), f32),
            vmem((4, 4, 2, KR, 128), f32),
            vmem((NB, 2, KR, 128), f32),
            vmem((NB, 2, KR, 128), f32),
            vmem((4, 4, 2, KR, 128), f32),
            vmem((2, NB, KR, 128), f32),
            vmem((D, 512), f32),
            vmem((4, 4, D, 128), f32),
            vmem((4, D, 128), f32),
            vmem((7, 2, 4, HD, 128), f32),
            vmem((n1, S, FC), bf16),
            vmem((n2, F, SC), bf16),
            vmem((7, n1, HD, FC // 2), f32),
            vmem((n1, 8, FC), f32),
            vmem((n2, 8, SC), f32),
            vmem((n2, D, SC), bf16),
            pltpu.SemaphoreType.DMA((8,)),
            pltpu.SemaphoreType.DMA((4,)),
            pltpu.SemaphoreType.DMA((10,)),
            pltpu.SemaphoreType.DMA((n1,)),
            pltpu.SemaphoreType.DMA((n2,)),
            pltpu.SemaphoreType.DMA((n2,)),
        ],
        compiler_params=pltpu.CompilerParams(vmem_limit_bytes=124 * 1024 * 1024),
    )(
        A_x.reshape(S, D).T, A_w_r.T, A_w_i.T, B_w1, B_b1.reshape(F // 128, 128),
        B_w2, B_b2.reshape(S // 128, 128), c, w_mod,
        jnp.asarray(dmat, dtype=bf16), jnp.asarray(smat),
    )
    return out_t.T.reshape(1, S, D)
```

```python
import functools
import math

import jax
import jax.numpy as jnp
import numpy as np
from jax import lax
import jax.experimental.pallas as pl
import jax.experimental.pallas.tpu as pltpu

S, D, F = 2048, 576, 4608
DF = D // 2 + 1
KR = 296
NB = S // 128
QD = D // 4
SLOTS = 2
EPS = 1e-5
PROFILE = False
import contextlib
def _scope(n):
    return jax.named_scope(n) if PROFILE else contextlib.nullcontext()

f32 = jnp.float32
bf16 = jnp.bfloat16
_NN = (((1,), (0,)), ((), ()))
_NT = (((1,), (1,)), ((), ()))


def _dot(a, b, dims=_NN):
    return lax.dot_general(a, b, dims, preferred_element_type=f32)


@functools.lru_cache(maxsize=None)
def _tables():
    r = np.arange(64)
    kk = np.arange(32)
    th = lambda k: 2 * np.pi * np.outer(k, r) / D

    def weave(re, im):
        n = re.shape[1]
        return np.stack([re.reshape(4, 8, n), im.reshape(4, 8, n)], 1).reshape(64, n)

    fwd = []
    for q in range(1, 5):
        a, b = th(q + 9 * kk), th(9 - q + 9 * kk)
        fwd.append(np.concatenate([
            weave(np.block([np.cos(a), np.sin(a)]), np.block([-np.sin(a), np.cos(a)])),
            weave(np.block([np.cos(b), -np.sin(b)]), np.block([-np.sin(b), -np.cos(b)]))], 0))
    l0 = np.concatenate(
        [weave(np.cos(th(9 * kk)), -np.sin(th(9 * kk))), np.cos(th(np.array([D // 2])))], 0)
    cw = np.full((65, 1), 2.0)
    cw[0] = cw[64] = 1.0
    l0f = np.zeros((80, 128))
    l0f[:65, :64] = l0
    l0i = np.zeros((64, 128))
    l0i[:, :65] = (l0 * cw).T
    dmat = np.concatenate(fwd + [l0f] + [2 * m.T for m in fwd] + [l0i], 0)

    n2 = np.arange(128)
    a16 = np.arange(16)
    tw = lambda m: np.exp(-2j * np.pi * np.outer(m, n2) / S)
    e, r1, r2 = tw(n2), tw(127 * a16), tw(127 * a16 + 128)
    t1, t2 = np.concatenate([r2, r1], 0), np.concatenate([r1, r1], 0)
    smat = np.concatenate([e.real, e.imag, t1.real, t1.imag, t2.real, t2.imag], 0)
    return dmat.astype(np.float32), smat.astype(np.float32)


_DF_OFF = 0
_D0F_OFF = 512
_DI_OFF = 592
_D0I_OFF = 1104
_DROWS = 1168
_SROWS = 384

_S3 = math.sqrt(3.0) / 2
_C1, _S1 = math.cos(2 * math.pi / 9), math.sin(2 * math.pi / 9)
_C2, _S2 = math.cos(4 * math.pi / 9), math.sin(4 * math.pi / 9)


def _radix9_fwd(a):
    b0, br, bd = [], [], []
    for j in range(3):
        t = a[3 + j] + a[6 + j]
        b0.append(a[j] + t)
        br.append(a[j] - 0.5 * t)
        bd.append(a[3 + j] - a[6 + j])
    t = b0[1] + b0[2]
    y0 = b0[0] + t
    y3 = (b0[0] - 0.5 * t, _S3 * (b0[2] - b0[1]))
    c0r, c0i = br[0], -_S3 * bd[0]
    c1r = _C1 * br[1] - (_S3 * _S1) * bd[1]
    c1i = -_S1 * br[1] - (_S3 * _C1) * bd[1]
    c2r = _C2 * br[2] - (_S3 * _S2) * bd[2]
    c2i = -_S2 * br[2] - (_S3 * _C2) * bd[2]
    tr, ti = c1r + c2r, c1i + c2i
    y1 = (c0r + tr, c0i + ti)
    ur, ui = c0r - 0.5 * tr, c0i - 0.5 * ti
    nvr, vi = _S3 * (c2r - c1r), _S3 * (c1i - c2i)
    y4 = (ur + vi, ui + nvr)
    y2 = (ur - vi, nvr - ui)
    return y0, {1: y1, 2: y2, 3: y3, 4: y4}


def _radix9_inv(p0, p):
    (p1r, p1i), (p2r, p2i), (p3r, p3i), (p4r, p4i) = p[1], p[2], p[3], p[4]
    ur, ui = p4r + p2r, p4i - p2i
    vi, nvr = _S3 * (p4r - p2r), _S3 * (p4i + p2i)
    c0r, c0i = p1r + ur, p1i + ui
    tr, ti = p1r - 0.5 * ur, p1i - 0.5 * ui
    c1r, c1i, c2r, c2i = tr - nvr, ti + vi, tr + nvr, ti - vi
    br = [c0r, _C1 * c1r - _S1 * c1i, _C2 * c2r - _S2 * c2i]
    nbd = [_S3 * c0i,
           (_S3 * _S1) * c1r + (_S3 * _C1) * c1i,
           (_S3 * _S2) * c2r + (_S3 * _C2) * c2i]
    ny3 = _S3 * p3i
    t = p0 - 0.5 * p3r
    b0 = [p0 + p3r, t - ny3, t + ny3]
    y = [None] * 9
    for j in range(3):
        t = b0[j] - 0.5 * br[j]
        y[j] = b0[j] + br[j]
        y[3 + j] = t - nbd[j]
        y[6 + j] = t + nbd[j]
    return y


def _radix4(x, inverse):
    (ar, ai), (br, bi), (cr, ci), (dr, di) = x
    sr, si, er, ei = ar + cr, ai + ci, ar - cr, ai - ci
    tr, ti, fr, fi = br + dr, bi + di, br - dr, bi - di
    y1, y3 = (er + fi, ei - fr), (er - fi, ei + fr)
    if inverse:
        y1, y3 = y3, y1
    return [(sr + tr, si + ti), y1, (sr - tr, si - ti), y3]


def _twiddle16(z, e):
    e %= 16
    re, im = z
    if e == 0:
        return z
    if e == 4:
        return (im, -re)
    if e == 12:
        return (-im, re)
    c, s = math.cos(math.pi * e / 8), math.sin(math.pi * e / 8)
    if e % 4 == 2:
        if (c > 0) == (s > 0):
            return (c * (re + im), c * (im - re))
        return (c * (re - im), c * (im + re))
    return (c * re + s * im, c * im - s * re)


class _Stats:
    def __init__(self):
        self.s = [None, None]
        self.q = [None, None]
        self.n = 0

    def add(self, v):
        i = self.n % 2
        self.n += 1
        self.s[i] = v if self.s[i] is None else self.s[i] + v
        self.q[i] = v * v if self.q[i] is None else self.q[i] + v * v

    def scale_shift(self):
        mean = jnp.sum(self.s[0] + self.s[1], axis=0, keepdims=True) * (1.0 / D)
        msq = jnp.sum(self.q[0] + self.q[1], axis=0, keepdims=True) * (1.0 / D)
        r = lax.rsqrt(jnp.maximum(msq - mean * mean, 0.0) + EPS)
        return (jnp.broadcast_to(r, (8, 128)), jnp.broadcast_to(-mean * r, (8, 128)))


_LHS = (((0, 1), (3, 1)), ((2, 1), (3, 1)), ((0, 1),), ((3, 1),), ((0, 1), (1, 1)),
        ((2, 1), (0, -1)), ((1, 1), (3, -1)))
_RHS = (((0, 1), (3, 1)), ((0, 1),), ((1, 1), (3, -1)), ((2, 1), (0, -1)), ((3, 1),),
        ((0, 1), (1, 1)), ((2, 1), (3, 1)))
_OUT = (((0, 1), (3, 1), (4, -1), (6, 1)), ((2, 1), (4, 1)), ((1, 1), (3, 1)),
        ((0, 1), (1, -1), (2, 1), (5, 1)))
_ORDER = (1, 4, 3, 2, 0, 6, 5)


def _combine(terms, get):
    acc = get(terms[0][0])
    for q, sign in terms[1:]:
        acc = acc + get(q) if sign > 0 else acc - get(q)
    return acc


def _block(outer, inner):
    return 2 * (outer // 2) + inner // 2, 2 * (outer % 2) + inner % 2


class _Quadrants:
    def __init__(self):
        self.acc = [None] * 4
        self.left = [len(t) for t in _OUT]

    def add(self, i, m):
        done = []
        for c, terms in enumerate(_OUT):
            for q, sign in terms:
                if q != i:
                    continue
                prev = self.acc[c]
                if prev is None:
                    self.acc[c] = (m, sign)
                elif prev[1] == sign:
                    self.acc[c] = (prev[0] + m, sign)
                else:
                    self.acc[c] = (m - prev[0] if sign > 0 else prev[0] - m, 1)
                self.left[c] -= 1
                if self.left[c] == 0:
                    assert self.acc[c][1] > 0
                    done.append((c, self.acc[c][0]))
        return done


def _strassen2(lhs, raw, tiles, stage, emit):
    def prepare(n):
        i = _ORDER[n]
        if len(_RHS[i]) > 1:
            for c in range(4):
                for t in range(tiles):
                    stage[n % SLOTS, c, 128 * t:128 * (t + 1), :] = _combine(
                        _RHS[i], lambda q: raw(*_block(q, c), t, False).astype(f32))

    outer = [_Quadrants() for _ in range(4)]
    for n, i in enumerate(_ORDER):
        if n + 1 < 7:
            prepare(n + 1)
        inner = _Quadrants()
        for j in _ORDER:
            if len(_RHS[i]) > 1:
                rhs = _combine(_RHS[j], lambda c: stage[n % SLOTS, c, 0:128 * tiles, :])
            elif len(_RHS[j]) > 1:
                rhs = _combine(_RHS[j], lambda c: jnp.concatenate(
                    [raw(*_block(_RHS[i][0][0], c), t, False).astype(f32)
                     for t in range(tiles)], 0))
            else:
                rhs = jnp.concatenate(
                    [raw(*_block(_RHS[i][0][0], _RHS[j][0][0]), t, True)
                     for t in range(tiles)], 0)
            for c, v in inner.add(j, _dot(lhs(i, j), rhs)):
                for o, w in outer[c].add(i, v):
                    emit(*_block(o, c), w)


def _gelu(u):
    k0 = math.sqrt(2.0 / math.pi)
    th = jnp.tanh(u * (k0 + (k0 * 0.044715) * (u * u)))
    hu = 0.5 * u
    return hu + hu * th


def _kernel(x_hbm, wr_hbm, wi_hbm, w1_hbm, b1_hbm, w2_hbm, b2_hbm, c_hbm, wm_hbm,
            dm_hbm, sm_hbm, o_hbm,
            x_v, w_v, wm_v, sm_v, mod_v, g_tab, y_v, s_v, z_v, wp_v, x1_v, t_v, u_v, h_v, hs_v, w1_v, w2_v, stage_v, bias1_v, bias2_v, o_v, act_v, dm_v, wn_v, c_v, b1_v, b2_v, zero_s, sem_in, sem_w1, sem_w2, sem_out):
    n1, n2 = F // 512, S // 512
    c_v, b1_v = c_v.at[0], b1_v.at[0]
    packed = lambda ref: ref.bitcast(jnp.int32)
    unpack = lambda v: pltpu.bitcast(v, bf16)

    zero_s[0] = 0
    zero = zero_s[0]
    z_v, wp_v = z_v.at[zero], wp_v.at[zero]

    def copy_in(i, src, dst):
        return pltpu.make_async_copy(src, dst, sem_in.at[zero + i])

    def wm_copy(i, lo, hi):
        return copy_in(i, wm_hbm.at[:, lo:hi], wm_v.at[:, lo:hi])

    cp_sm = copy_in(0, sm_hbm, sm_v)
    cp_c = copy_in(1, c_hbm, c_v)
    cp_wm = [wm_copy(2, 0, 1152), wm_copy(3, 1152, 2944), wm_copy(4, 2944, 6 * D)]
    cp_dm = [copy_in(5, dm_hbm.at[0:_DI_OFF], dm_v.at[0:_DI_OFF]),
             copy_in(22, dm_hbm.at[_DI_OFF:_DROWS], dm_v.at[_DI_OFF:_DROWS])]
    cp_b = [copy_in(6, b1_hbm, b1_v), copy_in(7, b2_hbm, b2_v)]
    cp_x = [copy_in(8 + b, x_hbm.at[:, 128 * (4 * a + b):128 * (4 * a + b + 1)], x_v.at[b, a])
            for b in range(4) for a in range(4)]
    w_rows = (0, 144, 288)
    cp_w = [[copy_in(12 + 2 * g + pln, src.at[w_rows[g]:w_rows[g + 1], :],
                     w_v.at[pln, w_rows[g]:w_rows[g + 1], :])
             for pln, src in enumerate((wr_hbm, wi_hbm))] for g in range(2)]
    cp_w[1] += [copy_in(20 + pln, src.at[288:DF, :], wn_v.at[pln])
                for pln, src in enumerate((wr_hbm, wi_hbm))]
    cp_w10 = [copy_in(23, w1_hbm.at[:, 128 * n:128 * (n + 1)], w1_v.at[n]) for n in range(4)]

    for cp in ([cp_sm, cp_c, cp_wm[0], cp_dm[0]] + cp_x + cp_w[0] + [cp_dm[1]] + cp_w[1]
               + [cp_wm[1]] + cp_w10 + cp_b + [cp_wm[2]]):
        cp.start()

    with _scope('wait_sm'):
        cp_sm.wait()
    for p in range(NB):
        for i in range(8):
            off = (256 if i == 0 else 320) + 16 - p
            hr, hi = sm_v[off:off + 16, :], sm_v[off + 32:off + 48, :]
            er, ei = sm_v[16 * i:16 * i + 16, :], sm_v[128 + 16 * i:144 + 16 * i, :]
            cr = er * hr - ei * hi
            ci = er * hi + ei * hr
            for t, m in enumerate((cr, ci - cr, cr + ci)):
                g_tab[p, t, 16 * i:16 * i + 16, :] = m.astype(bf16)

    never = sm_v[0:8, :] > 2.0

    def after(v, token):
        return v if token is None else jnp.where(never, token, v)

    class Pace:
        def __init__(self, results, n):
            self.tiles = [(o, r) for o in results for r in range(0, o.shape[0], 8)]
            self.n, self.i = n, 0

        def __call__(self):
            if not self.tiles:
                return None
            o, r = self.tiles[min(self.i, self.n - 1) * len(self.tiles) // self.n]
            self.i += 1
            return o[r:r + 8, 0:128]

    def modulation(lo, hi):
        cv = c_v[...].astype(f32)
        sc = jnp.broadcast_to(cv * jax.nn.sigmoid(cv), (8, D))
        m = _dot(sc, wm_v[:, lo:hi])
        col = lo + lax.broadcasted_iota(jnp.int32, m.shape, 1)
        which = lambda i: (col >= i * D) & (col < (i + 1) * D)
        m = jnp.where(which(1) | which(4), 1.0 + m, m)
        m = jnp.where(which(2), m * (1.0 / (S * D)), m)
        for t in range((hi - lo) // 128):
            row = jnp.broadcast_to(m[0:1, 128 * t:128 * (t + 1)], (128, 128))
            mod_v[lo + 128 * t:lo + 128 * (t + 1), :] = row.T

    def mod_tile(i, row, n=8):
        return mod_v[i * D + row:i * D + row + n, :]

    with _scope('wait_wm0'):
        cp_c.wait()
        cp_wm[0].wait()
    modulation(0, 1152)
    cp_dm[0].wait()

    def load_x(b, a, r):
        v = x_v[b, a, r:r + 16, :].astype(f32)
        return v[:8], v[8:]

    def norm_radix9(b, pace):
        for a in range(4):
            lanes = slice(128 * a, 128 * (a + 1))
            st = _Stats()
            for r in range(0, D, 16):
                for v in load_x(b, a, r):
                    st.add(v)
            rs, sh = st.scale_shift()
            for t in range(0, 64, 16):
                tiles = [load_x(b, a, 64 * j + t) for j in range(9)]
                for hf in range(2):
                    r = t + 8 * hf
                    scale = after(rs, pace())
                    h = [(tiles[j][hf] * scale + sh) * mod_tile(1, 64 * j + r)
                         + mod_tile(0, 64 * j + r) for j in range(9)]
                    y0, y = _radix9_fwd(h)
                    y_v[b, 512 + r:520 + r, lanes] = y0
                    for q in range(1, 5):
                        y_v[b, 128 * (q - 1) + r:128 * (q - 1) + r + 8, lanes] = y[q][0]
                        y_v[b, 128 * (q - 1) + 64 + r:128 * (q - 1) + 72 + r, lanes] = y[q][1]

    def channel_dft(b):
        def scatter(o, base, k0):
            for g in range(4):
                r = base + 16 * g
                t = _radix4([(o[r:r + 8, 128 * a:128 * (a + 1)],
                              o[r + 8:r + 16, 128 * a:128 * (a + 1)]) for a in range(4)], False)
                rows = pl.ds(72 * g + k0, 8, stride=9)
                for p0 in range(4):
                    s_v[b, p0, 0, rows, :] = t[p0][0]
                    s_v[b, p0, 1, rows, :] = t[p0][1]

        results = []
        for q in range(1, 5):
            o = _dot(dm_v[_DF_OFF + 128 * (q - 1):_DF_OFF + 128 * q, :],
                     y_v[b, 128 * (q - 1):128 * q, :])
            results.append(o)
            scatter(o, 0, q)
            scatter(o, 64, 9 - q)
        o = _dot(dm_v[_D0F_OFF:_D0F_OFF + 80, 0:64], y_v[b, 512:576, :])
        scatter(o, 0, 0)
        n = [o[64:72, 128 * a:128 * (a + 1)] for a in range(4)]
        s02, d02, s13, d13 = n[0] + n[2], n[0] - n[2], n[1] + n[3], n[1] - n[3]
        nil = jnp.zeros((8, 128), f32)
        for p0, (re, im) in enumerate(((s02 + s13, nil), (d02, -d13), (s02 - s13, nil), (d02, d13))):
            s_v[b, p0, 0, 288:296, :] = re
            s_v[b, p0, 1, 288:296, :] = im
        return results + [o]

    for b in range(4):
        with _scope('wait_x'):
            pltpu.make_async_copy(x_v.at[b], x_v.at[b], sem_in.at[8 + b]).wait()
        norm_radix9(b, Pace(channel_dft(b - 1) if b > 0 else [], 32))

    def start_w1(n, carry):
        pltpu.make_async_copy(w1_hbm.at[:, pl.ds(pl.multiple_of(n * 128, 128), 128)],
                              w1_v.at[n], sem_w1.at[n // 4]).start()
        return carry

    def start_w2(n, carry):
        pltpu.make_async_copy(w2_hbm.at[:, pl.ds(pl.multiple_of(n * 128, 128), 128)],
                              w2_v.at[n], sem_w2.at[n // 4]).start()
        return carry

    lax.fori_loop(4, F // 128, start_w1, None)
    lax.fori_loop(0, S // 128, start_w2, None)

    lane = lax.broadcasted_iota(jnp.int32, (8, 128), 1)
    lane_bit = [((lane >> t) & 1) == 1 for t in range(4)]

    def shuffle(v, token):
        v = [v[0]] + [pltpu.roll(v[a], a, 1) for a in range(15, 0, -1)]
        bits = list(lane_bit)
        if token is not None:
            bits[0] = (after(lane, pltpu.bitcast(token, jnp.int32)) & 1) == 1
        for t in range(4):
            v = [jnp.where(bits[t], v[(p - (1 << t)) % NB], v[p]) for p in range(NB)]
        return v

    def reorder_filter(pln, r, token):
        if r < 288:
            v = [pltpu.bitcast(w_v[pln, r:r + 16, 128 * a:128 * (a + 1)], jnp.int32)
                 for a in range(NB)]
            for p, w in enumerate(shuffle(v, token)):
                wp_v[pln, p, r:r + 16, :] = unpack(w).astype(f32)
        else:
            v = [jnp.broadcast_to(wn_v[pln, :, 128 * a:128 * (a + 1)].astype(f32), (8, 128))
                 for a in range(NB)]
            for p, w in enumerate(shuffle(v, token)):
                wp_v[pln, p, 288:296, :] = w

    gmat = lambda p, t: unpack(packed(g_tab)[p, t])

    def token_filter(g, p0, pace):
        r0, n = 72 * g, (80 if g == 3 else 72)
        rows = slice(r0, r0 + n)
        for r in range(r0, r0 + n, 8):
            token = pace()
            x = [(s_v[b, p0, 0, r:r + 8, :], s_v[b, p0, 1, r:r + 8, :]) for b in range(4)]
            for b in range(2 if p0 == 0 else 4):
                if p0 == 0 or b > 0:
                    x[b] = (after(x[b][0], token), after(x[b][1], token))
            x = [_twiddle16(x[b], b * p0) for b in range(4)]
            for p1, (re, im) in enumerate(_radix4(x, False)):
                s_v[p1, p0, 0, r:r + 8, :] = re
                s_v[p1, p0, 1, r:r + 8, :] = im
        spec, results = [], []
        for p1 in range(4):
            p = p0 + 4 * p1
            a, b = s_v[p1, p0, 0, rows, :], s_v[p1, p0, 1, rows, :]
            k1 = _dot(a + b, gmat(p, 0), _NT)
            results.append(k1)
            spec.append((k1 - _dot(b, gmat(p, 2), _NT), k1 + _dot(a, gmat(p, 1), _NT)))
        for p1, (xr, xi) in enumerate(spec):
            p = p0 + 4 * p1
            wr, wi = wp_v[0, p, rows, :], wp_v[1, p, rows, :]
            zr, zi = xr * wr - xi * wi, xr * wi + xi * wr
            k1 = _dot(zr + zi, gmat(p, 0))
            results.append(k1)
            s_v[p1, p0, 0, rows, :] = k1 + _dot(zi, gmat(p, 1))
            s_v[p1, p0, 1, rows, :] = k1 - _dot(zr, gmat(p, 2))
        for q in range(9 + (g == 3)):
            src = pl.ds(r0 + q, 8, stride=9) if q < 9 else pl.ds(288, 8)
            dst = 32 * q + 8 * g if q < 9 else 288
            x = [(s_v[p1, p0, 0, src, :], s_v[p1, p0, 1, src, :]) for p1 in range(4)]
            for b, z in enumerate(_radix4(x, True)):
                re, im = _twiddle16(z, -b * p0)
                z_v[b, p0, 0, dst:dst + 8, :] = re
                z_v[b, p0, 1, dst:dst + 8, :] = im
        return results

    for half in range(2):
        with _scope('wait_w'):
            for cp in cp_w[half]:
                cp.wait()
        results = channel_dft(3) if half == 0 else []
        base = 144 * half
        first = [(pln, r) for r in range(base, base + 80, 16) for pln in range(2)]
        later = [(pln, r) for r in range(base + 80, base + 144 + 16 * half, 16) for pln in range(2)]
        pace = Pace(results, len(first))
        for pln, r in first:
            reorder_filter(pln, r, pace())
        results = []
        for i, (g, p0) in enumerate((g, p0) for g in (2 * half, 2 * half + 1) for p0 in range(4)):
            if 1 <= i <= 3:
                jobs = later[(i - 1) * len(later) // 3:i * len(later) // 3]
                pace = Pace(results[4:], len(jobs))
                for pln, r in jobs:
                    reorder_filter(pln, r, pace())
            results = token_filter(g, p0, Pace(results[:4], 10))

    with _scope('wait_wm1'):
        cp_dm[1].wait()
        cp_wm[1].wait()
    modulation(1152, 2944)

    def channel_idft(b):
        def gather(r):
            t = _radix4([(z_v[b, p0, 0, r:r + 8, :], z_v[b, p0, 1, r:r + 8, :])
                         for p0 in range(4)], True)
            return [jnp.concatenate([t[a][pln] for a in range(4)], 1) for pln in range(2)]

        results = []
        for q in range(1, 5):
            rhs = jnp.concatenate(
                sum((gather(32 * k + 8 * g) for k in (q, 9 - q) for g in range(4)), []), 0)
            results.append(_dot(dm_v[_DI_OFF + 128 * (q - 1):_DI_OFF + 128 * q, :], rhs))
            y_v[b, 128 * (q - 1):128 * q, :] = results[-1]
        rhs = jnp.concatenate(sum((gather(8 * g) for g in range(4)), []) + gather(288)[:1], 0)
        results.append(_dot(dm_v[_D0I_OFF:_D0I_OFF + 64, 0:72], rhs))
        y_v[b, 512:576, :] = results[-1]
        return results

    def residual_norms(b, pace):
        norm = []
        for a in range(4):
            lanes = slice(128 * a, 128 * (a + 1))
            st = _Stats()
            for t in range(0, 64, 16):
                tiles = [load_x(b, a, 64 * j + t) for j in range(9)]
                for hf in range(2):
                    r = t + 8 * hf
                    p = {q: (y_v[b, 128 * (q - 1) + r:128 * (q - 1) + r + 8, lanes],
                             y_v[b, 128 * (q - 1) + 64 + r:128 * (q - 1) + 72 + r, lanes])
                         for q in range(1, 5)}
                    token = pace()
                    for q in (3, 4):
                        p[q] = (after(p[q][0], token), after(p[q][1], token))
                    y = _radix9_inv(y_v[b, 512 + r:520 + r, lanes], p)
                    for j in range(9):
                        row = 64 * j + r
                        x1 = tiles[j][hf] + mod_tile(2, row) * y[j]
                        st.add(x1)
                        x1_v[a, b, row:row + 8, :] = x1
            rs, sh = st.scale_shift()
            st = _Stats()
            for row in range(0, D, 8):
                if row % 120 == 0:
                    scale = after(rs, pace())
                t = (x1_v[a, b, row:row + 8, :] * scale + sh) * mod_tile(4, row) + mod_tile(3, row)
                st.add(t)
                t_v[a, row:row + 8, :] = t
            rs, sh = st.scale_shift()
            norm.append((rs, jnp.concatenate([sh, sh], 0)))
        for row in range(0, QD, 16):
            h = {}
            for k in range(4):
                if k < 3:
                    token = pace()
                scale = after(norm[k][0], token)
                scale = jnp.concatenate([scale, scale], 0)
                for r in range(4):
                    rows = slice(QD * r + row, QD * r + row + 16)
                    h[r, k] = t_v[k, rows, :] * scale + norm[k][1]
                    h_v[b, k, rows, :] = h[r, k].astype(bf16)
            for i in range(7):
                quad = [_combine(_LHS[i], lambda o: h[_block(o, c)]) for c in range(4)]
                for j in range(7):
                    hs_v[i, j, b, row:row + 16, :] = _combine(
                        _LHS[j], lambda c: quad[c]).astype(bf16)

    def first_chunk(b):
        lhs = jnp.concatenate([unpack(packed(h_v)[b, a]) for a in range(4)], 1)
        rhs = jnp.concatenate([jnp.concatenate(
            [unpack(packed(w1_v)[n, pl.ds(pl.multiple_of(64 * (4 * a + b), 64), 64), :])
             for a in range(4)], 0) for n in range(4)], 1)
        return _dot(lhs, rhs)

    steps = 4 * (8 + 5) + 27
    channel_idft(0)
    residual_norms(0, Pace(sum((channel_idft(b) for b in range(1, 4)), []), steps))
    with _scope('wait_w10'):
        pltpu.make_async_copy(w1_v.at[0:4], w1_v.at[0:4], sem_in.at[23]).wait()
    u_v[...] = jnp.zeros(u_v.shape, f32)

    def overlap(b, carry):
        part = first_chunk(b)
        u_v[...] += part
        residual_norms(b + 1, Pace([part[:, 128 * n:128 * (n + 1)] for n in range(4)], steps))
        return carry

    with _scope('phase3'):
        lax.fori_loop(0, 3, overlap, None)

    with _scope('wait_b'):
        for cp in cp_b + [cp_wm[2]]:
            cp.wait()
    modulation(2944, 6 * D)
    for src, dst in ((b1_v, bias1_v), (b2_v, bias2_v)):
        bv = src[...].astype(f32)
        for t in range(src.shape[0]):
            dst[t] = jnp.broadcast_to(bv[t:t + 1, :], (8, 128))

    def activate(j):
        g, made = {}, set()

        def emit(r, n, u):
            g[r, n] = _gelu(u + bias1_v[4 * j + n, 0:1, :])
            for i in range(7):
                for k in range(7):
                    need = [_block(o, c) for o, _ in _LHS[i] for c, _ in _LHS[k]]
                    if (i, k) not in made and all(e in g for e in need):
                        made.add((i, k))
                        act_v[i, k, j] = _combine(_LHS[k], lambda c: _combine(
                            _LHS[i], lambda o: g[_block(o, c)])).astype(bf16)
        return emit

    u0 = u_v[...] + first_chunk(3)
    emit0 = activate(0)
    for r in range(4):
        for n in range(4):
            emit0(r, n, u0[QD * r:QD * (r + 1), 128 * n:128 * (n + 1)])

    def mlp1(j, carry):
        with _scope('wait_w1'):
            pltpu.make_async_copy(w1_v.at[0:4], w1_v.at[0:4], sem_w1.at[j]).wait()

        def raw(k, n, t, keep_packed):
            if keep_packed:
                return unpack(packed(w1_v)[4 * j + n, 256 * k + 64 * t:256 * k + 64 * (t + 1), :])
            return w1_v[4 * j + n, 512 * k + 128 * t:512 * k + 128 * (t + 1), :]

        lhs = lambda i, k: jnp.concatenate([unpack(packed(hs_v)[i, k, t]) for t in range(4)], 1)
        _strassen2(lhs, raw, 4, stage_v, activate(j))
        return carry

    with _scope('mlp1'):
        lax.fori_loop(1, n1, mlp1, None)

    def out_copy(j, n):
        return pltpu.make_async_copy(
            o_v.at[j, n], o_hbm.at[:, pl.ds(pl.multiple_of((4 * j + n) * 128, 128), 128)],
            sem_out.at[0])

    def mlp2(j, carry):
        with _scope('wait_w2'):
            pltpu.make_async_copy(w2_v.at[0:4], w2_v.at[0:4], sem_w2.at[j]).wait()

        def raw(k, n, t, keep_packed):
            if keep_packed:
                return unpack(packed(w2_v)[4 * j + n, 64 * (4 * t + k):64 * (4 * t + k + 1), :])
            return w2_v[4 * j + n, 128 * (4 * t + k):128 * (4 * t + k + 1), :]

        def emit(r, n, y):
            rows = slice(QD * r, QD * (r + 1))
            y = y + bias2_v[4 * j + n, 0:1, :]
            o_v[j, n, rows, :] = (x1_v[j, n, rows, :] + mod_tile(5, QD * r, QD) * y).astype(bf16)

        lhs = lambda i, k: jnp.concatenate([unpack(packed(act_v)[i, k, t]) for t in range(n1)], 1)
        _strassen2(lhs, raw, n1, stage_v, emit)
        for n in range(4):
            out_copy(j, n).start()
        return carry

    with _scope('mlp2'):
        lax.fori_loop(0, n2, mlp2, None)
    with _scope('wait_out'):
        pltpu.make_async_copy(o_v, o_v, sem_out.at[0]).wait()


@jax.jit
def pallas_adaLN_cond__spectral_gfnet__mixer_token_mlp__prompt_kernel(
    A_x, A_w_r, A_w_i, B_x, B_w1, B_b1, B_w2, B_b2, c, w_mod,
):
    del B_x
    assert A_x.shape == (1, S, D)
    dmat, smat = _tables()
    n1, n2 = F // 512, S // 512
    vmem = pltpu.VMEM
    out_t = pl.pallas_call(
        _kernel,
        in_specs=[pl.BlockSpec(memory_space=pltpu.HBM)] * 11,
        out_specs=pl.BlockSpec(memory_space=pltpu.HBM),
        out_shape=jax.ShapeDtypeStruct((D, S), bf16),
        scratch_shapes=[
            vmem((4, 4, D, 128), bf16),
            vmem((2, 288, S), bf16),
            vmem((D, 6 * D), bf16),
            vmem((_SROWS, 128), f32),
            vmem((6 * D, 128), f32),
            vmem((NB, 3, 128, 128), bf16),
            vmem((4, D, 512), f32),
            vmem((4, 4, 2, KR, 128), f32),
            vmem((1, 4, 4, 2, KR, 128), f32),
            vmem((1, 2, NB, KR, 128), f32),
            vmem((4, 4, D, 128), f32),
            vmem((4, D, 128), f32),
            vmem((D, 512), f32),
            vmem((4, 4, D, 128), bf16),
            vmem((7, 7, 4, QD, 128), bf16),
            vmem((F // 128, S, 128), bf16),
            vmem((S // 128, F, 128), bf16),
            vmem((SLOTS, 4, F // 4, 128), f32),
            vmem((F // 128, 8, 128), f32),
            vmem((S // 128, 8, 128), f32),
            vmem((4, 4, D, 128), bf16),
            vmem((7, 7, n1, QD, 128), bf16),
            vmem((_DROWS, 128), bf16),
            vmem((2, 1, S), bf16),
            vmem((8, 1, D), bf16),
            vmem((2, F // 128, 128), bf16),
            vmem((S // 128, 128), bf16),
            pltpu.SMEM((1,), jnp.int32),
            pltpu.SemaphoreType.DMA((24,)),
            pltpu.SemaphoreType.DMA((n1,)),
            pltpu.SemaphoreType.DMA((n2,)),
            pltpu.SemaphoreType.DMA((1,)),
        ],
        compiler_params=pltpu.CompilerParams(vmem_limit_bytes=124 * 1024 * 1024),
    )(
        A_x.reshape(S, D).T, A_w_r.T, A_w_i.T, B_w1, B_b1.reshape(F // 128, 128),
        B_w2, B_b2.reshape(S // 128, 128), c, w_mod,
        jnp.asarray(dmat, dtype=bf16), jnp.asarray(smat),
    )
    return out_t.T.reshape(1, S, D)
```

```python
import functools
import math

import jax
import jax.numpy as jnp
import numpy as np
from jax import lax
import jax.experimental.pallas as pl
import jax.experimental.pallas.tpu as pltpu

S, D, F = 2048, 576, 4608
DF = D // 2 + 1
KR = 296
NB = S // 128
QD = D // 4
SLOTS = 3
WJOB = lambda fwd, inv: inv
EPS = 1e-5
PROFILE = False
import contextlib
def _scope(n):
    return jax.named_scope(n) if PROFILE else contextlib.nullcontext()

f32 = jnp.float32
bf16 = jnp.bfloat16
_NN = (((1,), (0,)), ((), ()))
_NT = (((1,), (1,)), ((), ()))


def _dot(a, b, dims=_NN):
    return lax.dot_general(a, b, dims, preferred_element_type=f32)


@functools.lru_cache(maxsize=None)
def _tables():
    r = np.arange(64)
    kk = np.arange(32)
    th = lambda k: 2 * np.pi * np.outer(k, r) / D

    def weave(re, im):
        n = re.shape[1]
        return np.stack([re.reshape(4, 8, n), im.reshape(4, 8, n)], 1).reshape(64, n)

    fwd = []
    for q in range(1, 5):
        a, b = th(q + 9 * kk), th(9 - q + 9 * kk)
        fwd.append(np.concatenate([
            weave(np.block([np.cos(a), np.sin(a)]), np.block([-np.sin(a), np.cos(a)])),
            weave(np.block([np.cos(b), -np.sin(b)]), np.block([-np.sin(b), -np.cos(b)]))], 0))
    l0 = np.concatenate(
        [weave(np.cos(th(9 * kk)), -np.sin(th(9 * kk))), np.cos(th(np.array([D // 2])))], 0)
    cw = np.full((65, 1), 2.0)
    cw[0] = cw[64] = 1.0
    l0f = np.zeros((80, 128))
    l0f[:65, :64] = l0
    l0i = np.zeros((64, 128))
    l0i[:, :65] = (l0 * cw).T
    dmat = np.concatenate(fwd + [l0f] + [2 * m.T for m in fwd] + [l0i], 0)

    n2 = np.arange(128)
    a16 = np.arange(16)
    tw = lambda m: np.exp(-2j * np.pi * np.outer(m, n2) / S)
    e, r1, r2 = tw(n2), tw(127 * a16), tw(127 * a16 + 128)
    t1, t2 = np.concatenate([r2, r1], 0), np.concatenate([r1, r1], 0)
    smat = np.concatenate([e.real, e.imag, t1.real, t1.imag, t2.real, t2.imag], 0)
    return dmat.astype(np.float32), smat.astype(np.float32)


_DF_OFF = 0
_D0F_OFF = 512
_DI_OFF = 592
_D0I_OFF = 1104
_DROWS = 1168
_SROWS = 384

_S3 = math.sqrt(3.0) / 2
_C1, _S1 = math.cos(2 * math.pi / 9), math.sin(2 * math.pi / 9)
_C2, _S2 = math.cos(4 * math.pi / 9), math.sin(4 * math.pi / 9)


def _radix9_fwd(a):
    b0, br, bd = [], [], []
    for j in range(3):
        t = a[3 + j] + a[6 + j]
        b0.append(a[j] + t)
        br.append(a[j] - 0.5 * t)
        bd.append(a[3 + j] - a[6 + j])
    t = b0[1] + b0[2]
    y0 = b0[0] + t
    y3 = (b0[0] - 0.5 * t, _S3 * (b0[2] - b0[1]))
    c0r, c0i = br[0], -_S3 * bd[0]
    c1r = _C1 * br[1] - (_S3 * _S1) * bd[1]
    c1i = -_S1 * br[1] - (_S3 * _C1) * bd[1]
    c2r = _C2 * br[2] - (_S3 * _S2) * bd[2]
    c2i = -_S2 * br[2] - (_S3 * _C2) * bd[2]
    tr, ti = c1r + c2r, c1i + c2i
    y1 = (c0r + tr, c0i + ti)
    ur, ui = c0r - 0.5 * tr, c0i - 0.5 * ti
    nvr, vi = _S3 * (c2r - c1r), _S3 * (c1i - c2i)
    y4 = (ur + vi, ui + nvr)
    y2 = (ur - vi, nvr - ui)
    return y0, {1: y1, 2: y2, 3: y3, 4: y4}


def _radix9_inv(p0, p):
    (p1r, p1i), (p2r, p2i), (p3r, p3i), (p4r, p4i) = p[1], p[2], p[3], p[4]
    ur, ui = p4r + p2r, p4i - p2i
    vi, nvr = _S3 * (p4r - p2r), _S3 * (p4i + p2i)
    c0r, c0i = p1r + ur, p1i + ui
    tr, ti = p1r - 0.5 * ur, p1i - 0.5 * ui
    c1r, c1i, c2r, c2i = tr - nvr, ti + vi, tr + nvr, ti - vi
    br = [c0r, _C1 * c1r - _S1 * c1i, _C2 * c2r - _S2 * c2i]
    nbd = [_S3 * c0i,
           (_S3 * _S1) * c1r + (_S3 * _C1) * c1i,
           (_S3 * _S2) * c2r + (_S3 * _C2) * c2i]
    ny3 = _S3 * p3i
    t = p0 - 0.5 * p3r
    b0 = [p0 + p3r, t - ny3, t + ny3]
    y = [None] * 9
    for j in range(3):
        t = b0[j] - 0.5 * br[j]
        y[j] = b0[j] + br[j]
        y[3 + j] = t - nbd[j]
        y[6 + j] = t + nbd[j]
    return y


def _radix4(x, inverse):
    (ar, ai), (br, bi), (cr, ci), (dr, di) = x
    sr, si, er, ei = ar + cr, ai + ci, ar - cr, ai - ci
    tr, ti, fr, fi = br + dr, bi + di, br - dr, bi - di
    y1, y3 = (er + fi, ei - fr), (er - fi, ei + fr)
    if inverse:
        y1, y3 = y3, y1
    return [(sr + tr, si + ti), y1, (sr - tr, si - ti), y3]


def _twiddle16(z, e):
    e %= 16
    re, im = z
    if e == 0:
        return z
    if e == 4:
        return (im, -re)
    if e == 12:
        return (-im, re)
    c, s = math.cos(math.pi * e / 8), math.sin(math.pi * e / 8)
    if e % 4 == 2:
        if (c > 0) == (s > 0):
            return (c * (re + im), c * (im - re))
        return (c * (re - im), c * (im + re))
    return (c * re + s * im, c * im - s * re)


class _Stats:
    def __init__(self):
        self.s = [None, None]
        self.q = [None, None]
        self.n = 0

    def add(self, v):
        i = self.n % 2
        self.n += 1
        self.s[i] = v if self.s[i] is None else self.s[i] + v
        self.q[i] = v * v if self.q[i] is None else self.q[i] + v * v

    def scale_shift(self):
        mean = jnp.sum(self.s[0] + self.s[1], axis=0, keepdims=True) * (1.0 / D)
        msq = jnp.sum(self.q[0] + self.q[1], axis=0, keepdims=True) * (1.0 / D)
        r = lax.rsqrt(jnp.maximum(msq - mean * mean, 0.0) + EPS)
        return (jnp.broadcast_to(r, (8, 128)), jnp.broadcast_to(-mean * r, (8, 128)))


_LHS = (((0, 1), (3, 1)), ((2, 1), (3, 1)), ((0, 1),), ((3, 1),), ((0, 1), (1, 1)),
        ((2, 1), (0, -1)), ((1, 1), (3, -1)))
_RHS = (((0, 1), (3, 1)), ((0, 1),), ((1, 1), (3, -1)), ((2, 1), (0, -1)), ((3, 1),),
        ((0, 1), (1, 1)), ((2, 1), (3, 1)))
_OUT = (((0, 1), (3, 1), (4, -1), (6, 1)), ((2, 1), (4, 1)), ((1, 1), (3, 1)),
        ((0, 1), (1, -1), (2, 1), (5, 1)))
_ORDER = (1, 4, 2, 0, 5, 3, 6)


def _combine(terms, get):
    acc = get(terms[0][0])
    for q, sign in terms[1:]:
        acc = acc + get(q) if sign > 0 else acc - get(q)
    return acc


def _block(outer, inner):
    return 2 * (outer // 2) + inner // 2, 2 * (outer % 2) + inner % 2


class _Quadrants:
    def __init__(self):
        self.acc = [None] * 4
        self.left = [len(t) for t in _OUT]

    def add(self, i, m):
        done = []
        for c, terms in enumerate(_OUT):
            for q, sign in terms:
                if q != i:
                    continue
                prev = self.acc[c]
                if prev is None:
                    self.acc[c] = (m, sign)
                elif prev[1] == sign:
                    self.acc[c] = (prev[0] + m, sign)
                else:
                    self.acc[c] = (m - prev[0] if sign > 0 else prev[0] - m, 1)
                self.left[c] -= 1
                if self.left[c] == 0:
                    assert self.acc[c][1] > 0
                    done.append((c, self.acc[c][0]))
        return done


def _strassen2(lhs, raw, tiles, stage, emit):
    def prepare(n):
        i = _ORDER[n]
        if len(_RHS[i]) > 1:
            for c in range(4):
                for t in range(tiles):
                    stage[n % SLOTS, c, 128 * t:128 * (t + 1), :] = _combine(
                        _RHS[i], lambda q: raw(*_block(q, c), t, False).astype(f32))

    outer = [_Quadrants() for _ in range(4)]
    for n, i in enumerate(_ORDER):
        if n + 1 < 7:
            prepare(n + 1)
        inner = _Quadrants()
        for j in _ORDER:
            if len(_RHS[i]) > 1:
                rhs = _combine(_RHS[j], lambda c: stage[n % SLOTS, c, 0:128 * tiles, :])
            elif len(_RHS[j]) > 1:
                rhs = _combine(_RHS[j], lambda c: jnp.concatenate(
                    [raw(*_block(_RHS[i][0][0], c), t, False).astype(f32)
                     for t in range(tiles)], 0))
            else:
                rhs = jnp.concatenate(
                    [raw(*_block(_RHS[i][0][0], _RHS[j][0][0]), t, True)
                     for t in range(tiles)], 0)
            for c, v in inner.add(j, _dot(lhs(i, j), rhs.astype(bf16))):
                for o, w in outer[c].add(i, v):
                    emit(*_block(o, c), w)


def _gelu(u):
    k0 = math.sqrt(2.0 / math.pi)
    th = jnp.tanh(u * (k0 + (k0 * 0.044715) * (u * u)))
    hu = 0.5 * u
    return hu + hu * th


def _kernel(x_hbm, wr_hbm, wi_hbm, w1_hbm, b1_hbm, w2_hbm, b2_hbm, c_hbm, wm_hbm,
            dm_hbm, sm_hbm, o_hbm,
            x_v, w_v, wm_v, sm_v, mod_v, g_tab, y_v, s_v, z_v, wp_v, x1_v, t_v, u_v, h_v, hs_v, w1_v, w2_v, stage_v, bias1_v, bias2_v, o_v, act_v, dm_v, wn_v, c_v, b1_v, b2_v, zero_s, sem_in, sem_w1, sem_w2, sem_out):
    n1, n2 = F // 512, S // 512
    c_v, b1_v = c_v.at[0], b1_v.at[0]
    packed = lambda ref: ref.bitcast(jnp.int32)
    unpack = lambda v: pltpu.bitcast(v, bf16)

    zero_s[0] = 0
    zero = zero_s[0]
    z_v, wp_v = z_v.at[zero], wp_v.at[zero]

    def copy_in(i, src, dst):
        return pltpu.make_async_copy(src, dst, sem_in.at[zero + i])

    def wm_copy(i, lo, hi):
        return copy_in(i, wm_hbm.at[:, lo:hi], wm_v.at[:, lo:hi])

    cp_sm = copy_in(0, sm_hbm, sm_v)
    cp_c = copy_in(1, c_hbm, c_v)
    cp_wm = [wm_copy(2, 0, 1152), wm_copy(3, 1152, 2944), wm_copy(4, 2944, 6 * D)]
    cp_dm = [copy_in(5, dm_hbm.at[0:_DI_OFF], dm_v.at[0:_DI_OFF]),
             copy_in(22, dm_hbm.at[_DI_OFF:_DROWS], dm_v.at[_DI_OFF:_DROWS])]
    cp_b = [copy_in(6, b1_hbm, b1_v), copy_in(7, b2_hbm, b2_v)]
    cp_x = [copy_in(8 + b, x_hbm.at[:, 128 * (4 * a + b):128 * (4 * a + b + 1)], x_v.at[b, a])
            for b in range(4) for a in range(4)]
    w_rows = (0, 144, 288)
    cp_w = [[copy_in(12 + 2 * g + pln, src.at[w_rows[g]:w_rows[g + 1], :],
                     w_v.at[pln, w_rows[g]:w_rows[g + 1], :])
             for pln, src in enumerate((wr_hbm, wi_hbm))] for g in range(2)]
    cp_w[1] += [copy_in(20 + pln, src.at[288:DF, :], wn_v.at[pln])
                for pln, src in enumerate((wr_hbm, wi_hbm))]
    cp_w10 = [copy_in(23, w1_hbm.at[:, 128 * n:128 * (n + 1)], w1_v.at[n]) for n in range(4)]

    for cp in ([cp_sm, cp_c, cp_wm[0], cp_dm[0]] + cp_x + cp_w[0] + cp_w[1] + [cp_dm[1]]
               + [cp_wm[1]] + cp_w10 + cp_b + [cp_wm[2]]):
        cp.start()

    def column(n):
        return pl.ds(n * 128 if isinstance(n, int) else pl.multiple_of(n * 128, 128), 128)

    def start_w1(j):
        for n in range(4):
            pltpu.make_async_copy(
                w1_hbm.at[:, column(4 * j + n)], w1_v.at[4 * j + n], sem_w1.at[j]).start()

    def start_w2(j):
        for n in range(2):
            pltpu.make_async_copy(
                w2_hbm.at[:, column(2 * j + n)], w2_v.at[2 * j + n], sem_w2.at[j // 2]).start()

    @pl.loop(0, D // 8)
    def _(i):
        u_v[pl.ds(pl.multiple_of(8 * i, 8), 8), :] = jnp.zeros((8, 512), f32)

    with _scope('wait_sm'):
        cp_sm.wait()

    @pl.loop(0, NB)
    def _(p):
        for i in range(8):
            off = (256 if i == 0 else 320) + 16 - p
            hr, hi = sm_v[pl.ds(off, 16), :], sm_v[pl.ds(off + 32, 16), :]
            er, ei = sm_v[16 * i:16 * i + 16, :], sm_v[128 + 16 * i:144 + 16 * i, :]
            cr = er * hr - ei * hi
            ci = er * hi + ei * hr
            for t, m in enumerate((cr, ci - cr, cr + ci)):
                g_tab[p, t, 16 * i:16 * i + 16, :] = m.astype(bf16)

    never = sm_v[0:8, :] > 2.0

    def after(v, token):
        return v if token is None else jnp.where(never, token, v)

    class Pace:
        def __init__(self, results, n):
            self.tiles = [(o, r) for o in results for r in range(0, o.shape[0], 8)]
            self.n, self.i = n, 0

        def __call__(self):
            if not self.tiles:
                return None
            o, r = self.tiles[min(self.i, self.n - 1) * len(self.tiles) // self.n]
            self.i += 1
            return o[r:r + 8, 0:128]

    def modulation(lo, hi):
        cv = c_v[...].astype(f32)
        sc = jnp.broadcast_to(cv * jax.nn.sigmoid(cv), (8, D))
        m = _dot(sc, wm_v[:, lo:hi])
        col = lo + lax.broadcasted_iota(jnp.int32, m.shape, 1)
        which = lambda i: (col >= i * D) & (col < (i + 1) * D)
        m = jnp.where(which(1) | which(4), 1.0 + m, m)
        m = jnp.where(which(2), m * (1.0 / (S * D)), m)
        for t in range((hi - lo) // 128):
            row = jnp.broadcast_to(m[0:1, 128 * t:128 * (t + 1)], (128, 128))
            mod_v[lo + 128 * t:lo + 128 * (t + 1), :] = row.T

    def mod_tile(i, row, n=8):
        return mod_v[i * D + row:i * D + row + n, :]

    with _scope('wait_wm0'):
        cp_c.wait()
        cp_wm[0].wait()
    modulation(0, 1152)
    cp_dm[0].wait()

    def load_x(b, a, r):
        v = x_v[b, a, r:r + 16, :].astype(f32)
        return v[:8], v[8:]

    def norm_radix9(b, pace):
        for a in range(4):
            lanes = slice(128 * a, 128 * (a + 1))
            st = _Stats()
            for r in range(0, D, 16):
                for v in load_x(b, a, r):
                    st.add(v)
            rs, sh = st.scale_shift()
            for t in range(0, 64, 16):
                tiles = [load_x(b, a, 64 * j + t) for j in range(9)]
                for hf in range(2):
                    r = t + 8 * hf
                    scale = after(rs, pace())
                    h = [(tiles[j][hf] * scale + sh) * mod_tile(1, 64 * j + r)
                         + mod_tile(0, 64 * j + r) for j in range(9)]
                    y0, y = _radix9_fwd(h)
                    y_v[b, 512 + r:520 + r, lanes] = y0
                    for q in range(1, 5):
                        y_v[b, 128 * (q - 1) + r:128 * (q - 1) + r + 8, lanes] = y[q][0]
                        y_v[b, 128 * (q - 1) + 64 + r:128 * (q - 1) + 72 + r, lanes] = y[q][1]

    def channel_dft(b):
        def scatter(o, base, k0):
            for g in range(4):
                r = base + 16 * g
                t = _radix4([(o[r:r + 8, 128 * a:128 * (a + 1)],
                              o[r + 8:r + 16, 128 * a:128 * (a + 1)]) for a in range(4)], False)
                rows = pl.ds(72 * g + k0, 8, stride=9)
                for p0 in range(4):
                    s_v[b, p0, 0, rows, :] = t[p0][0]
                    s_v[b, p0, 1, rows, :] = t[p0][1]

        results = []
        for q in range(1, 5):
            o = _dot(dm_v[_DF_OFF + 128 * (q - 1):_DF_OFF + 128 * q, :],
                     y_v[b, 128 * (q - 1):128 * q, :])
            results.append(o)
            scatter(o, 0, q)
            scatter(o, 64, 9 - q)
        o = _dot(dm_v[_D0F_OFF:_D0F_OFF + 80, 0:64], y_v[b, 512:576, :])
        scatter(o, 0, 0)
        n = [o[64:72, 128 * a:128 * (a + 1)] for a in range(4)]
        s02, d02, s13, d13 = n[0] + n[2], n[0] - n[2], n[1] + n[3], n[1] - n[3]
        nil = jnp.zeros((8, 128), f32)
        for p0, (re, im) in enumerate(((s02 + s13, nil), (d02, -d13), (s02 - s13, nil), (d02, d13))):
            s_v[b, p0, 0, 288:296, :] = re
            s_v[b, p0, 1, 288:296, :] = im
        return results + [o]

    for b in range(4):
        with _scope('wait_x'):
            pltpu.make_async_copy(x_v.at[b], x_v.at[b], sem_in.at[8 + b]).wait()
        norm_radix9(b, Pace(channel_dft(b - 1) if b > 0 else [], 32))

    lane = lax.broadcasted_iota(jnp.int32, (8, 128), 1)
    lane_bit = [((lane >> t) & 1) == 1 for t in range(4)]

    def shuffle(v, token):
        v = [v[0]] + [pltpu.roll(v[a], a, 1) for a in range(15, 0, -1)]
        bits = list(lane_bit)
        if token is not None:
            bits[0] = (after(lane, pltpu.bitcast(token, jnp.int32)) & 1) == 1
        for t in range(4):
            v = [jnp.where(bits[t], v[(p - (1 << t)) % NB], v[p]) for p in range(NB)]
        return v

    def reorder_filter(pln, r, token):
        if r < 288:
            v = [pltpu.bitcast(w_v[pln, r:r + 16, 128 * a:128 * (a + 1)], jnp.int32)
                 for a in range(NB)]
            for p, w in enumerate(shuffle(v, token)):
                wp_v[pln, p, r:r + 16, :] = unpack(w).astype(f32)
        else:
            v = [jnp.broadcast_to(wn_v[pln, :, 128 * a:128 * (a + 1)].astype(f32), (8, 128))
                 for a in range(NB)]
            for p, w in enumerate(shuffle(v, token)):
                wp_v[pln, p, 288:296, :] = w

    gmat = lambda p, t: unpack(packed(g_tab)[p, t])

    span = lambda g: (72 * g, 80 if g == 3 else 72)

    def butterflies_in(g, p0, pace):
        r0, n = span(g)
        for r in range(r0, r0 + n, 8):
            token = pace()
            x = [(s_v[b, p0, 0, r:r + 8, :], s_v[b, p0, 1, r:r + 8, :]) for b in range(4)]
            for b in (range(2) if p0 == 0 else range(1, 4)):
                x[b] = (after(x[b][0], token), after(x[b][1], token))
            x = [_twiddle16(x[b], b * p0) for b in range(4)]
            for p1, (re, im) in enumerate(_radix4(x, False)):
                s_v[p1, p0, 0, r:r + 8, :] = re
                s_v[p1, p0, 1, r:r + 8, :] = im

    def token_filter(g, p0):
        r0, n = span(g)
        rows = slice(r0, r0 + n)
        spec, fwd, inv = [], [], []
        for p1 in range(4):
            p = p0 + 4 * p1
            a, b = s_v[p1, p0, 0, rows, :], s_v[p1, p0, 1, rows, :]
            k1 = _dot(a + b, gmat(p, 0), _NT)
            fwd.append(k1)
            spec.append((k1 - _dot(b, gmat(p, 2), _NT), k1 + _dot(a, gmat(p, 1), _NT)))
        for p1, (xr, xi) in enumerate(spec):
            p = p0 + 4 * p1
            wr, wi = wp_v[0, p, rows, :], wp_v[1, p, rows, :]
            zr, zi = xr * wr - xi * wi, xr * wi + xi * wr
            k1 = _dot(zr + zi, gmat(p, 0))
            inv.append(k1)
            s_v[p1, p0, 0, rows, :] = k1 + _dot(zi, gmat(p, 1))
            s_v[p1, p0, 1, rows, :] = k1 - _dot(zr, gmat(p, 2))
        return fwd, inv

    def butterflies_out(g, p0):
        r0, _ = span(g)
        for q in range(9 + (g == 3)):
            src = pl.ds(r0 + q, 8, stride=9) if q < 9 else pl.ds(288, 8)
            dst = 32 * q + 8 * g if q < 9 else 288
            x = [(s_v[p1, p0, 0, src, :], s_v[p1, p0, 1, src, :]) for p1 in range(4)]
            for b, z in enumerate(_radix4(x, True)):
                re, im = _twiddle16(z, -b * p0)
                z_v[b, p0, 0, dst:dst + 8, :] = re
                z_v[b, p0, 1, dst:dst + 8, :] = im

    def reorder_rows(lo, hi, results):
        jobs = [(pln, r) for r in range(lo, hi, 16) for pln in range(2)]
        pace = Pace(results, len(jobs))
        for pln, r in jobs:
            reorder_filter(pln, r, pace())

    units = [(g, p0) for g in range(4) for p0 in range(4)]
    filter_rows = {0: (80, 112), 1: (112, 144), 6: (144, 192), 7: (192, 224),
                   8: (224, 256), 9: (256, 288), 10: (288, 304)}
    with _scope('wait_w'):
        for cp in cp_w[0]:
            cp.wait()
    start_w1(1)
    start_w1(2)
    reorder_rows(0, 80, channel_dft(3))
    butterflies_in(*units[0], Pace([], 1))
    butterflies_in(*units[1], Pace([], 1))
    for i, unit in enumerate(units):
        if i == 6:
            with _scope('wait_w'):
                for cp in cp_w[1]:
                    cp.wait()
            start_w1(3)
            start_w1(4)
        if i > 0:
            butterflies_out(*units[i - 1])
        fwd, inv = token_filter(*unit)
        if i + 2 < len(units):
            butterflies_in(*units[i + 2], Pace(inv, 10))
        if i in filter_rows:
            reorder_rows(*filter_rows[i], WJOB(fwd, inv))
    butterflies_out(*units[-1])

    with _scope('wait_wm1'):
        cp_dm[1].wait()
        cp_wm[1].wait()
    modulation(1152, 2944)

    def channel_idft(b):
        def gather(r):
            t = _radix4([(z_v[b, p0, 0, r:r + 8, :], z_v[b, p0, 1, r:r + 8, :])
                         for p0 in range(4)], True)
            return [jnp.concatenate([t[a][pln] for a in range(4)], 1) for pln in range(2)]

        results = []
        for q in range(1, 5):
            rhs = jnp.concatenate(
                sum((gather(32 * k + 8 * g) for k in (q, 9 - q) for g in range(4)), []), 0)
            results.append(_dot(dm_v[_DI_OFF + 128 * (q - 1):_DI_OFF + 128 * q, :], rhs))
            y_v[b, 128 * (q - 1):128 * q, :] = results[-1]
        rhs = jnp.concatenate(sum((gather(8 * g) for g in range(4)), []) + gather(288)[:1], 0)
        results.append(_dot(dm_v[_D0I_OFF:_D0I_OFF + 64, 0:72], rhs))
        y_v[b, 512:576, :] = results[-1]
        return results

    def residual_norms(b, pace):
        norm = []
        for a in range(4):
            lanes = slice(128 * a, 128 * (a + 1))
            st = _Stats()
            for t in range(0, 64, 16):
                tiles = [load_x(b, a, 64 * j + t) for j in range(9)]
                for hf in range(2):
                    r = t + 8 * hf
                    p = {q: (y_v[b, 128 * (q - 1) + r:128 * (q - 1) + r + 8, lanes],
                             y_v[b, 128 * (q - 1) + 64 + r:128 * (q - 1) + 72 + r, lanes])
                         for q in range(1, 5)}
                    token = pace()
                    for q in (3, 4):
                        p[q] = (after(p[q][0], token), after(p[q][1], token))
                    y = _radix9_inv(y_v[b, 512 + r:520 + r, lanes], p)
                    for j in range(9):
                        row = 64 * j + r
                        x1 = tiles[j][hf] + mod_tile(2, row) * y[j]
                        st.add(x1)
                        x1_v[a, b, row:row + 8, :] = x1
            rs, sh = st.scale_shift()
            st = _Stats()
            for row in range(0, D, 8):
                if row % 120 == 0:
                    scale = after(rs, pace())
                t = (x1_v[a, b, row:row + 8, :] * scale + sh) * mod_tile(4, row) + mod_tile(3, row)
                st.add(t)
                t_v[a, row:row + 8, :] = t
            rs, sh = st.scale_shift()
            norm.append((rs, jnp.concatenate([sh, sh], 0)))
        for row in range(0, QD, 16):
            h = {}
            for k in range(4):
                if k < 3:
                    token = pace()
                scale = after(norm[k][0], token)
                scale = jnp.concatenate([scale, scale], 0)
                for r in range(4):
                    rows = slice(QD * r + row, QD * r + row + 16)
                    h[r, k] = t_v[k, rows, :] * scale + norm[k][1]
                    h_v[b, k, rows, :] = h[r, k].astype(bf16)
            for i in range(7):
                quad = [_combine(_LHS[i], lambda o: h[_block(o, c)]) for c in range(4)]
                for j in range(7):
                    hs_v[i, j, b, row:row + 16, :] = _combine(
                        _LHS[j], lambda c: quad[c]).astype(bf16)

    def first_chunk(b):
        lhs = jnp.concatenate([unpack(packed(h_v)[b, a]) for a in range(4)], 1)
        rhs = jnp.concatenate([jnp.concatenate(
            [unpack(packed(w1_v)[n, pl.ds(pl.multiple_of(64 * (4 * a + b), 64), 64), :])
             for a in range(4)], 0) for n in range(4)], 1)
        return _dot(lhs, rhs)

    steps = 4 * (8 + 5) + 27
    channel_idft(0)
    residual_norms(0, Pace(sum((channel_idft(b) for b in range(1, 4)), []), steps))
    with _scope('wait_w10'):
        pltpu.make_async_copy(w1_v.at[0:4], w1_v.at[0:4], sem_in.at[23]).wait()

    def overlap(b, carry):
        part = first_chunk(b)
        u_v[...] += part
        residual_norms(b + 1, Pace([part[:, 128 * n:128 * (n + 1)] for n in range(4)], steps))
        return carry

    with _scope('phase3'):
        lax.fori_loop(0, 3, overlap, None)

    with _scope('wait_b'):
        for cp in cp_b + [cp_wm[2]]:
            cp.wait()
    modulation(2944, 6 * D)
    for src, dst in ((b1_v, bias1_v), (b2_v, bias2_v)):
        bv = src[...].astype(f32)
        for t in range(src.shape[0]):
            dst[t] = jnp.broadcast_to(bv[t:t + 1, :], (8, 128))

    def activate(j):
        g, made = {}, set()

        def emit(r, n, u):
            g[r, n] = _gelu(u + bias1_v[4 * j + n, 0:1, :])
            for i in range(7):
                for k in range(7):
                    need = [_block(o, c) for o, _ in _LHS[i] for c, _ in _LHS[k]]
                    if (i, k) not in made and all(e in g for e in need):
                        made.add((i, k))
                        act_v[i, k, j] = _combine(_LHS[k], lambda c: _combine(
                            _LHS[i], lambda o: g[_block(o, c)])).astype(bf16)
        return emit

    u0 = u_v[...] + first_chunk(3)
    emit0 = activate(0)
    for r in range(4):
        for n in range(4):
            emit0(r, n, u0[QD * r:QD * (r + 1), 128 * n:128 * (n + 1)])

    def mlp1(j, carry):
        with _scope('wait_w1'):
            pltpu.make_async_copy(w1_v.at[0:4], w1_v.at[0:4], sem_w1.at[j]).wait()
        pl.when(j + 4 < n1)(lambda: start_w1(j + 4))
        start_w2(j - 1)

        def raw(k, n, t, keep_packed):
            if keep_packed:
                return unpack(packed(w1_v)[4 * j + n, 256 * k + 64 * t:256 * k + 64 * (t + 1), :])
            return w1_v[4 * j + n, 512 * k + 128 * t:512 * k + 128 * (t + 1), :]

        lhs = lambda i, k: jnp.concatenate([unpack(packed(hs_v)[i, k, t]) for t in range(4)], 1)
        _strassen2(lhs, raw, 4, stage_v, activate(j))
        return carry

    with _scope('mlp1'):
        lax.fori_loop(1, n1, mlp1, None)

    def mlp2(j, carry):
        with _scope('wait_w2'):
            pltpu.make_async_copy(w2_v.at[0:4], w2_v.at[0:4], sem_w2.at[j]).wait()

        def raw(k, n, t, keep_packed):
            if keep_packed:
                return unpack(packed(w2_v)[4 * j + n, 64 * (4 * t + k):64 * (4 * t + k + 1), :])
            return w2_v[4 * j + n, 128 * (4 * t + k):128 * (4 * t + k + 1), :]

        def emit(r, n, y):
            rows = slice(QD * r, QD * (r + 1))
            y = y + bias2_v[4 * j + n, 0:1, :]
            o_v[j, n, rows, :] = (x1_v[j, n, rows, :] + mod_tile(5, QD * r, QD) * y).astype(bf16)
            pltpu.make_async_copy(o_v.at[j, n, rows, :], o_hbm.at[rows, column(4 * j + n)],
                                  sem_out.at[0]).start()

        lhs = lambda i, k: jnp.concatenate([unpack(packed(act_v)[i, k, t]) for t in range(n1)], 1)
        _strassen2(lhs, raw, n1, stage_v, emit)
        return carry

    with _scope('mlp2'):
        lax.fori_loop(0, n2, mlp2, None)
    with _scope('wait_out'):
        pltpu.make_async_copy(o_v, o_v, sem_out.at[0]).wait()


@jax.jit
def pallas_adaLN_cond__spectral_gfnet__mixer_token_mlp__prompt_kernel(
    A_x, A_w_r, A_w_i, B_x, B_w1, B_b1, B_w2, B_b2, c, w_mod,
):
    del B_x
    assert A_x.shape == (1, S, D)
    dmat, smat = _tables()
    n1, n2 = F // 512, S // 512
    vmem = pltpu.VMEM
    out_t = pl.pallas_call(
        _kernel,
        in_specs=[pl.BlockSpec(memory_space=pltpu.HBM)] * 11,
        out_specs=pl.BlockSpec(memory_space=pltpu.HBM),
        out_shape=jax.ShapeDtypeStruct((D, S), bf16),
        scratch_shapes=[
            vmem((4, 4, D, 128), bf16),
            vmem((2, 288, S), bf16),
            vmem((D, 6 * D), bf16),
            vmem((_SROWS, 128), f32),
            vmem((6 * D, 128), f32),
            vmem((NB, 3, 128, 128), bf16),
            vmem((4, D, 512), f32),
            vmem((4, 4, 2, KR, 128), f32),
            vmem((1, 4, 4, 2, KR, 128), f32),
            vmem((1, 2, NB, KR, 128), f32),
            vmem((4, 4, D, 128), f32),
            vmem((4, D, 128), f32),
            vmem((D, 512), f32),
            vmem((4, 4, D, 128), bf16),
            vmem((7, 7, 4, QD, 128), bf16),
            vmem((F // 128, S, 128), bf16),
            vmem((S // 128, F, 128), bf16),
            vmem((SLOTS, 4, F // 4, 128), f32),
            vmem((F // 128, 8, 128), f32),
            vmem((S // 128, 8, 128), f32),
            vmem((4, 4, D, 128), bf16),
            vmem((7, 7, n1, QD, 128), bf16),
            vmem((_DROWS, 128), bf16),
            vmem((2, 1, S), bf16),
            vmem((8, 1, D), bf16),
            vmem((2, F // 128, 128), bf16),
            vmem((S // 128, 128), bf16),
            pltpu.SMEM((1,), jnp.int32),
            pltpu.SemaphoreType.DMA((24,)),
            pltpu.SemaphoreType.DMA((n1,)),
            pltpu.SemaphoreType.DMA((n2,)),
            pltpu.SemaphoreType.DMA((1,)),
        ],
        compiler_params=pltpu.CompilerParams(vmem_limit_bytes=124 * 1024 * 1024),
    )(
        A_x.reshape(S, D).T, A_w_r.T, A_w_i.T, B_w1, B_b1.reshape(F // 128, 128),
        B_w2, B_b2.reshape(S // 128, 128), c, w_mod,
        jnp.asarray(dmat, dtype=bf16), jnp.asarray(smat),
    )
    return out_t.T.reshape(1, S, D)
```

```python
import functools
import math

import jax
import jax.numpy as jnp
import numpy as np
from jax import lax
import jax.experimental.pallas as pl
import jax.experimental.pallas.tpu as pltpu

S, D, F = 2048, 576, 4608
DF = D // 2 + 1
KR = 296
NB = S // 128
QD = D // 4
SLOTS = 3
WJOB = lambda fwd, inv: inv
EPS = 1e-5
PROFILE = False
import contextlib
def _scope(n):
    return jax.named_scope(n) if PROFILE else contextlib.nullcontext()

f32 = jnp.float32
bf16 = jnp.bfloat16
_NN = (((1,), (0,)), ((), ()))
_NT = (((1,), (1,)), ((), ()))


def _dot(a, b, dims=_NN):
    return lax.dot_general(a, b, dims, preferred_element_type=f32)


@functools.lru_cache(maxsize=None)
def _tables():
    r = np.arange(64)
    kk = np.arange(32)
    th = lambda k: 2 * np.pi * np.outer(k, r) / D

    def weave(re, im):
        n = re.shape[1]
        return np.stack([re.reshape(4, 8, n), im.reshape(4, 8, n)], 1).reshape(64, n)

    fwd = []
    for q in range(1, 5):
        a, b = th(q + 9 * kk), th(9 - q + 9 * kk)
        fwd.append(np.concatenate([
            weave(np.block([np.cos(a), np.sin(a)]), np.block([-np.sin(a), np.cos(a)])),
            weave(np.block([np.cos(b), -np.sin(b)]), np.block([-np.sin(b), -np.cos(b)]))], 0))
    l0 = np.concatenate(
        [weave(np.cos(th(9 * kk)), -np.sin(th(9 * kk))), np.cos(th(np.array([D // 2])))], 0)
    cw = np.full((65, 1), 2.0)
    cw[0] = cw[64] = 1.0
    l0f = np.zeros((80, 128))
    l0f[:65, :64] = l0
    l0i = np.zeros((64, 128))
    l0i[:, :65] = (l0 * cw).T
    dmat = np.concatenate(fwd + [l0f] + [2 * m.T for m in fwd] + [l0i], 0)

    n2 = np.arange(128)
    a16 = np.arange(16)
    tw = lambda m: np.exp(-2j * np.pi * np.outer(m, n2) / S)
    r1, r2 = tw(127 * a16), tw(127 * a16 + 128)
    parts = np.concatenate([tw(np.arange(8)), tw(8 * a16), r2, r1, r1], 0)
    smat = np.concatenate([parts.real, parts.imag], 0)
    return dmat.astype(np.float32), smat.astype(np.float32)


_DF_OFF = 0
_D0F_OFF = 512
_DI_OFF = 592
_D0I_OFF = 1104
_DROWS = 1168
_SROWS = 144

_S3 = math.sqrt(3.0) / 2
_C1, _S1 = math.cos(2 * math.pi / 9), math.sin(2 * math.pi / 9)
_C2, _S2 = math.cos(4 * math.pi / 9), math.sin(4 * math.pi / 9)


def _radix9_fwd(a):
    b0, br, bd = [], [], []
    for j in range(3):
        t = a[3 + j] + a[6 + j]
        b0.append(a[j] + t)
        br.append(a[j] - 0.5 * t)
        bd.append(a[3 + j] - a[6 + j])
    t = b0[1] + b0[2]
    y0 = b0[0] + t
    y3 = (b0[0] - 0.5 * t, _S3 * (b0[2] - b0[1]))
    c0r, c0i = br[0], -_S3 * bd[0]
    c1r = _C1 * br[1] - (_S3 * _S1) * bd[1]
    c1i = -_S1 * br[1] - (_S3 * _C1) * bd[1]
    c2r = _C2 * br[2] - (_S3 * _S2) * bd[2]
    c2i = -_S2 * br[2] - (_S3 * _C2) * bd[2]
    tr, ti = c1r + c2r, c1i + c2i
    y1 = (c0r + tr, c0i + ti)
    ur, ui = c0r - 0.5 * tr, c0i - 0.5 * ti
    nvr, vi = _S3 * (c2r - c1r), _S3 * (c1i - c2i)
    y4 = (ur + vi, ui + nvr)
    y2 = (ur - vi, nvr - ui)
    return y0, {1: y1, 2: y2, 3: y3, 4: y4}


def _radix9_inv(p0, p):
    (p1r, p1i), (p2r, p2i), (p3r, p3i), (p4r, p4i) = p[1], p[2], p[3], p[4]
    ur, ui = p4r + p2r, p4i - p2i
    vi, nvr = _S3 * (p4r - p2r), _S3 * (p4i + p2i)
    c0r, c0i = p1r + ur, p1i + ui
    tr, ti = p1r - 0.5 * ur, p1i - 0.5 * ui
    c1r, c1i, c2r, c2i = tr - nvr, ti + vi, tr + nvr, ti - vi
    br = [c0r, _C1 * c1r - _S1 * c1i, _C2 * c2r - _S2 * c2i]
    nbd = [_S3 * c0i,
           (_S3 * _S1) * c1r + (_S3 * _C1) * c1i,
           (_S3 * _S2) * c2r + (_S3 * _C2) * c2i]
    ny3 = _S3 * p3i
    t = p0 - 0.5 * p3r
    b0 = [p0 + p3r, t - ny3, t + ny3]
    y = [None] * 9
    for j in range(3):
        t = b0[j] - 0.5 * br[j]
        y[j] = b0[j] + br[j]
        y[3 + j] = t - nbd[j]
        y[6 + j] = t + nbd[j]
    return y


def _radix4(x, inverse):
    (ar, ai), (br, bi), (cr, ci), (dr, di) = x
    sr, si, er, ei = ar + cr, ai + ci, ar - cr, ai - ci
    tr, ti, fr, fi = br + dr, bi + di, br - dr, bi - di
    y1, y3 = (er + fi, ei - fr), (er - fi, ei + fr)
    if inverse:
        y1, y3 = y3, y1
    return [(sr + tr, si + ti), y1, (sr - tr, si - ti), y3]


def _twiddle16(z, e):
    e %= 16
    re, im = z
    if e == 0:
        return z
    if e == 4:
        return (im, -re)
    if e == 12:
        return (-im, re)
    c, s = math.cos(math.pi * e / 8), math.sin(math.pi * e / 8)
    if e % 4 == 2:
        if (c > 0) == (s > 0):
            return (c * (re + im), c * (im - re))
        return (c * (re - im), c * (im + re))
    return (c * re + s * im, c * im - s * re)


class _Stats:
    def __init__(self):
        self.s = [None, None]
        self.q = [None, None]
        self.n = 0

    def add(self, v):
        i = self.n % 2
        self.n += 1
        self.s[i] = v if self.s[i] is None else self.s[i] + v
        self.q[i] = v * v if self.q[i] is None else self.q[i] + v * v

    def scale_shift(self):
        mean = jnp.sum(self.s[0] + self.s[1], axis=0, keepdims=True) * (1.0 / D)
        msq = jnp.sum(self.q[0] + self.q[1], axis=0, keepdims=True) * (1.0 / D)
        r = lax.rsqrt(jnp.maximum(msq - mean * mean, 0.0) + EPS)
        return (jnp.broadcast_to(r, (8, 128)), jnp.broadcast_to(-mean * r, (8, 128)))


_LHS = (((0, 1), (3, 1)), ((2, 1), (3, 1)), ((0, 1),), ((3, 1),), ((0, 1), (1, 1)),
        ((2, 1), (0, -1)), ((1, 1), (3, -1)))
_RHS = (((0, 1), (3, 1)), ((0, 1),), ((1, 1), (3, -1)), ((2, 1), (0, -1)), ((3, 1),),
        ((0, 1), (1, 1)), ((2, 1), (3, 1)))
_OUT = (((0, 1), (3, 1), (4, -1), (6, 1)), ((2, 1), (4, 1)), ((1, 1), (3, 1)),
        ((0, 1), (1, -1), (2, 1), (5, 1)))
_ORDER = ((1, 0, 2, 4, 3, 6, 5), (1, 4, 3, 2, 0, 6, 5), (4, 1, 3, 2, 0, 5, 6))


def _combine(terms, get):
    acc = get(terms[0][0])
    for q, sign in terms[1:]:
        acc = acc + get(q) if sign > 0 else acc - get(q)
    return acc


def _block(outer, inner):
    return 2 * (outer // 2) + inner // 2, 2 * (outer % 2) + inner % 2


class _Quadrants:
    def __init__(self):
        self.acc = [None] * 4
        self.left = [len(t) for t in _OUT]

    def add(self, i, m):
        done = []
        for c, terms in enumerate(_OUT):
            for q, sign in terms:
                if q != i:
                    continue
                prev = self.acc[c]
                if prev is None:
                    self.acc[c] = (m, sign)
                elif prev[1] == sign:
                    self.acc[c] = (prev[0] + m, sign)
                else:
                    self.acc[c] = (m - prev[0] if sign > 0 else prev[0] - m, 1)
                self.left[c] -= 1
                if self.left[c] == 0:
                    assert self.acc[c][1] > 0
                    done.append((c, self.acc[c][0]))
        return done


def _strassen2(lhs, raw, tiles, stage, emit, order):
    def prepare(n):
        i = order[0][n]
        if len(_RHS[i]) > 1:
            for c in range(4):
                for t in range(tiles):
                    stage[n % SLOTS, c, 128 * t:128 * (t + 1), :] = _combine(
                        _RHS[i], lambda q: raw(*_block(q, c), t, False).astype(f32))

    outer = [_Quadrants() for _ in range(4)]
    for n, i in enumerate(order[0]):
        if n + 1 < 7:
            prepare(n + 1)
        inner = _Quadrants()
        for j in order[1 if n < 6 else 2]:
            if len(_RHS[i]) > 1:
                rhs = _combine(_RHS[j], lambda c: stage[n % SLOTS, c, 0:128 * tiles, :])
            elif len(_RHS[j]) > 1:
                rhs = _combine(_RHS[j], lambda c: jnp.concatenate(
                    [raw(*_block(_RHS[i][0][0], c), t, False).astype(f32)
                     for t in range(tiles)], 0))
            else:
                rhs = jnp.concatenate(
                    [raw(*_block(_RHS[i][0][0], _RHS[j][0][0]), t, True)
                     for t in range(tiles)], 0)
            for c, v in inner.add(j, _dot(lhs(i, j), rhs.astype(bf16))):
                for o, w in outer[c].add(i, v):
                    emit(*_block(o, c), w)


def _gelu2(u):
    k0 = math.sqrt(2.0 / math.pi)
    th = jnp.tanh(u * (k0 + (k0 * 0.044715) * (u * u)))
    return u + u * th


def _kernel(x_hbm, wr_hbm, wi_hbm, w1_hbm, b1_hbm, w2_hbm, b2_hbm, c_hbm, wm_hbm,
            dm_hbm, sm_hbm, o_hbm,
            x_v, w_v, wm_v, e_v, mod_v, g_tab, y_v, s_v, z_v, wp_v, x1_v, t_v, u_v, h_v, hs_v, w1_v, w2_v, stage_v, bias1_v, bias2_v, o_v, act_v, dm_v, sm_v, wn_v, c_v, b1_v, b2_v, zero_s, sem_in, sem_w1, sem_w2, sem_out):
    n1, n2 = F // 512, S // 512
    c_v, b1_v = c_v.at[0], b1_v.at[0]
    packed = lambda ref: ref.bitcast(jnp.int32)
    unpack = lambda v: pltpu.bitcast(v, bf16)

    zero_s[0] = 0
    zero = zero_s[0]
    z_v, wp_v = z_v.at[zero], wp_v.at[zero]

    def copy_in(i, src, dst):
        return pltpu.make_async_copy(src, dst, sem_in.at[zero + i])

    def wm_copy(i, lo, hi):
        return copy_in(i, wm_hbm.at[:, lo:hi], wm_v.at[:, lo:hi])

    cp_sm = copy_in(0, sm_hbm, sm_v)
    cp_c = copy_in(1, c_hbm, c_v)
    cp_wm = [wm_copy(2, 0, 1152), wm_copy(3, 1152, 2944), wm_copy(4, 2944, 6 * D)]
    cp_dm = [copy_in(5, dm_hbm.at[0:_DI_OFF], dm_v.at[0:_DI_OFF]),
             copy_in(22, dm_hbm.at[_DI_OFF:_DROWS], dm_v.at[_DI_OFF:_DROWS])]
    cp_b = [copy_in(6, b1_hbm, b1_v), copy_in(7, b2_hbm, b2_v)]
    cp_x = [copy_in(8 + b, x_hbm.at[:, 128 * (4 * a + b):128 * (4 * a + b + 1)], x_v.at[b, a])
            for b in range(4) for a in range(4)]
    w_rows = (0, 80, 144, 288)
    cp_w = [[copy_in(12 + 2 * g + pln, src.at[w_rows[g]:w_rows[g + 1], :],
                     w_v.at[pln, w_rows[g]:w_rows[g + 1], :])
             for pln, src in enumerate((wr_hbm, wi_hbm))] for g in range(3)]
    cp_w[2] += [copy_in(20 + pln, src.at[288:DF, :], wn_v.at[pln])
                for pln, src in enumerate((wr_hbm, wi_hbm))]
    cp_w10 = [copy_in(23, w1_hbm.at[:, 128 * n:128 * (n + 1)], w1_v.at[n]) for n in range(4)]

    for cp in ([cp_sm, cp_c, cp_wm[0], cp_dm[0]] + cp_x + cp_w[0] + cp_w[1] + cp_w[2] + [cp_dm[1]]
               + [cp_wm[1]] + cp_w10 + cp_b + [cp_wm[2]]):
        cp.start()

    def column(n):
        return pl.ds(n * 128 if isinstance(n, int) else pl.multiple_of(n * 128, 128), 128)

    def start_w1(j):
        for n in range(4):
            pltpu.make_async_copy(
                w1_hbm.at[:, column(4 * j + n)], w1_v.at[4 * j + n], sem_w1.at[j]).start()

    def start_w2(j):
        for n in range(2):
            pltpu.make_async_copy(
                w2_hbm.at[:, column(2 * j + n)], w2_v.at[2 * j + n], sem_w2.at[j // 2]).start()

    @pl.loop(0, D // 8)
    def _(i):
        u_v[pl.ds(pl.multiple_of(8 * i, 8), 8), :] = jnp.zeros((8, 512), f32)

    with _scope('wait_sm'):
        cp_sm.wait()

    half = _SROWS // 2
    for i in range(NB):
        ar, ai = sm_v[0:8, :], sm_v[half:half + 8, :]
        br, bi = sm_v[8 + i:9 + i, :], sm_v[half + 8 + i:half + 9 + i, :]
        e_v[0, 8 * i:8 * i + 8, :] = ar * br - ai * bi
        e_v[1, 8 * i:8 * i + 8, :] = ar * bi + ai * br

    @pl.loop(0, NB)
    def _(p):
        for i in range(8):
            off = (24 if i == 0 else 40) + 16 - p
            hr, hi = sm_v[pl.ds(off, 16), :], sm_v[pl.ds(off + half, 16), :]
            er, ei = e_v[0, 16 * i:16 * i + 16, :], e_v[1, 16 * i:16 * i + 16, :]
            cr = er * hr - ei * hi
            ci = er * hi + ei * hr
            for t, m in enumerate((cr, ci - cr, cr + ci)):
                g_tab[p, t, 16 * i:16 * i + 16, :] = m.astype(bf16)

    never = sm_v[0:8, :] > 2.0

    def after(v, token):
        return v if token is None else jnp.where(never, token, v)

    class Pace:
        def __init__(self, results, n):
            self.tiles = [(o, r) for o in results for r in range(0, o.shape[0], 8)]
            self.n, self.i = n, 0

        def __call__(self):
            if not self.tiles:
                return None
            o, r = self.tiles[min(self.i, self.n - 1) * len(self.tiles) // self.n]
            self.i += 1
            return o[r:r + 8, 0:128]

    def modulation(lo, hi):
        cv = c_v[...].astype(f32)
        sc = jnp.broadcast_to(cv * jax.nn.sigmoid(cv), (8, D))
        m = _dot(sc, wm_v[:, lo:hi])
        col = lo + lax.broadcasted_iota(jnp.int32, m.shape, 1)
        which = lambda i: (col >= i * D) & (col < (i + 1) * D)
        m = jnp.where(which(1) | which(4), 1.0 + m, m)
        m = jnp.where(which(2), m * (1.0 / (S * D)), m)
        m = jnp.where(which(5), 0.5 * m, m)
        for t in range((hi - lo) // 128):
            row = jnp.broadcast_to(m[0:1, 128 * t:128 * (t + 1)], (128, 128))
            mod_v[lo + 128 * t:lo + 128 * (t + 1), :] = row.T

    def mod_tile(i, row, n=8):
        return mod_v[i * D + row:i * D + row + n, :]

    with _scope('wait_wm0'):
        cp_c.wait()
        cp_wm[0].wait()
    modulation(0, 1152)

    def load_x(b, a, r):
        v = x_v[b, a, r:r + 16, :].astype(f32)
        return v[:8], v[8:]

    def norm_radix9(b, pace):
        for a in range(4):
            lanes = slice(128 * a, 128 * (a + 1))
            st = _Stats()
            for r in range(0, D, 16):
                for hf, v in enumerate(load_x(b, a, r)):
                    st.add(v)
                    x1_v[a, b, r + 8 * hf:r + 8 * hf + 8, :] = v
            rs, sh = st.scale_shift()
            for t in range(0, 64, 16):
                for hf in range(2):
                    r = t + 8 * hf
                    scale = after(rs, pace())
                    h = [(x1_v[a, b, 64 * j + r:64 * j + r + 8, :] * scale + sh) * mod_tile(1, 64 * j + r)
                         + mod_tile(0, 64 * j + r) for j in range(9)]
                    y0, y = _radix9_fwd(h)
                    y_v[b, 512 + r:520 + r, lanes] = y0
                    for q in range(1, 5):
                        y_v[b, 128 * (q - 1) + r:128 * (q - 1) + r + 8, lanes] = y[q][0]
                        y_v[b, 128 * (q - 1) + 64 + r:128 * (q - 1) + 72 + r, lanes] = y[q][1]

    def channel_dft(b):
        def scatter(o, base, k0):
            for g in range(4):
                r = base + 16 * g
                t = _radix4([(o[r:r + 8, 128 * a:128 * (a + 1)],
                              o[r + 8:r + 16, 128 * a:128 * (a + 1)]) for a in range(4)], False)
                rows = pl.ds(72 * g + k0, 8, stride=9)
                for p0 in range(4):
                    s_v[b, p0, 0, rows, :] = t[p0][0]
                    s_v[b, p0, 1, rows, :] = t[p0][1]

        results = []
        for q in range(1, 5):
            o = _dot(dm_v[_DF_OFF + 128 * (q - 1):_DF_OFF + 128 * q, :],
                     y_v[b, 128 * (q - 1):128 * q, :])
            results.append(o)
            scatter(o, 0, q)
            scatter(o, 64, 9 - q)
        o = _dot(dm_v[_D0F_OFF:_D0F_OFF + 80, 0:64], y_v[b, 512:576, :])
        scatter(o, 0, 0)
        n = [o[64:72, 128 * a:128 * (a + 1)] for a in range(4)]
        s02, d02, s13, d13 = n[0] + n[2], n[0] - n[2], n[1] + n[3], n[1] - n[3]
        nil = jnp.zeros((8, 128), f32)
        for p0, (re, im) in enumerate(((s02 + s13, nil), (d02, -d13), (s02 - s13, nil), (d02, d13))):
            s_v[b, p0, 0, 288:296, :] = re
            s_v[b, p0, 1, 288:296, :] = im
        return results + [o]

    for b in range(4):
        with _scope('wait_x'):
            pltpu.make_async_copy(x_v.at[b], x_v.at[b], sem_in.at[8 + b]).wait()
            if b == 0:
                cp_dm[0].wait()
        norm_radix9(b, Pace(channel_dft(b - 1) if b > 0 else [], 32))

    lane = lax.broadcasted_iota(jnp.int32, (8, 128), 1)
    lane_bit = [((lane >> t) & 1) == 1 for t in range(4)]

    def shuffle(v, token):
        v = [v[0]] + [pltpu.roll(v[a], a, 1) for a in range(15, 0, -1)]
        bits = list(lane_bit)
        if token is not None:
            bits[0] = (after(lane, pltpu.bitcast(token, jnp.int32)) & 1) == 1
        for t in range(4):
            v = [jnp.where(bits[t], v[(p - (1 << t)) % NB], v[p]) for p in range(NB)]
        return v

    def reorder_filter(pln, r, token):
        if r < 288:
            v = [pltpu.bitcast(w_v[pln, r:r + 16, 128 * a:128 * (a + 1)], jnp.int32)
                 for a in range(NB)]
            for p, w in enumerate(shuffle(v, token)):
                wp_v[pln, p, r:r + 16, :] = unpack(w).astype(f32)
        else:
            v = [jnp.broadcast_to(wn_v[pln, :, 128 * a:128 * (a + 1)].astype(f32), (8, 128))
                 for a in range(NB)]
            for p, w in enumerate(shuffle(v, token)):
                wp_v[pln, p, 288:296, :] = w

    gmat = lambda p, t: unpack(packed(g_tab)[p, t])

    span = lambda g: (72 * g, 80 if g == 3 else 72)

    def butterflies_in(g, p0, pace):
        r0, n = span(g)
        for r in range(r0, r0 + n, 8):
            token = pace()
            x = [(s_v[b, p0, 0, r:r + 8, :], s_v[b, p0, 1, r:r + 8, :]) for b in range(4)]
            for b in (range(2) if p0 == 0 else range(1, 4)):
                x[b] = (after(x[b][0], token), after(x[b][1], token))
            x = [_twiddle16(x[b], b * p0) for b in range(4)]
            for p1, (re, im) in enumerate(_radix4(x, False)):
                s_v[p1, p0, 0, r:r + 8, :] = re
                s_v[p1, p0, 1, r:r + 8, :] = im

    def token_filter(g, p0):
        r0, n = span(g)
        rows = slice(r0, r0 + n)
        spec, fwd, inv = [], [], []
        for p1 in range(4):
            p = p0 + 4 * p1
            a, b = s_v[p1, p0, 0, rows, :], s_v[p1, p0, 1, rows, :]
            k1 = _dot(a + b, gmat(p, 0), _NT)
            fwd.append(k1)
            spec.append((k1 - _dot(b, gmat(p, 2), _NT), k1 + _dot(a, gmat(p, 1), _NT)))
        for p1, (xr, xi) in enumerate(spec):
            p = p0 + 4 * p1
            wr, wi = wp_v[0, p, rows, :], wp_v[1, p, rows, :]
            zr, zi = xr * wr - xi * wi, xr * wi + xi * wr
            k1 = _dot(zr + zi, gmat(p, 0))
            inv.append(k1)
            s_v[p1, p0, 0, rows, :] = k1 + _dot(zi, gmat(p, 1))
            s_v[p1, p0, 1, rows, :] = k1 - _dot(zr, gmat(p, 2))
        return fwd, inv

    def butterflies_out(g, p0):
        r0, _ = span(g)
        for q in range(9 + (g == 3)):
            src = pl.ds(r0 + q, 8, stride=9) if q < 9 else pl.ds(288, 8)
            dst = 32 * q + 8 * g if q < 9 else 288
            x = [(s_v[p1, p0, 0, src, :], s_v[p1, p0, 1, src, :]) for p1 in range(4)]
            for b, z in enumerate(_radix4(x, True)):
                re, im = _twiddle16(z, -b * p0)
                z_v[b, p0, 0, dst:dst + 8, :] = re
                z_v[b, p0, 1, dst:dst + 8, :] = im

    def reorder_rows(lo, hi, results):
        jobs = [(pln, r) for r in range(lo, hi, 16) for pln in range(2)]
        pace = Pace(results, len(jobs))
        for pln, r in jobs:
            reorder_filter(pln, r, pace())

    units = [(g, p0) for g in range(4) for p0 in range(4)]
    filter_rows = {0: (80, 112), 1: (112, 144), 6: (144, 192), 7: (192, 224),
                   8: (224, 256), 9: (256, 288), 10: (288, 304)}
    with _scope('wait_w'):
        for cp in cp_w[0]:
            cp.wait()
    start_w1(1)
    start_w1(2)
    reorder_rows(0, 80, channel_dft(3))
    butterflies_in(*units[0], Pace([], 1))
    butterflies_in(*units[1], Pace([], 1))
    for cp in cp_w[1]:
        cp.wait()
    for i, unit in enumerate(units):
        if i == 6:
            with _scope('wait_w'):
                for cp in cp_w[2]:
                    cp.wait()
            start_w1(3)
            start_w1(4)
        if i > 0:
            butterflies_out(*units[i - 1])
        fwd, inv = token_filter(*unit)
        if i + 2 < len(units):
            butterflies_in(*units[i + 2], Pace(inv, 10))
        if i in filter_rows:
            reorder_rows(*filter_rows[i], WJOB(fwd, inv))
    butterflies_out(*units[-1])

    with _scope('wait_wm1'):
        cp_dm[1].wait()
        cp_wm[1].wait()
    modulation(1152, 2944)

    def channel_idft(b):
        def gather(r):
            t = _radix4([(z_v[b, p0, 0, r:r + 8, :], z_v[b, p0, 1, r:r + 8, :])
                         for p0 in range(4)], True)
            return [jnp.concatenate([t[a][pln] for a in range(4)], 1) for pln in range(2)]

        results = []
        for q in range(1, 5):
            rhs = jnp.concatenate(
                sum((gather(32 * k + 8 * g) for k in (q, 9 - q) for g in range(4)), []), 0)
            results.append(_dot(dm_v[_DI_OFF + 128 * (q - 1):_DI_OFF + 128 * q, :], rhs))
            y_v[b, 128 * (q - 1):128 * q, :] = results[-1]
        rhs = jnp.concatenate(sum((gather(8 * g) for g in range(4)), []) + gather(288)[:1], 0)
        results.append(_dot(dm_v[_D0I_OFF:_D0I_OFF + 64, 0:72], rhs))
        y_v[b, 512:576, :] = results[-1]
        return results

    def residual_norms(b, pace):
        norm = []
        for a in range(4):
            lanes = slice(128 * a, 128 * (a + 1))
            st = _Stats()
            for t in range(0, 64, 16):
                for hf in range(2):
                    r = t + 8 * hf
                    p = {q: (y_v[b, 128 * (q - 1) + r:128 * (q - 1) + r + 8, lanes],
                             y_v[b, 128 * (q - 1) + 64 + r:128 * (q - 1) + 72 + r, lanes])
                         for q in range(1, 5)}
                    token = pace()
                    for q in (3, 4):
                        p[q] = (after(p[q][0], token), after(p[q][1], token))
                    y = _radix9_inv(y_v[b, 512 + r:520 + r, lanes], p)
                    for j in range(9):
                        row = 64 * j + r
                        x1 = x1_v[a, b, row:row + 8, :] + mod_tile(2, row) * y[j]
                        st.add(x1)
                        x1_v[a, b, row:row + 8, :] = x1
            rs, sh = st.scale_shift()
            st = _Stats()
            for row in range(0, D, 8):
                if row % 120 == 0:
                    scale = after(rs, pace())
                t = (x1_v[a, b, row:row + 8, :] * scale + sh) * mod_tile(4, row) + mod_tile(3, row)
                st.add(t)
                t_v[a, row:row + 8, :] = t
            rs, sh = st.scale_shift()
            norm.append((rs, jnp.concatenate([sh, sh], 0)))
        for row in range(0, QD, 16):
            h = {}
            for k in range(4):
                if k < 3:
                    token = pace()
                scale = after(norm[k][0], token)
                scale = jnp.concatenate([scale, scale], 0)
                for r in range(4):
                    rows = slice(QD * r + row, QD * r + row + 16)
                    h[r, k] = t_v[k, rows, :] * scale + norm[k][1]
                    h_v[b, k, rows, :] = h[r, k].astype(bf16)
            for i in range(7):
                quad = [_combine(_LHS[i], lambda o: h[_block(o, c)]) for c in range(4)]
                for j in range(7):
                    hs_v[i, j, b, row:row + 16, :] = _combine(
                        _LHS[j], lambda c: quad[c]).astype(bf16)

    def first_chunk(b):
        lhs = jnp.concatenate([unpack(packed(h_v)[b, a]) for a in range(4)], 1)
        rhs = jnp.concatenate([jnp.concatenate(
            [unpack(packed(w1_v)[n, pl.ds(pl.multiple_of(64 * (4 * a + b), 64), 64), :])
             for a in range(4)], 0) for n in range(4)], 1)
        return _dot(lhs, rhs)

    steps = 4 * (8 + 5) + 27
    channel_idft(0)
    residual_norms(0, Pace(sum((channel_idft(b) for b in range(1, 4)), []), steps))
    with _scope('wait_w10'):
        pltpu.make_async_copy(w1_v.at[0:4], w1_v.at[0:4], sem_in.at[23]).wait()

    def overlap(b, carry):
        start_w1(5 + b)
        part = first_chunk(b)
        u_v[...] += part
        residual_norms(b + 1, Pace([part[:, 128 * n:128 * (n + 1)] for n in range(4)], steps))
        return carry

    with _scope('phase3'):
        lax.fori_loop(0, 3, overlap, None)

    with _scope('wait_b'):
        for cp in cp_b + [cp_wm[2]]:
            cp.wait()
    modulation(2944, 6 * D)
    bias1_v[0:F // 128, :] = b1_v[...].astype(f32)
    bias2_v[0:S // 128, :] = 2.0 * b2_v[...].astype(f32)

    def activate(j):
        g, made = {}, set()

        def emit(r, n, u):
            g[r, 3 - n] = _gelu2(u + bias1_v[pl.ds(4 * j + n, 1), :])
            for i in range(7):
                for k in range(7):
                    need = [_block(o, c) for o, _ in _LHS[i] for c, _ in _LHS[k]]
                    if (i, k) not in made and all(e in g for e in need):
                        made.add((i, k))
                        act_v[i, k, j] = _combine(_LHS[k], lambda c: _combine(
                            _LHS[i], lambda o: g[_block(o, c)])).astype(bf16)
        return emit

    start_w1(8)
    u0 = u_v[...] + first_chunk(3)
    emit0 = activate(0)
    for r in range(4):
        for n in range(4):
            emit0(r, n, u0[QD * r:QD * (r + 1), 128 * n:128 * (n + 1)])

    def mlp1(j, carry):
        with _scope('wait_w1'):
            pltpu.make_async_copy(w1_v.at[0:4], w1_v.at[0:4], sem_w1.at[j]).wait()
        start_w2(j - 1)

        def raw(k, n, t, keep_packed):
            if keep_packed:
                return unpack(packed(w1_v)[4 * j + n, 256 * k + 64 * t:256 * k + 64 * (t + 1), :])
            return w1_v[4 * j + n, 512 * k + 128 * t:512 * k + 128 * (t + 1), :]

        lhs = lambda i, k: jnp.concatenate([unpack(packed(hs_v)[i, k, t]) for t in range(4)], 1)
        _strassen2(lhs, raw, 4, stage_v, activate(j), _ORDER)
        return carry

    with _scope('mlp1'):
        lax.fori_loop(1, n1, mlp1, None)

    def mlp2(j, carry):
        with _scope('wait_w2'):
            pltpu.make_async_copy(w2_v.at[0:4], w2_v.at[0:4], sem_w2.at[j]).wait()

        def raw(k, n, t, keep_packed):
            tile = 4 * t + 3 - k
            if keep_packed:
                return unpack(packed(w2_v)[4 * j + n, 64 * tile:64 * (tile + 1), :])
            return w2_v[4 * j + n, 128 * tile:128 * (tile + 1), :]

        def emit(r, n, y):
            rows = slice(QD * r, QD * (r + 1))
            y = y + bias2_v[pl.ds(4 * j + n, 1), :]
            o_v[j, n, rows, :] = (x1_v[j, n, rows, :] + mod_tile(5, QD * r, QD) * y).astype(bf16)
            pltpu.make_async_copy(o_v.at[j, n, rows, :], o_hbm.at[rows, column(4 * j + n)],
                                  sem_out.at[0]).start()

        lhs = lambda i, k: jnp.concatenate([unpack(packed(act_v)[i, k, t]) for t in range(n1)], 1)
        _strassen2(lhs, raw, n1, stage_v, emit, _ORDER)
        return carry

    with _scope('mlp2'):
        lax.fori_loop(0, n2, mlp2, None)
    with _scope('wait_out'):
        pltpu.make_async_copy(o_v, o_v, sem_out.at[0]).wait()


@jax.jit
def pallas_adaLN_cond__spectral_gfnet__mixer_token_mlp__prompt_kernel(
    A_x, A_w_r, A_w_i, B_x, B_w1, B_b1, B_w2, B_b2, c, w_mod,
):
    del B_x
    assert A_x.shape == (1, S, D)
    dmat, smat = _tables()
    n1, n2 = F // 512, S // 512
    vmem = pltpu.VMEM
    out_t = pl.pallas_call(
        _kernel,
        in_specs=[pl.BlockSpec(memory_space=pltpu.HBM)] * 11,
        out_specs=pl.BlockSpec(memory_space=pltpu.HBM),
        out_shape=jax.ShapeDtypeStruct((D, S), bf16),
        scratch_shapes=[
            vmem((4, 4, D, 128), bf16),
            vmem((2, 288, S), bf16),
            vmem((D, 6 * D), bf16),
            vmem((2, 128, 128), f32),
            vmem((6 * D, 128), f32),
            vmem((NB, 3, 128, 128), bf16),
            vmem((4, D, 512), f32),
            vmem((4, 4, 2, KR, 128), f32),
            vmem((1, 4, 4, 2, KR, 128), f32),
            vmem((1, 2, NB, KR, 128), f32),
            vmem((4, 4, D, 128), f32),
            vmem((4, D, 128), f32),
            vmem((D, 512), f32),
            vmem((4, 4, D, 128), bf16),
            vmem((7, 7, 4, QD, 128), bf16),
            vmem((F // 128, S, 128), bf16),
            vmem((S // 128, F, 128), bf16),
            vmem((SLOTS, 4, F // 4, 128), f32),
            vmem((64, 128), f32),
            vmem((32, 128), f32),
            vmem((4, 4, D, 128), bf16),
            vmem((7, 7, n1, QD, 128), bf16),
            vmem((_DROWS, 128), bf16),
            vmem((_SROWS, 128), f32),
            vmem((2, 1, S), bf16),
            vmem((8, 1, D), bf16),
            vmem((2, F // 128, 128), bf16),
            vmem((S // 128, 128), bf16),
            pltpu.SMEM((1,), jnp.int32),
            pltpu.SemaphoreType.DMA((24,)),
            pltpu.SemaphoreType.DMA((n1,)),
            pltpu.SemaphoreType.DMA((n2,)),
            pltpu.SemaphoreType.DMA((1,)),
        ],
        compiler_params=pltpu.CompilerParams(vmem_limit_bytes=124 * 1024 * 1024),
    )(
        A_x.reshape(S, D).T, A_w_r.T, A_w_i.T, B_w1, B_b1.reshape(F // 128, 128),
        B_w2, B_b2.reshape(S // 128, 128), c, w_mod,
        jnp.asarray(dmat, dtype=bf16), jnp.asarray(smat),
    )
    return out_t.T.reshape(1, S, D)
```

```python
import functools
import math

import jax
import jax.numpy as jnp
import numpy as np
from jax import lax
import jax.experimental.pallas as pl
import jax.experimental.pallas.tpu as pltpu

S, D, F = 2048, 576, 4608
DF = D // 2 + 1
KR = 296
NB = S // 128
QD = D // 4
SLOTS = 3
BAR_C = 11
SHIFT_AT = 13
QJOB = lambda fwd, inv: fwd[1:]
WJOB = lambda fwd, inv: inv
EPS = 1e-5
PROFILE = False
import contextlib
def _scope(n):
    return jax.named_scope(n) if PROFILE else contextlib.nullcontext()

f32 = jnp.float32
bf16 = jnp.bfloat16
_NN = (((1,), (0,)), ((), ()))
_NT = (((1,), (1,)), ((), ()))


def _dot(a, b, dims=_NN):
    return lax.dot_general(a, b, dims, preferred_element_type=f32)


@functools.lru_cache(maxsize=None)
def _tables():
    r = np.arange(64)
    kk = np.arange(32)
    th = lambda k: 2 * np.pi * np.outer(k, r) / D

    def weave(re, im):
        n = re.shape[1]
        return np.stack([re.reshape(4, 8, n), im.reshape(4, 8, n)], 1).reshape(64, n)

    fwd = []
    for q in range(1, 5):
        a, b = th(q + 9 * kk), th(9 - q + 9 * kk)
        fwd.append(np.concatenate([
            weave(np.block([np.cos(a), np.sin(a)]), np.block([-np.sin(a), np.cos(a)])),
            weave(np.block([np.cos(b), -np.sin(b)]), np.block([-np.sin(b), -np.cos(b)]))], 0))
    l0 = np.concatenate(
        [weave(np.cos(th(9 * kk)), -np.sin(th(9 * kk))), np.cos(th(np.array([D // 2])))], 0)
    cw = np.full((65, 1), 2.0)
    cw[0] = cw[64] = 1.0
    l0f = np.zeros((80, 128))
    l0f[:65, :64] = l0
    l0i = np.zeros((64, 128))
    l0i[:, :65] = (l0 * cw).T
    dmat = np.concatenate(fwd + [l0f] + [2 * m.T for m in fwd] + [l0i], 0)

    n2 = np.arange(128)
    a16 = np.arange(16)
    tw = lambda m: np.exp(-2j * np.pi * np.outer(m, n2) / S)
    r1, r2 = tw(127 * a16), tw(127 * a16 + 128)
    parts = np.concatenate([tw(np.arange(8)), tw(8 * a16), r2, r1, r1], 0)
    smat = np.concatenate([parts.real, parts.imag], 0)
    return dmat.astype(np.float32), smat.astype(np.float32)


_DF_OFF = 0
_D0F_OFF = 512
_DI_OFF = 592
_D0I_OFF = 1104
_DROWS = 1168
_SROWS = 144

_S3 = math.sqrt(3.0) / 2
_C1, _S1 = math.cos(2 * math.pi / 9), math.sin(2 * math.pi / 9)
_C2, _S2 = math.cos(4 * math.pi / 9), math.sin(4 * math.pi / 9)


def _radix9_fwd(a):
    b0, br, bd = [], [], []
    for j in range(3):
        t = a[3 + j] + a[6 + j]
        b0.append(a[j] + t)
        br.append(a[j] - 0.5 * t)
        bd.append(a[3 + j] - a[6 + j])
    t = b0[1] + b0[2]
    y0 = b0[0] + t
    y3 = (b0[0] - 0.5 * t, _S3 * (b0[2] - b0[1]))
    c0r, c0i = br[0], -_S3 * bd[0]
    c1r = _C1 * br[1] - (_S3 * _S1) * bd[1]
    c1i = -_S1 * br[1] - (_S3 * _C1) * bd[1]
    c2r = _C2 * br[2] - (_S3 * _S2) * bd[2]
    c2i = -_S2 * br[2] - (_S3 * _C2) * bd[2]
    tr, ti = c1r + c2r, c1i + c2i
    y1 = (c0r + tr, c0i + ti)
    ur, ui = c0r - 0.5 * tr, c0i - 0.5 * ti
    nvr, vi = _S3 * (c2r - c1r), _S3 * (c1i - c2i)
    y4 = (ur + vi, ui + nvr)
    y2 = (ur - vi, nvr - ui)
    return y0, {1: y1, 2: y2, 3: y3, 4: y4}


def _radix9_inv(p0, p):
    (p1r, p1i), (p2r, p2i), (p3r, p3i), (p4r, p4i) = p[1], p[2], p[3], p[4]
    ur, ui = p4r + p2r, p4i - p2i
    vi, nvr = _S3 * (p4r - p2r), _S3 * (p4i + p2i)
    c0r, c0i = p1r + ur, p1i + ui
    tr, ti = p1r - 0.5 * ur, p1i - 0.5 * ui
    c1r, c1i, c2r, c2i = tr - nvr, ti + vi, tr + nvr, ti - vi
    br = [c0r, _C1 * c1r - _S1 * c1i, _C2 * c2r - _S2 * c2i]
    nbd = [_S3 * c0i,
           (_S3 * _S1) * c1r + (_S3 * _C1) * c1i,
           (_S3 * _S2) * c2r + (_S3 * _C2) * c2i]
    ny3 = _S3 * p3i
    t = p0 - 0.5 * p3r
    b0 = [p0 + p3r, t - ny3, t + ny3]
    y = [None] * 9
    for j in range(3):
        t = b0[j] - 0.5 * br[j]
        y[j] = b0[j] + br[j]
        y[3 + j] = t - nbd[j]
        y[6 + j] = t + nbd[j]
    return y


def _radix4(x, inverse):
    (ar, ai), (br, bi), (cr, ci), (dr, di) = x
    sr, si, er, ei = ar + cr, ai + ci, ar - cr, ai - ci
    tr, ti, fr, fi = br + dr, bi + di, br - dr, bi - di
    y1, y3 = (er + fi, ei - fr), (er - fi, ei + fr)
    if inverse:
        y1, y3 = y3, y1
    return [(sr + tr, si + ti), y1, (sr - tr, si - ti), y3]


def _twiddle16(z, e):
    e %= 16
    re, im = z
    if e == 0:
        return z
    if e == 4:
        return (im, -re)
    if e == 12:
        return (-im, re)
    c, s = math.cos(math.pi * e / 8), math.sin(math.pi * e / 8)
    if e % 4 == 2:
        if (c > 0) == (s > 0):
            return (c * (re + im), c * (im - re))
        return (c * (re - im), c * (im + re))
    return (c * re + s * im, c * im - s * re)


class _Stats:
    def __init__(self):
        self.s = [None, None]
        self.q = [None, None]
        self.n = 0

    def add(self, v):
        i = self.n % 2
        self.n += 1
        self.s[i] = v if self.s[i] is None else self.s[i] + v
        self.q[i] = v * v if self.q[i] is None else self.q[i] + v * v

    def scale_shift(self):
        mean = jnp.sum(self.s[0] + self.s[1], axis=0, keepdims=True) * (1.0 / D)
        msq = jnp.sum(self.q[0] + self.q[1], axis=0, keepdims=True) * (1.0 / D)
        r = lax.rsqrt(jnp.maximum(msq - mean * mean, 0.0) + EPS)
        return (jnp.broadcast_to(r, (8, 128)), jnp.broadcast_to(-mean * r, (8, 128)))


_LHS = (((0, 1), (3, 1)), ((2, 1), (3, 1)), ((0, 1),), ((3, 1),), ((0, 1), (1, 1)),
        ((2, 1), (0, -1)), ((1, 1), (3, -1)))
_RHS = (((0, 1), (3, 1)), ((0, 1),), ((1, 1), (3, -1)), ((2, 1), (0, -1)), ((3, 1),),
        ((0, 1), (1, 1)), ((2, 1), (3, 1)))
_OUT = (((0, 1), (3, 1), (4, -1), (6, 1)), ((2, 1), (4, 1)), ((1, 1), (3, 1)),
        ((0, 1), (1, -1), (2, 1), (5, 1)))
_ORDER = ((1, 0, 2, 4, 3, 6, 5), (1, 4, 3, 2, 0, 6, 5), (4, 1, 3, 2, 0, 5, 6))


def _combine(terms, get):
    acc = get(terms[0][0])
    for q, sign in terms[1:]:
        acc = acc + get(q) if sign > 0 else acc - get(q)
    return acc


def _block(outer, inner):
    return 2 * (outer // 2) + inner // 2, 2 * (outer % 2) + inner % 2


class _Quadrants:
    def __init__(self):
        self.acc = [None] * 4
        self.left = [len(t) for t in _OUT]

    def add(self, i, m):
        done = []
        for c, terms in enumerate(_OUT):
            for q, sign in terms:
                if q != i:
                    continue
                prev = self.acc[c]
                if prev is None:
                    self.acc[c] = (m, sign)
                elif prev[1] == sign:
                    self.acc[c] = (prev[0] + m, sign)
                else:
                    self.acc[c] = (m - prev[0] if sign > 0 else prev[0] - m, 1)
                self.left[c] -= 1
                if self.left[c] == 0:
                    assert self.acc[c][1] > 0
                    done.append((c, self.acc[c][0]))
        return done


def _strassen2(lhs, raw, tiles, stage, emit, order):
    def prepare(n):
        i = order[0][n]
        if len(_RHS[i]) > 1:
            for c in range(4):
                for t in range(tiles):
                    stage[n % SLOTS, c, 128 * t:128 * (t + 1), :] = _combine(
                        _RHS[i], lambda q: raw(*_block(q, c), t, False).astype(f32))

    outer = [_Quadrants() for _ in range(4)]
    for n, i in enumerate(order[0]):
        if n + 1 < 7:
            prepare(n + 1)
        inner = _Quadrants()
        for j in order[1 if n < 6 else 2]:
            if len(_RHS[i]) > 1:
                rhs = _combine(_RHS[j], lambda c: stage[n % SLOTS, c, 0:128 * tiles, :])
            elif len(_RHS[j]) > 1:
                rhs = _combine(_RHS[j], lambda c: jnp.concatenate(
                    [raw(*_block(_RHS[i][0][0], c), t, False).astype(f32)
                     for t in range(tiles)], 0))
            else:
                rhs = jnp.concatenate(
                    [raw(*_block(_RHS[i][0][0], _RHS[j][0][0]), t, True)
                     for t in range(tiles)], 0)
            for c, v in inner.add(j, _dot(lhs(i, j), rhs.astype(bf16))):
                for o, w in outer[c].add(i, v):
                    emit(*_block(o, c), w)


def _gelu2(u):
    k0 = math.sqrt(2.0 / math.pi)
    th = jnp.tanh(u * (k0 + (k0 * 0.044715) * (u * u)))
    return u + u * th


def _kernel(x_hbm, wr_hbm, wi_hbm, w1_hbm, b1_hbm, w2_hbm, b2_hbm, c_hbm, wm_hbm,
            dm_hbm, sm_hbm, o_hbm,
            x_v, w_v, wm_v, e_v, mod_v, g_tab, y_v, s_v, z_v, wp_v, x1_v, t_v, u_v, h_v, hs_v, w1_v, w2_v, stage_v, bias1_v, bias2_v, o_v, act_v, dm_v, sm_v, dc_v, wn_v, c_v, b1_v, b2_v, zero_s, sem_in, sem_w1, sem_w2, sem_out):
    n1, n2 = F // 512, S // 512
    c_v, b1_v = c_v.at[0], b1_v.at[0]
    packed = lambda ref: ref.bitcast(jnp.int32)
    unpack = lambda v: pltpu.bitcast(v, bf16)

    zero_s[0] = 0
    zero = zero_s[0]
    z_v, wp_v = z_v.at[zero], wp_v.at[zero]

    def copy_in(i, src, dst):
        return pltpu.make_async_copy(src, dst, sem_in.at[zero + i])

    def wm_copy(i, lo, hi):
        return copy_in(i, wm_hbm.at[:, lo:hi], wm_v.at[:, lo:hi])

    cp_sm = copy_in(0, sm_hbm, sm_v)
    cp_c = copy_in(1, c_hbm, c_v)
    cp_wm = [wm_copy(2, 512, 1152), wm_copy(3, 1792, 2944), wm_copy(4, 2944, 6 * D),
             wm_copy(18, 0, 512), wm_copy(19, 1152, 1792)]
    cp_dm = [copy_in(5, dm_hbm.at[0:_DI_OFF], dm_v.at[0:_DI_OFF]),
             copy_in(22, dm_hbm.at[_DI_OFF:_DROWS], dm_v.at[_DI_OFF:_DROWS])]
    cp_b = [copy_in(6, b1_hbm, b1_v), copy_in(7, b2_hbm, b2_v)]
    cp_x = [copy_in(8 + b, x_hbm.at[:, 128 * (4 * a + b):128 * (4 * a + b + 1)], x_v.at[b, a])
            for b in range(4) for a in range(4)]
    w_rows = (0, 80, 144, 288)
    cp_w = [[copy_in(12 + 2 * g + pln, src.at[w_rows[g]:w_rows[g + 1], :],
                     w_v.at[pln, w_rows[g]:w_rows[g + 1], :])
             for pln, src in enumerate((wr_hbm, wi_hbm))] for g in range(3)]
    cp_w[2] += [copy_in(20 + pln, src.at[288:DF, :], wn_v.at[pln])
                for pln, src in enumerate((wr_hbm, wi_hbm))]
    cp_w10 = [copy_in(23, w1_hbm.at[:, 128 * n:128 * (n + 1)], w1_v.at[n]) for n in range(4)]

    for cp in ([cp_sm, cp_c, cp_wm[0], cp_dm[0]] + cp_x + cp_w[0] + cp_w[1] + cp_w[2] + [cp_wm[3], cp_wm[4], cp_dm[1]]
               + [cp_wm[1]] + cp_w10 + cp_b + [cp_wm[2]]):
        cp.start()

    def column(n):
        return pl.ds(n * 128 if isinstance(n, int) else pl.multiple_of(n * 128, 128), 128)

    def start_w1(j):
        for n in range(4):
            pltpu.make_async_copy(
                w1_hbm.at[:, column(4 * j + n)], w1_v.at[4 * j + n], sem_w1.at[j]).start()

    def start_w2(j):
        for n in range(2):
            pltpu.make_async_copy(
                w2_hbm.at[:, column(2 * j + n)], w2_v.at[2 * j + n], sem_w2.at[j // 2]).start()

    @pl.loop(0, D // 8)
    def _(i):
        u_v[pl.ds(pl.multiple_of(8 * i, 8), 8), :] = jnp.zeros((8, 512), f32)

    with _scope('wait_sm'):
        cp_sm.wait()

    half = _SROWS // 2
    for i in range(NB):
        ar, ai = sm_v[0:8, :], sm_v[half:half + 8, :]
        br, bi = sm_v[8 + i:9 + i, :], sm_v[half + 8 + i:half + 9 + i, :]
        e_v[0, 8 * i:8 * i + 8, :] = ar * br - ai * bi
        e_v[1, 8 * i:8 * i + 8, :] = ar * bi + ai * br

    @pl.loop(0, NB)
    def _(p):
        for i in range(8):
            off = (24 if i == 0 else 40) + 16 - p
            hr, hi = sm_v[pl.ds(off, 16), :], sm_v[pl.ds(off + half, 16), :]
            er, ei = e_v[0, 16 * i:16 * i + 16, :], e_v[1, 16 * i:16 * i + 16, :]
            cr = er * hr - ei * hi
            ci = er * hi + ei * hr
            for t, m in enumerate((cr, ci - cr, cr + ci)):
                g_tab[p, t, 16 * i:16 * i + 16, :] = m.astype(bf16)

    never = sm_v[0:8, :] > 2.0

    def after(v, token):
        return v if token is None else jnp.where(never, token, v)

    class Pace:
        def __init__(self, results, n):
            self.tiles = [(o, r) for o in results for r in range(0, o.shape[0], 8)]
            self.n, self.i = n, 0

        def __call__(self):
            if not self.tiles:
                return None
            o, r = self.tiles[min(self.i, self.n - 1) * len(self.tiles) // self.n]
            self.i += 1
            return o[r:r + 8, 0:128]

    def modulation(lo, hi):
        cv = c_v[...].astype(f32)
        sc = jnp.broadcast_to(cv * jax.nn.sigmoid(cv), (8, D))
        m = _dot(sc, wm_v[:, lo:hi])
        col = lo + lax.broadcasted_iota(jnp.int32, m.shape, 1)
        which = lambda i: (col >= i * D) & (col < (i + 1) * D)
        m = jnp.where(which(1) | which(4), 1.0 + m, m)
        m = jnp.where(which(2), m * (1.0 / (S * D)), m)
        m = jnp.where(which(5), 0.5 * m, m)
        for t in range((hi - lo) // 128):
            row = jnp.broadcast_to(m[0:1, 128 * t:128 * (t + 1)], (128, 128))
            mod_v[lo + 128 * t:lo + 128 * (t + 1), :] = row.T

    def mod_tile(i, row, n=8):
        return mod_v[i * D + row:i * D + row + n, :]

    with _scope('wait_wm0'):
        cp_c.wait()
        cp_wm[0].wait()
    modulation(512, 1152)

    def load_x(b, a, r):
        v = x_v[b, a, r:r + 16, :].astype(f32)
        return v[:8], v[8:]

    def norm_radix9(b, pace):
        for a in range(4):
            lanes = slice(128 * a, 128 * (a + 1))
            st = _Stats()
            for r in range(0, D, 16):
                for hf, v in enumerate(load_x(b, a, r)):
                    st.add(v)
                    x1_v[a, b, r + 8 * hf:r + 8 * hf + 8, :] = v
            rs, sh = st.scale_shift()
            for t in range(0, 64, 16):
                for hf in range(2):
                    r = t + 8 * hf
                    scale = after(rs, pace())
                    h = [(x1_v[a, b, 64 * j + r:64 * j + r + 8, :] * scale + sh)
                         * mod_tile(1, 64 * j + r) for j in range(9)]
                    y0, y = _radix9_fwd(h)
                    y_v[b, 512 + r:520 + r, lanes] = y0
                    for q in range(1, 5):
                        y_v[b, 128 * (q - 1) + r:128 * (q - 1) + r + 8, lanes] = y[q][0]
                        y_v[b, 128 * (q - 1) + 64 + r:128 * (q - 1) + 72 + r, lanes] = y[q][1]

    def channel_dft(b):
        def scatter(o, base, k0):
            for g in range(4):
                r = base + 16 * g
                t = _radix4([(o[r:r + 8, 128 * a:128 * (a + 1)],
                              o[r + 8:r + 16, 128 * a:128 * (a + 1)]) for a in range(4)], False)
                rows = pl.ds(72 * g + k0, 8, stride=9)
                for p0 in range(4):
                    s_v[b, p0, 0, rows, :] = t[p0][0]
                    s_v[b, p0, 1, rows, :] = t[p0][1]

        results = []
        for q in range(1, 5):
            o = _dot(dm_v[_DF_OFF + 128 * (q - 1):_DF_OFF + 128 * q, :],
                     y_v[b, 128 * (q - 1):128 * q, :])
            results.append(o)
            scatter(o, 0, q)
            scatter(o, 64, 9 - q)
        o = _dot(dm_v[_D0F_OFF:_D0F_OFF + 80, 0:64], y_v[b, 512:576, :])
        scatter(o, 0, 0)
        n = [o[64:72, 128 * a:128 * (a + 1)] for a in range(4)]
        s02, d02, s13, d13 = n[0] + n[2], n[0] - n[2], n[1] + n[3], n[1] - n[3]
        nil = jnp.zeros((8, 128), f32)
        for p0, (re, im) in enumerate(((s02 + s13, nil), (d02, -d13), (s02 - s13, nil), (d02, d13))):
            s_v[b, p0, 0, 288:296, :] = re
            s_v[b, p0, 1, 288:296, :] = im
        return results + [o]

    for b in range(4):
        with _scope('wait_x'):
            pltpu.make_async_copy(x_v.at[b], x_v.at[b], sem_in.at[8 + b]).wait()
            if b == 0:
                cp_dm[0].wait()
        norm_radix9(b, Pace(channel_dft(b - 1) if b > 0 else [], 32))

    lane = lax.broadcasted_iota(jnp.int32, (8, 128), 1)
    lane_bit = [((lane >> t) & 1) == 1 for t in range(4)]

    def shuffle(v, token):
        v = [v[0]] + [pltpu.roll(v[a], a, 1) for a in range(15, 0, -1)]
        bits = list(lane_bit)
        if token is not None:
            bits[0] = (after(lane, pltpu.bitcast(token, jnp.int32)) & 1) == 1
        for t in range(4):
            v = [jnp.where(bits[t], v[(p - (1 << t)) % NB], v[p]) for p in range(NB)]
        return v

    def reorder_filter(pln, r, token):
        if r < 288:
            v = [pltpu.bitcast(w_v[pln, r:r + 16, 128 * a:128 * (a + 1)], jnp.int32)
                 for a in range(NB)]
            for p, w in enumerate(shuffle(v, token)):
                wp_v[pln, p, r:r + 16, :] = unpack(w).astype(f32)
        else:
            v = [jnp.broadcast_to(wn_v[pln, :, 128 * a:128 * (a + 1)].astype(f32), (8, 128))
                 for a in range(NB)]
            for p, w in enumerate(shuffle(v, token)):
                wp_v[pln, p, 288:296, :] = w

    gmat = lambda p, t: unpack(packed(g_tab)[p, t])

    span = lambda g: (72 * g, 80 if g == 3 else 72)

    def butterflies_in(g, p0, pace):
        r0, n = span(g)
        for r in range(r0, r0 + n, 8):
            token = pace()
            x = [(s_v[b, p0, 0, r:r + 8, :], s_v[b, p0, 1, r:r + 8, :]) for b in range(4)]
            for b in (range(2) if p0 == 0 else range(1, 4)):
                x[b] = (after(x[b][0], token), after(x[b][1], token))
            x = [_twiddle16(x[b], b * p0) for b in range(4)]
            for p1, (re, im) in enumerate(_radix4(x, False)):
                s_v[p1, p0, 0, r:r + 8, :] = re
                s_v[p1, p0, 1, r:r + 8, :] = im

    def token_filter(g, p0):
        r0, n = span(g)
        rows = slice(r0, r0 + n)
        spec, fwd, inv = [], [], []
        for p1 in range(4):
            p = p0 + 4 * p1
            a, b = s_v[p1, p0, 0, rows, :], s_v[p1, p0, 1, rows, :]
            k1 = _dot(a + b, gmat(p, 0), _NT)
            fwd.append(k1)
            spec.append((k1 - _dot(b, gmat(p, 2), _NT), k1 + _dot(a, gmat(p, 1), _NT)))
        for p1, (xr, xi) in enumerate(spec):
            p = p0 + 4 * p1
            wr, wi = wp_v[0, p, rows, :], wp_v[1, p, rows, :]
            zr, zi = xr * wr - xi * wi, xr * wi + xi * wr
            k1 = _dot(zr + zi, gmat(p, 0))
            inv.append(k1)
            s_v[p1, p0, 0, rows, :] = k1 + _dot(zi, gmat(p, 1))
            s_v[p1, p0, 1, rows, :] = k1 - _dot(zr, gmat(p, 2))
        return fwd, inv

    def butterflies_out(g, p0, pace):
        r0, _ = span(g)
        for q in range(9 + (g == 3)):
            src = pl.ds(r0 + q, 8, stride=9) if q < 9 else pl.ds(288, 8)
            dst = 32 * q + 8 * g if q < 9 else 288
            x = [(s_v[p1, p0, 0, src, :], s_v[p1, p0, 1, src, :]) for p1 in range(4)]
            token = pace()
            for p1 in range(2):
                x[p1] = (after(x[p1][0], token), after(x[p1][1], token))
            for b, z in enumerate(_radix4(x, True)):
                re, im = _twiddle16(z, -b * p0)
                z_v[b, p0, 0, dst:dst + 8, :] = re
                z_v[b, p0, 1, dst:dst + 8, :] = im

    def reorder_rows(lo, hi, results):
        jobs = [(pln, r) for r in range(lo, hi, 16) for pln in range(2)]
        pace = Pace(results, len(jobs))
        for pln, r in jobs:
            reorder_filter(pln, r, pace())

    def shift_response():
        for r in range(0, 64, 8):
            y0, y = _radix9_fwd([mod_tile(0, 64 * j + r) for j in range(9)])
            t_v[0, 512 + r:520 + r, :] = y0
            for q in range(1, 5):
                t_v[0, 128 * (q - 1) + r:128 * (q - 1) + r + 8, :] = y[q][0]
                t_v[0, 128 * (q - 1) + 64 + r:128 * (q - 1) + 72 + r, :] = y[q][1]

        def dc(pln, rows):
            return jnp.broadcast_to(wp_v[pln, 0, rows, :][:, 0:1], (8, 128)) * float(S)

        def store(o, base, k0):
            for g in range(4):
                br, bi = o[base + 16 * g:base + 16 * g + 8], o[base + 16 * g + 8:base + 16 * g + 16]
                rows = pl.ds(72 * g + k0, 8, stride=9)
                wr, wi = dc(0, rows), dc(1, rows)
                dc_v[0, 32 * k0 + 8 * g:32 * k0 + 8 * g + 8, :] = br * wr - bi * wi
                dc_v[1, 32 * k0 + 8 * g:32 * k0 + 8 * g + 8, :] = br * wi + bi * wr

        for q in range(1, 5):
            o = _dot(dm_v[_DF_OFF + 128 * (q - 1):_DF_OFF + 128 * q, :],
                     t_v[0, 128 * (q - 1):128 * q, :])
            store(o, 0, q)
            store(o, 64, 9 - q)
        o = _dot(dm_v[_D0F_OFF:_D0F_OFF + 80, 0:64], t_v[0, 512:576, :])
        store(o, 0, 0)
        for pln in range(2):
            dc_v[pln, 288:296, :] = o[64:72] * dc(pln, pl.ds(288, 8))

    units = [(g, p0) for g in range(4) for p0 in range(4)]
    filter_rows = {0: (80, 112), 1: (112, 128), 2: (128, 144), 6: (144, 192), 7: (192, 224),
                   8: (224, 256), 9: (256, 288), 10: (288, 304)}
    with _scope('wait_w'):
        for cp in cp_w[0]:
            cp.wait()
    start_w1(1)
    start_w1(2)
    reorder_rows(0, 80, channel_dft(3))
    butterflies_in(*units[0], Pace([], 1))
    for cp in cp_w[1]:
        cp.wait()
    for i, unit in enumerate(units):
        if i == 6:
            with _scope('wait_w'):
                for cp in cp_w[2]:
                    cp.wait()
            start_w1(3)
            start_w1(4)
        if i == BAR_C:
            with _scope('wait_w'):
                cp_wm[3].wait()
                cp_wm[4].wait()
            modulation(0, 512)
        if i == BAR_C + 1:
            modulation(1152, 1792)
        fwd, inv = token_filter(*unit)
        if i > 0:
            butterflies_out(*units[i - 1], Pace(QJOB(fwd, inv), 10))
        if i == 0:
            butterflies_in(*units[1], Pace(fwd[:3], 10))
        if i + 2 < len(units):
            butterflies_in(*units[i + 2], Pace(inv, 10))
        if i in filter_rows:
            reorder_rows(*filter_rows[i], WJOB(fwd, inv))
        if i == SHIFT_AT:
            shift_response()
    butterflies_out(*units[-1], Pace([], 1))

    with _scope('wait_wm1'):
        cp_dm[1].wait()
        cp_wm[1].wait()

    def channel_idft(b):
        def gather(r):
            z = [(z_v[b, p0, 0, r:r + 8, :], z_v[b, p0, 1, r:r + 8, :]) for p0 in range(4)]
            z[0] = (z[0][0] + dc_v[0, r:r + 8, :], z[0][1] + dc_v[1, r:r + 8, :])
            t = _radix4(z, True)
            return [jnp.concatenate([t[a][pln] for a in range(4)], 1) for pln in range(2)]

        results = []
        for q in range(1, 5):
            rhs = jnp.concatenate(
                sum((gather(32 * k + 8 * g) for k in (q, 9 - q) for g in range(4)), []), 0)
            results.append(_dot(dm_v[_DI_OFF + 128 * (q - 1):_DI_OFF + 128 * q, :], rhs))
            y_v[b, 128 * (q - 1):128 * q, :] = results[-1]
        rhs = jnp.concatenate(sum((gather(8 * g) for g in range(4)), []) + gather(288)[:1], 0)
        results.append(_dot(dm_v[_D0I_OFF:_D0I_OFF + 64, 0:72], rhs))
        y_v[b, 512:576, :] = results[-1]
        return results

    def residual_norms(b, pace):
        norm = []
        for a in range(4):
            lanes = slice(128 * a, 128 * (a + 1))
            st = _Stats()
            for t in range(0, 64, 16):
                for hf in range(2):
                    r = t + 8 * hf
                    p = {q: (y_v[b, 128 * (q - 1) + r:128 * (q - 1) + r + 8, lanes],
                             y_v[b, 128 * (q - 1) + 64 + r:128 * (q - 1) + 72 + r, lanes])
                         for q in range(1, 5)}
                    token = pace()
                    for q in (3, 4):
                        p[q] = (after(p[q][0], token), after(p[q][1], token))
                    y = _radix9_inv(y_v[b, 512 + r:520 + r, lanes], p)
                    for j in range(9):
                        row = 64 * j + r
                        x1 = x1_v[a, b, row:row + 8, :] + mod_tile(2, row) * y[j]
                        st.add(x1)
                        x1_v[a, b, row:row + 8, :] = x1
            rs, sh = st.scale_shift()
            st = _Stats()
            for row in range(0, D, 8):
                if row % 120 == 0:
                    scale = after(rs, pace())
                t = (x1_v[a, b, row:row + 8, :] * scale + sh) * mod_tile(4, row) + mod_tile(3, row)
                st.add(t)
                t_v[a, row:row + 8, :] = t
            rs, sh = st.scale_shift()
            norm.append((rs, jnp.concatenate([sh, sh], 0)))
        for row in range(0, QD, 16):
            h = {}
            for k in range(4):
                if k < 3:
                    token = pace()
                scale = after(norm[k][0], token)
                scale = jnp.concatenate([scale, scale], 0)
                for r in range(4):
                    rows = slice(QD * r + row, QD * r + row + 16)
                    h[r, k] = t_v[k, rows, :] * scale + norm[k][1]
                    h_v[b, k, rows, :] = h[r, k].astype(bf16)
            for i in range(7):
                quad = [_combine(_LHS[i], lambda o: h[_block(o, c)]) for c in range(4)]
                for j in range(7):
                    hs_v[i, j, b, row:row + 16, :] = _combine(
                        _LHS[j], lambda c: quad[c]).astype(bf16)

    def first_chunk(b):
        lhs = jnp.concatenate([unpack(packed(h_v)[b, a]) for a in range(4)], 1)
        rhs = jnp.concatenate([jnp.concatenate(
            [unpack(packed(w1_v)[n, pl.ds(pl.multiple_of(64 * (4 * a + b), 64), 64), :])
             for a in range(4)], 0) for n in range(4)], 1)
        return _dot(lhs, rhs)

    steps = 4 * (8 + 5) + 27
    channel_idft(0)
    modulation(1792, 2944)
    residual_norms(0, Pace(sum((channel_idft(b) for b in range(1, 4)), []), steps))
    with _scope('wait_w10'):
        pltpu.make_async_copy(w1_v.at[0:4], w1_v.at[0:4], sem_in.at[23]).wait()

    def overlap(b, carry):
        start_w1(5 + b)
        part = first_chunk(b)
        u_v[...] += part
        residual_norms(b + 1, Pace([part[:, 128 * n:128 * (n + 1)] for n in range(4)], steps))
        return carry

    with _scope('phase3'):
        lax.fori_loop(0, 3, overlap, None)

    with _scope('wait_b'):
        for cp in cp_b + [cp_wm[2]]:
            cp.wait()
    modulation(2944, 6 * D)
    bias1_v[0:F // 128, :] = b1_v[...].astype(f32)
    bias2_v[0:S // 128, :] = 2.0 * b2_v[...].astype(f32)

    def activate(j):
        g, made = {}, set()

        def emit(r, n, u):
            g[r, 3 - n] = _gelu2(u + bias1_v[pl.ds(4 * j + n, 1), :])
            for i in range(7):
                for k in range(7):
                    need = [_block(o, c) for o, _ in _LHS[i] for c, _ in _LHS[k]]
                    if (i, k) not in made and all(e in g for e in need):
                        made.add((i, k))
                        act_v[i, k, j] = _combine(_LHS[k], lambda c: _combine(
                            _LHS[i], lambda o: g[_block(o, c)])).astype(bf16)
        return emit

    start_w1(8)
    u0 = u_v[...] + first_chunk(3)
    emit0 = activate(0)
    for r in range(4):
        for n in range(4):
            emit0(r, n, u0[QD * r:QD * (r + 1), 128 * n:128 * (n + 1)])

    def mlp1(j, carry):
        with _scope('wait_w1'):
            pltpu.make_async_copy(w1_v.at[0:4], w1_v.at[0:4], sem_w1.at[j]).wait()
        start_w2(j - 1)

        def raw(k, n, t, keep_packed):
            if keep_packed:
                return unpack(packed(w1_v)[4 * j + n, 256 * k + 64 * t:256 * k + 64 * (t + 1), :])
            return w1_v[4 * j + n, 512 * k + 128 * t:512 * k + 128 * (t + 1), :]

        lhs = lambda i, k: jnp.concatenate([unpack(packed(hs_v)[i, k, t]) for t in range(4)], 1)
        _strassen2(lhs, raw, 4, stage_v, activate(j), _ORDER)
        return carry

    with _scope('mlp1'):
        lax.fori_loop(1, n1, mlp1, None)

    def mlp2(j, carry):
        with _scope('wait_w2'):
            pltpu.make_async_copy(w2_v.at[0:4], w2_v.at[0:4], sem_w2.at[j]).wait()

        def raw(k, n, t, keep_packed):
            tile = 4 * t + 3 - k
            if keep_packed:
                return unpack(packed(w2_v)[4 * j + n, 64 * tile:64 * (tile + 1), :])
            return w2_v[4 * j + n, 128 * tile:128 * (tile + 1), :]

        def emit(r, n, y):
            rows = slice(QD * r, QD * (r + 1))
            y = y + bias2_v[pl.ds(4 * j + n, 1), :]
            o_v[j, n, rows, :] = (x1_v[j, n, rows, :] + mod_tile(5, QD * r, QD) * y).astype(bf16)
            pltpu.make_async_copy(o_v.at[j, n, rows, :], o_hbm.at[rows, column(4 * j + n)],
                                  sem_out.at[0]).start()

        lhs = lambda i, k: jnp.concatenate([unpack(packed(act_v)[i, k, t]) for t in range(n1)], 1)
        _strassen2(lhs, raw, n1, stage_v, emit, _ORDER)
        return carry

    with _scope('mlp2'):
        lax.fori_loop(0, n2, mlp2, None)
    with _scope('wait_out'):
        pltpu.make_async_copy(o_v, o_v, sem_out.at[0]).wait()


@jax.jit
def pallas_adaLN_cond__spectral_gfnet__mixer_token_mlp__prompt_kernel(
    A_x, A_w_r, A_w_i, B_x, B_w1, B_b1, B_w2, B_b2, c, w_mod,
):
    del B_x
    assert A_x.shape == (1, S, D)
    dmat, smat = _tables()
    n1, n2 = F // 512, S // 512
    vmem = pltpu.VMEM
    out_t = pl.pallas_call(
        _kernel,
        in_specs=[pl.BlockSpec(memory_space=pltpu.HBM)] * 11,
        out_specs=pl.BlockSpec(memory_space=pltpu.HBM),
        out_shape=jax.ShapeDtypeStruct((D, S), bf16),
        scratch_shapes=[
            vmem((4, 4, D, 128), bf16),
            vmem((2, 288, S), bf16),
            vmem((D, 6 * D), bf16),
            vmem((2, 128, 128), f32),
            vmem((6 * D, 128), f32),
            vmem((NB, 3, 128, 128), bf16),
            vmem((4, D, 512), f32),
            vmem((4, 4, 2, KR, 128), f32),
            vmem((1, 4, 4, 2, KR, 128), f32),
            vmem((1, 2, NB, KR, 128), f32),
            vmem((4, 4, D, 128), f32),
            vmem((4, D, 128), f32),
            vmem((D, 512), f32),
            vmem((4, 4, D, 128), bf16),
            vmem((7, 7, 4, QD, 128), bf16),
            vmem((F // 128, S, 128), bf16),
            vmem((S // 128, F, 128), bf16),
            vmem((SLOTS, 4, F // 4, 128), f32),
            vmem((64, 128), f32),
            vmem((32, 128), f32),
            vmem((4, 4, D, 128), bf16),
            vmem((7, 7, n1, QD, 128), bf16),
            vmem((_DROWS, 128), bf16),
            vmem((_SROWS, 128), f32),
            vmem((2, KR, 128), f32),
            vmem((2, 1, S), bf16),
            vmem((8, 1, D), bf16),
            vmem((2, F // 128, 128), bf16),
            vmem((S // 128, 128), bf16),
            pltpu.SMEM((1,), jnp.int32),
            pltpu.SemaphoreType.DMA((24,)),
            pltpu.SemaphoreType.DMA((n1,)),
            pltpu.SemaphoreType.DMA((n2,)),
            pltpu.SemaphoreType.DMA((1,)),
        ],
        compiler_params=pltpu.CompilerParams(vmem_limit_bytes=124 * 1024 * 1024),
    )(
        A_x.reshape(S, D).T, A_w_r.T, A_w_i.T, B_w1, B_b1.reshape(F // 128, 128),
        B_w2, B_b2.reshape(S // 128, 128), c, w_mod,
        jnp.asarray(dmat, dtype=bf16), jnp.asarray(smat),
    )
    return out_t.T.reshape(1, S, D)
```

```python
import functools
import math

import jax
import jax.numpy as jnp
import numpy as np
from jax import lax
import jax.experimental.pallas as pl
import jax.experimental.pallas.tpu as pltpu

S, D, F = 2048, 576, 4608
DF = D // 2 + 1
KR = 296
NB = S // 128
QD = D // 4
SLOTS = 3
EPS = 1e-5

f32 = jnp.float32
bf16 = jnp.bfloat16
_NN = (((1,), (0,)), ((), ()))
_NT = (((1,), (1,)), ((), ()))


def _dot(a, b, dims=_NN):
    return lax.dot_general(a, b, dims, preferred_element_type=f32)


_DF_OFF = 0
_D0F_OFF = 512
_DI_OFF = 592
_D0I_OFF = 1104
_DROWS = 1168
_SROWS = 144


@functools.lru_cache(maxsize=None)
def _tables():
    r = np.arange(64)
    kk = np.arange(32)
    th = lambda k: 2 * np.pi * np.outer(k, r) / D

    def weave(re, im):
        n = re.shape[1]
        return np.stack([re.reshape(4, 8, n), im.reshape(4, 8, n)], 1).reshape(64, n)

    fwd = []
    for q in range(1, 5):
        a, b = th(q + 9 * kk), th(9 - q + 9 * kk)
        fwd.append(np.concatenate([
            weave(np.block([np.cos(a), np.sin(a)]), np.block([-np.sin(a), np.cos(a)])),
            weave(np.block([np.cos(b), -np.sin(b)]), np.block([-np.sin(b), -np.cos(b)]))], 0))
    l0 = np.concatenate(
        [weave(np.cos(th(9 * kk)), -np.sin(th(9 * kk))), np.cos(th(np.array([D // 2])))], 0)
    weight = np.full((65, 1), 2.0)
    weight[0] = weight[64] = 1.0
    l0f = np.zeros((80, 128))
    l0f[:65, :64] = l0
    l0i = np.zeros((64, 128))
    l0i[:, :65] = (l0 * weight).T
    channel = np.concatenate(fwd + [l0f] + [2 * m.T for m in fwd] + [l0i], 0)

    n = np.arange(128)
    a16 = np.arange(16)
    tw = lambda m: np.exp(-2j * np.pi * np.outer(m, n) / S)
    r1, r2 = tw(127 * a16), tw(127 * a16 + 128)
    parts = np.concatenate([tw(np.arange(8)), tw(8 * a16), r2, r1, r1], 0)
    token = np.concatenate([parts.real, parts.imag], 0)
    return channel.astype(np.float32).astype(bf16), token.astype(np.float32)


_S3 = math.sqrt(3.0) / 2
_C1, _S1 = math.cos(2 * math.pi / 9), math.sin(2 * math.pi / 9)
_C2, _S2 = math.cos(4 * math.pi / 9), math.sin(4 * math.pi / 9)


def _radix9_fwd(a):
    b0, br, bd = [], [], []
    for j in range(3):
        t = a[3 + j] + a[6 + j]
        b0.append(a[j] + t)
        br.append(a[j] - 0.5 * t)
        bd.append(a[3 + j] - a[6 + j])
    t = b0[1] + b0[2]
    y0 = b0[0] + t
    y3 = (b0[0] - 0.5 * t, _S3 * (b0[2] - b0[1]))
    c0r, c0i = br[0], -_S3 * bd[0]
    c1r = _C1 * br[1] - (_S3 * _S1) * bd[1]
    c1i = -_S1 * br[1] - (_S3 * _C1) * bd[1]
    c2r = _C2 * br[2] - (_S3 * _S2) * bd[2]
    c2i = -_S2 * br[2] - (_S3 * _C2) * bd[2]
    tr, ti = c1r + c2r, c1i + c2i
    y1 = (c0r + tr, c0i + ti)
    ur, ui = c0r - 0.5 * tr, c0i - 0.5 * ti
    nvr, vi = _S3 * (c2r - c1r), _S3 * (c1i - c2i)
    y4 = (ur + vi, ui + nvr)
    y2 = (ur - vi, nvr - ui)
    return y0, {1: y1, 2: y2, 3: y3, 4: y4}


def _radix9_inv(p0, p):
    (p1r, p1i), (p2r, p2i), (p3r, p3i), (p4r, p4i) = p[1], p[2], p[3], p[4]
    ur, ui = p4r + p2r, p4i - p2i
    vi, nvr = _S3 * (p4r - p2r), _S3 * (p4i + p2i)
    c0r, c0i = p1r + ur, p1i + ui
    tr, ti = p1r - 0.5 * ur, p1i - 0.5 * ui
    c1r, c1i, c2r, c2i = tr - nvr, ti + vi, tr + nvr, ti - vi
    br = [c0r, _C1 * c1r - _S1 * c1i, _C2 * c2r - _S2 * c2i]
    nbd = [_S3 * c0i,
           (_S3 * _S1) * c1r + (_S3 * _C1) * c1i,
           (_S3 * _S2) * c2r + (_S3 * _C2) * c2i]
    ny3 = _S3 * p3i
    t = p0 - 0.5 * p3r
    b0 = [p0 + p3r, t - ny3, t + ny3]
    y = [None] * 9
    for j in range(3):
        t = b0[j] - 0.5 * br[j]
        y[j] = b0[j] + br[j]
        y[3 + j] = t - nbd[j]
        y[6 + j] = t + nbd[j]
    return y


def _radix4(x, inverse):
    (ar, ai), (br, bi), (cr, ci), (dr, di) = x
    sr, si, er, ei = ar + cr, ai + ci, ar - cr, ai - ci
    tr, ti, fr, fi = br + dr, bi + di, br - dr, bi - di
    y1, y3 = (er + fi, ei - fr), (er - fi, ei + fr)
    if inverse:
        y1, y3 = y3, y1
    return [(sr + tr, si + ti), y1, (sr - tr, si - ti), y3]


def _twiddle16(z, e):
    e %= 16
    re, im = z
    if e == 0:
        return z
    if e == 4:
        return (im, -re)
    if e == 12:
        return (-im, re)
    c, s = math.cos(math.pi * e / 8), math.sin(math.pi * e / 8)
    if e % 4 == 2:
        if (c > 0) == (s > 0):
            return (c * (re + im), c * (im - re))
        return (c * (re - im), c * (im + re))
    return (c * re + s * im, c * im - s * re)


class _Stats:
    def __init__(self):
        self.s = [None, None]
        self.q = [None, None]
        self.n = 0

    def add(self, v):
        i = self.n % 2
        self.n += 1
        self.s[i] = v if self.s[i] is None else self.s[i] + v
        self.q[i] = v * v if self.q[i] is None else self.q[i] + v * v

    def scale_shift(self):
        mean = jnp.sum(self.s[0] + self.s[1], axis=0, keepdims=True) * (1.0 / D)
        msq = jnp.sum(self.q[0] + self.q[1], axis=0, keepdims=True) * (1.0 / D)
        r = lax.rsqrt(jnp.maximum(msq - mean * mean, 0.0) + EPS)
        return (jnp.broadcast_to(r, (8, 128)), jnp.broadcast_to(-mean * r, (8, 128)))


class _Pace:
    def __init__(self, results, n):
        self.tiles = [(o, r) for o in results for r in range(0, o.shape[0], 8)]
        self.n, self.i = n, 0

    def __call__(self):
        if not self.tiles:
            return None
        o, r = self.tiles[min(self.i, self.n - 1) * len(self.tiles) // self.n]
        self.i += 1
        return o[r:r + 8, 0:128]


_LHS = (((0, 1), (3, 1)), ((2, 1), (3, 1)), ((0, 1),), ((3, 1),), ((0, 1), (1, 1)),
        ((2, 1), (0, -1)), ((1, 1), (3, -1)))
_RHS = (((0, 1), (3, 1)), ((0, 1),), ((1, 1), (3, -1)), ((2, 1), (0, -1)), ((3, 1),),
        ((0, 1), (1, 1)), ((2, 1), (3, 1)))
_OUT = (((0, 1), (3, 1), (4, -1), (6, 1)), ((2, 1), (4, 1)), ((1, 1), (3, 1)),
        ((0, 1), (1, -1), (2, 1), (5, 1)))
_ORDER = ((1, 0, 2, 4, 3, 6, 5), (1, 4, 3, 6, 2, 0, 5), (4, 1, 2, 0, 5, 3, 6))


def _combine(terms, get):
    acc = get(terms[0][0])
    for q, sign in terms[1:]:
        acc = acc + get(q) if sign > 0 else acc - get(q)
    return acc


def _block(outer, inner):
    return 2 * (outer // 2) + inner // 2, 2 * (outer % 2) + inner % 2


class _Quadrants:
    def __init__(self):
        self.acc = [None] * 4
        self.left = [len(t) for t in _OUT]

    def add(self, i, m):
        done = []
        for c, terms in enumerate(_OUT):
            for q, sign in terms:
                if q != i:
                    continue
                prev = self.acc[c]
                if prev is None:
                    self.acc[c] = (m, sign)
                elif prev[1] == sign:
                    self.acc[c] = (prev[0] + m, sign)
                else:
                    self.acc[c] = (m - prev[0] if sign > 0 else prev[0] - m, 1)
                self.left[c] -= 1
                if self.left[c] == 0:
                    assert self.acc[c][1] > 0
                    done.append((c, self.acc[c][0]))
        return done


def _strassen2(lhs, weights, tiles, stage, emit):
    assert len(_RHS[_ORDER[0][0]]) == 1

    def prepare(n):
        i = _ORDER[0][n]
        if len(_RHS[i]) > 1:
            for c in range(4):
                for t in range(tiles):
                    stage[n % SLOTS, c, 128 * t:128 * (t + 1), :] = _combine(
                        _RHS[i], lambda q: weights(*_block(q, c), t).astype(f32))

    outer = [_Quadrants() for _ in range(4)]
    for n, i in enumerate(_ORDER[0]):
        if n + 1 < 7:
            prepare(n + 1)
        inner = _Quadrants()
        for j in _ORDER[1 if n < 6 else 2]:
            if len(_RHS[i]) > 1:
                rhs = _combine(_RHS[j], lambda c: stage[n % SLOTS, c, 0:128 * tiles, :])
            elif len(_RHS[j]) > 1:
                rhs = _combine(_RHS[j], lambda c: jnp.concatenate(
                    [weights(*_block(_RHS[i][0][0], c), t).astype(f32)
                     for t in range(tiles)], 0))
            else:
                rhs = jnp.concatenate(
                    [weights(*_block(_RHS[i][0][0], _RHS[j][0][0]), t)
                     for t in range(tiles)], 0)
            for c, v in inner.add(j, _dot(lhs(i, j), rhs.astype(bf16))):
                for o, w in outer[c].add(i, v):
                    emit(*_block(o, c), w)


def _gelu2(u):
    k0 = math.sqrt(2.0 / math.pi)
    th = jnp.tanh(u * (k0 + (k0 * 0.044715) * (u * u)))
    return u + u * th


def _kernel(x_hbm, wr_hbm, wi_hbm, w1_hbm, b1_hbm, w2_hbm, b2_hbm, c_hbm, wm_hbm,
            dm_hbm, sm_hbm, o_hbm,
            x_v, w_v, wm_v, e_v, mod_v, g_tab, y_v, s_v, z_v, wp_v, x1_v, t_v, u_v,
            h_v, hs_v, w1_v, w2_v, stage_v, bias1_v, bias2_v, o_v, act_v, dm_v, sm_v,
            dc_v, wn_v, c_v, b1_v, b2_v, zero_s, sem_in, sem_w1, sem_w2, sem_out):
    n1, n2 = F // 512, S // 512
    c_v, b1_v = c_v.at[0], b1_v.at[0]
    as_bf16 = lambda v: pltpu.bitcast(v, bf16)

    zero_s[0] = 0
    zero = zero_s[0]
    z_v, wp_v = z_v.at[zero], wp_v.at[zero]

    def copy_in(i, src, dst):
        return pltpu.make_async_copy(src, dst, sem_in.at[zero + i])

    def wm_copy(i, lo, hi):
        return copy_in(i, wm_hbm.at[:, lo:hi], wm_v.at[:, lo:hi])

    cp_sm = copy_in(0, sm_hbm, sm_v)
    cp_c = copy_in(1, c_hbm, c_v)
    cp_ca, cp_sb_cb, cp_gb = wm_copy(2, 512, 1152), wm_copy(3, 1792, 2944), wm_copy(4, 2944, 6 * D)
    cp_sa, cp_ga = wm_copy(18, 0, 512), wm_copy(19, 1152, 1792)
    cp_dm = [copy_in(5, dm_hbm.at[0:_DI_OFF], dm_v.at[0:_DI_OFF]),
             copy_in(22, dm_hbm.at[_DI_OFF:_DROWS], dm_v.at[_DI_OFF:_DROWS])]
    cp_b = [copy_in(6, b1_hbm, b1_v), copy_in(7, b2_hbm, b2_v)]
    cp_x = [copy_in(8 + b, x_hbm.at[:, 128 * (4 * a + b):128 * (4 * a + b + 1)], x_v.at[b, a])
            for b in range(4) for a in range(4)]
    w_rows = (0, 80, 144, 288)
    cp_w = [[copy_in(12 + 2 * g + pln, src.at[w_rows[g]:w_rows[g + 1], :],
                     w_v.at[pln, w_rows[g]:w_rows[g + 1], :])
             for pln, src in enumerate((wr_hbm, wi_hbm))] for g in range(3)]
    cp_w[2] += [copy_in(20 + pln, src.at[288:DF, :], wn_v.at[pln])
                for pln, src in enumerate((wr_hbm, wi_hbm))]
    cp_w1 = [copy_in(23, w1_hbm.at[:, 128 * n:128 * (n + 1)], w1_v.at[n]) for n in range(4)]

    for cp in ([cp_sm, cp_c, cp_ca, cp_dm[0]] + cp_x + cp_w[0] + cp_w[1] + cp_w[2]
               + [cp_sa, cp_ga, cp_dm[1], cp_sb_cb] + cp_w1 + cp_b + [cp_gb]):
        cp.start()

    def wait_all(buf, sem):
        pltpu.make_async_copy(buf, buf, sem).wait()

    def column(n):
        return pl.ds(n * 128 if isinstance(n, int) else pl.multiple_of(n * 128, 128), 128)

    def start_w1(j):
        for n in range(4):
            pltpu.make_async_copy(
                w1_hbm.at[:, column(4 * j + n)], w1_v.at[4 * j + n], sem_w1.at[j]).start()

    def start_w2(j):
        for n in range(2):
            pltpu.make_async_copy(
                w2_hbm.at[:, column(2 * j + n)], w2_v.at[2 * j + n], sem_w2.at[j // 2]).start()

    @pl.loop(0, D // 8)
    def _(i):
        u_v[pl.ds(pl.multiple_of(8 * i, 8), 8), :] = jnp.zeros((8, 512), f32)

    cp_sm.wait()
    half = _SROWS // 2
    for i in range(NB):
        ar, ai = sm_v[0:8, :], sm_v[half:half + 8, :]
        br, bi = sm_v[8 + i:9 + i, :], sm_v[half + 8 + i:half + 9 + i, :]
        e_v[0, 8 * i:8 * i + 8, :] = ar * br - ai * bi
        e_v[1, 8 * i:8 * i + 8, :] = ar * bi + ai * br

    @pl.loop(0, NB)
    def _(p):
        for i in range(8):
            off = (24 if i == 0 else 40) + 16 - p
            hr, hi = sm_v[pl.ds(off, 16), :], sm_v[pl.ds(off + half, 16), :]
            er, ei = e_v[0, 16 * i:16 * i + 16, :], e_v[1, 16 * i:16 * i + 16, :]
            cr = er * hr - ei * hi
            ci = er * hi + ei * hr
            for t, m in enumerate((cr, ci - cr, cr + ci)):
                g_tab[p, t, 8 * i:8 * i + 8, :] = pltpu.bitcast(m.astype(bf16), jnp.int32)

    never = sm_v[0:8, :] > 2.0

    def after(v, token):
        return v if token is None else jnp.where(never, token, v)

    def modulation(lo, hi):
        cv = c_v[...].astype(f32)
        sc = jnp.broadcast_to(cv * jax.nn.sigmoid(cv), (8, D))
        m = _dot(sc, wm_v[:, lo:hi])
        col = lo + lax.broadcasted_iota(jnp.int32, m.shape, 1)
        which = lambda i: (col >= i * D) & (col < (i + 1) * D)
        m = jnp.where(which(1) | which(4), 1.0 + m, m)
        m = jnp.where(which(2), m * (1.0 / (S * D)), m)
        m = jnp.where(which(5), 0.5 * m, m)
        for t in range((hi - lo) // 128):
            row = jnp.broadcast_to(m[0:1, 128 * t:128 * (t + 1)], (128, 128))
            mod_v[lo + 128 * t:lo + 128 * (t + 1), :] = row.T

    def mod_tile(i, row, n=8):
        return mod_v[i * D + row:i * D + row + n, :]

    cp_c.wait()
    cp_ca.wait()
    modulation(512, 1152)

    def norm_radix9(b, pace):
        for a in range(4):
            lanes = slice(128 * a, 128 * (a + 1))
            st = _Stats()
            for r in range(0, D, 16):
                v = x_v[b, a, r:r + 16, :].astype(f32)
                for hf, tile in enumerate((v[:8], v[8:])):
                    st.add(tile)
                    x1_v[a, b, r + 8 * hf:r + 8 * hf + 8, :] = tile
            rs, sh = st.scale_shift()
            for r in range(0, 64, 8):
                scale = after(rs, pace())
                h = [(x1_v[a, b, 64 * j + r:64 * j + r + 8, :] * scale + sh)
                     * mod_tile(1, 64 * j + r) for j in range(9)]
                y0, y = _radix9_fwd(h)
                y_v[b, 512 + r:520 + r, lanes] = y0
                for q in range(1, 5):
                    y_v[b, 128 * (q - 1) + r:128 * (q - 1) + r + 8, lanes] = y[q][0]
                    y_v[b, 128 * (q - 1) + 64 + r:128 * (q - 1) + 72 + r, lanes] = y[q][1]

    def channel_dft(b):
        def scatter(o, base, k0):
            for g in range(4):
                r = base + 16 * g
                t = _radix4([(o[r:r + 8, 128 * a:128 * (a + 1)],
                              o[r + 8:r + 16, 128 * a:128 * (a + 1)]) for a in range(4)], False)
                rows = pl.ds(72 * g + k0, 8, stride=9)
                for p0 in range(4):
                    s_v[b, p0, 0, rows, :] = t[p0][0]
                    s_v[b, p0, 1, rows, :] = t[p0][1]

        results = []
        for q in range(1, 5):
            o = _dot(dm_v[_DF_OFF + 128 * (q - 1):_DF_OFF + 128 * q, :],
                     y_v[b, 128 * (q - 1):128 * q, :])
            results.append(o)
            scatter(o, 0, q)
            scatter(o, 64, 9 - q)
        o = _dot(dm_v[_D0F_OFF:_D0F_OFF + 80, 0:64], y_v[b, 512:576, :])
        scatter(o, 0, 0)
        n = [o[64:72, 128 * a:128 * (a + 1)] for a in range(4)]
        s02, d02, s13, d13 = n[0] + n[2], n[0] - n[2], n[1] + n[3], n[1] - n[3]
        nil = jnp.zeros((8, 128), f32)
        for p0, (re, im) in enumerate(((s02 + s13, nil), (d02, -d13), (s02 - s13, nil), (d02, d13))):
            s_v[b, p0, 0, 288:296, :] = re
            s_v[b, p0, 1, 288:296, :] = im
        return results + [o]

    for b in range(4):
        wait_all(x_v.at[b], sem_in.at[8 + b])
        if b == 0:
            cp_dm[0].wait()
        norm_radix9(b, _Pace(channel_dft(b - 1) if b > 0 else [], 32))

    lane = lax.broadcasted_iota(jnp.int32, (8, 128), 1)
    lane_bit = [((lane >> t) & 1) == 1 for t in range(4)]

    def shuffle(v, token):
        v = [v[0]] + [pltpu.roll(v[a], a, 1) for a in range(15, 0, -1)]
        bits = list(lane_bit)
        if token is not None:
            bits[0] = (after(lane, pltpu.bitcast(token, jnp.int32)) & 1) == 1
        for t in range(4):
            v = [jnp.where(bits[t], v[(p - (1 << t)) % NB], v[p]) for p in range(NB)]
        return v

    def reorder_filter(lo, hi, results):
        jobs = [(pln, r) for r in range(lo, hi, 16) for pln in range(2)]
        pace = _Pace(results, len(jobs))
        for pln, r in jobs:
            token = pace()
            if r < 288:
                v = [pltpu.bitcast(w_v[pln, r:r + 16, 128 * a:128 * (a + 1)], jnp.int32)
                     for a in range(NB)]
                for p, w in enumerate(shuffle(v, token)):
                    wp_v[pln, p, r:r + 16, :] = as_bf16(w).astype(f32)
            else:
                v = [jnp.broadcast_to(wn_v[pln, :, 128 * a:128 * (a + 1)].astype(f32), (8, 128))
                     for a in range(NB)]
                for p, w in enumerate(shuffle(v, token)):
                    wp_v[pln, p, 288:296, :] = w

    gmat = lambda p, t: as_bf16(g_tab[p, t])
    span = lambda g: (72 * g, 80 if g == 3 else 72)

    def butterflies_in(g, p0, pace):
        r0, n = span(g)
        for r in range(r0, r0 + n, 8):
            token = pace()
            x = [(s_v[b, p0, 0, r:r + 8, :], s_v[b, p0, 1, r:r + 8, :]) for b in range(4)]
            for b in (range(2) if p0 == 0 else range(1, 4)):
                x[b] = (after(x[b][0], token), after(x[b][1], token))
            x = [_twiddle16(x[b], b * p0) for b in range(4)]
            for p1, (re, im) in enumerate(_radix4(x, False)):
                s_v[p1, p0, 0, r:r + 8, :] = re
                s_v[p1, p0, 1, r:r + 8, :] = im

    def token_filter(g, p0):
        r0, n = span(g)
        rows = slice(r0, r0 + n)
        spec, fwd, inv = [], [], []
        for p1 in range(4):
            p = p0 + 4 * p1
            a, b = s_v[p1, p0, 0, rows, :], s_v[p1, p0, 1, rows, :]
            k1 = _dot(a + b, gmat(p, 0), _NT)
            fwd.append(k1)
            spec.append((k1 - _dot(b, gmat(p, 2), _NT), k1 + _dot(a, gmat(p, 1), _NT)))
        for p1, (xr, xi) in enumerate(spec):
            p = p0 + 4 * p1
            wr, wi = wp_v[0, p, rows, :], wp_v[1, p, rows, :]
            zr, zi = xr * wr - xi * wi, xr * wi + xi * wr
            k1 = _dot(zr + zi, gmat(p, 0))
            inv.append(k1)
            s_v[p1, p0, 0, rows, :] = k1 + _dot(zi, gmat(p, 1))
            s_v[p1, p0, 1, rows, :] = k1 - _dot(zr, gmat(p, 2))
        return fwd, inv

    def butterflies_out(g, p0, pace):
        r0, _ = span(g)
        for q in range(9 + (g == 3)):
            src = pl.ds(r0 + q, 8, stride=9) if q < 9 else pl.ds(288, 8)
            dst = 32 * q + 8 * g if q < 9 else 288
            x = [(s_v[p1, p0, 0, src, :], s_v[p1, p0, 1, src, :]) for p1 in range(4)]
            token = pace()
            for p1 in range(2):
                x[p1] = (after(x[p1][0], token), after(x[p1][1], token))
            for b, z in enumerate(_radix4(x, True)):
                re, im = _twiddle16(z, -b * p0)
                z_v[b, p0, 0, dst:dst + 8, :] = re
                z_v[b, p0, 1, dst:dst + 8, :] = im

    def shift_response():
        for r in range(0, 64, 8):
            y0, y = _radix9_fwd([mod_tile(0, 64 * j + r) for j in range(9)])
            t_v[0, 512 + r:520 + r, :] = y0
            for q in range(1, 5):
                t_v[0, 128 * (q - 1) + r:128 * (q - 1) + r + 8, :] = y[q][0]
                t_v[0, 128 * (q - 1) + 64 + r:128 * (q - 1) + 72 + r, :] = y[q][1]

        def dc(pln, rows):
            return jnp.broadcast_to(wp_v[pln, 0, rows, :][:, 0:1], (8, 128)) * float(S)

        def store(o, base, k0):
            for g in range(4):
                br, bi = o[base + 16 * g:base + 16 * g + 8], o[base + 16 * g + 8:base + 16 * g + 16]
                rows = pl.ds(72 * g + k0, 8, stride=9)
                wr, wi = dc(0, rows), dc(1, rows)
                dc_v[0, 32 * k0 + 8 * g:32 * k0 + 8 * g + 8, :] = br * wr - bi * wi
                dc_v[1, 32 * k0 + 8 * g:32 * k0 + 8 * g + 8, :] = br * wi + bi * wr

        for q in range(1, 5):
            o = _dot(dm_v[_DF_OFF + 128 * (q - 1):_DF_OFF + 128 * q, :],
                     t_v[0, 128 * (q - 1):128 * q, :])
            store(o, 0, q)
            store(o, 64, 9 - q)
        o = _dot(dm_v[_D0F_OFF:_D0F_OFF + 80, 0:64], t_v[0, 512:576, :])
        store(o, 0, 0)
        for pln in range(2):
            dc_v[pln, 288:296, :] = o[64:72] * dc(pln, pl.ds(288, 8))

    units = [(g, p0) for g in range(4) for p0 in range(4)]
    filter_rows = {0: (80, 112), 1: (112, 128), 2: (128, 144), 6: (144, 192), 7: (192, 224),
                   8: (224, 256), 9: (256, 288), 10: (288, 304)}
    for cp in cp_w[0]:
        cp.wait()
    start_w1(1)
    start_w1(2)
    reorder_filter(0, 80, channel_dft(3))
    butterflies_in(*units[0], _Pace([], 1))
    for cp in cp_w[1]:
        cp.wait()
    for i, unit in enumerate(units):
        if i == 6:
            for cp in cp_w[2]:
                cp.wait()
            start_w1(3)
            start_w1(4)
        if i == 11:
            cp_sa.wait()
            cp_ga.wait()
            modulation(0, 512)
        if i == 12:
            modulation(1152, 1792)
        fwd, inv = token_filter(*unit)
        if i > 0:
            butterflies_out(*units[i - 1], _Pace(fwd[1:], 10))
        if i == 0:
            butterflies_in(*units[1], _Pace(fwd[:3], 10))
        if i + 2 < len(units):
            butterflies_in(*units[i + 2], _Pace(inv, 10))
        if i in filter_rows:
            reorder_filter(*filter_rows[i], inv)
        if i == 13:
            shift_response()
    butterflies_out(*units[-1], _Pace([], 1))

    cp_dm[1].wait()
    cp_sb_cb.wait()

    def channel_idft(b):
        def gather(r):
            z = [(z_v[b, p0, 0, r:r + 8, :], z_v[b, p0, 1, r:r + 8, :]) for p0 in range(4)]
            z[0] = (z[0][0] + dc_v[0, r:r + 8, :], z[0][1] + dc_v[1, r:r + 8, :])
            t = _radix4(z, True)
            return [jnp.concatenate([t[a][pln] for a in range(4)], 1) for pln in range(2)]

        results = []
        for q in range(1, 5):
            rhs = jnp.concatenate(
                sum((gather(32 * k + 8 * g) for k in (q, 9 - q) for g in range(4)), []), 0)
            results.append(_dot(dm_v[_DI_OFF + 128 * (q - 1):_DI_OFF + 128 * q, :], rhs))
            y_v[b, 128 * (q - 1):128 * q, :] = results[-1]
        rhs = jnp.concatenate(sum((gather(8 * g) for g in range(4)), []) + gather(288)[:1], 0)
        results.append(_dot(dm_v[_D0I_OFF:_D0I_OFF + 64, 0:72], rhs))
        y_v[b, 512:576, :] = results[-1]
        return results

    def residual_norms(b, pace):
        norm = []
        for a in range(4):
            lanes = slice(128 * a, 128 * (a + 1))
            st = _Stats()
            for r in range(0, 64, 8):
                p = {q: (y_v[b, 128 * (q - 1) + r:128 * (q - 1) + r + 8, lanes],
                         y_v[b, 128 * (q - 1) + 64 + r:128 * (q - 1) + 72 + r, lanes])
                     for q in range(1, 5)}
                token = pace()
                for q in (3, 4):
                    p[q] = (after(p[q][0], token), after(p[q][1], token))
                y = _radix9_inv(y_v[b, 512 + r:520 + r, lanes], p)
                for j in range(9):
                    row = 64 * j + r
                    x1 = x1_v[a, b, row:row + 8, :] + mod_tile(2, row) * y[j]
                    st.add(x1)
                    x1_v[a, b, row:row + 8, :] = x1
            rs, sh = st.scale_shift()
            st = _Stats()
            for row in range(0, D, 8):
                if row % 96 == 0:
                    scale = after(rs, pace())
                t = (x1_v[a, b, row:row + 8, :] * scale + sh) * mod_tile(4, row) + mod_tile(3, row)
                st.add(t)
                t_v[a, row:row + 8, :] = t
            rs, sh = st.scale_shift()
            norm.append((rs, jnp.concatenate([sh, sh], 0)))
        for row in range(0, QD, 16):
            h = {}
            for k in range(4):
                if k < 3:
                    token = pace()
                scale = after(norm[k][0], token)
                scale = jnp.concatenate([scale, scale], 0)
                for r in range(4):
                    rows = slice(QD * r + row, QD * r + row + 16)
                    h[r, k] = t_v[k, rows, :] * scale + norm[k][1]
                    h_v[b, k, rows, :] = h[r, k].astype(bf16)
            for i in range(7):
                quad = [_combine(_LHS[i], lambda o: h[_block(o, c)]) for c in range(4)]
                for j in range(7):
                    hs_v[i, j, b, row:row + 16, :] = _combine(
                        _LHS[j], lambda c: quad[c]).astype(bf16)

    def first_columns(b):
        lhs = jnp.concatenate([h_v[b, a] for a in range(4)], 1)
        rhs = jnp.concatenate([jnp.concatenate(
            [w1_v[n, pl.ds(pl.multiple_of(128 * (4 * a + b), 128), 128), :]
             for a in range(4)], 0) for n in range(4)], 1)
        return _dot(lhs, rhs)

    steps = 4 * (8 + 6) + 9 * 3
    channel_idft(0)
    modulation(1792, 2944)
    residual_norms(0, _Pace(sum((channel_idft(b) for b in range(1, 4)), []), 64))
    wait_all(w1_v.at[0:4], sem_in.at[23])

    def overlap(b, carry):
        start_w1(5 + b)
        part = first_columns(b)
        u_v[...] += part
        residual_norms(b + 1, _Pace([part[:, 128 * n:128 * (n + 1)] for n in range(4)], steps))
        return carry

    lax.fori_loop(0, 3, overlap, None)

    for cp in cp_b + [cp_gb]:
        cp.wait()
    modulation(2944, 6 * D)
    bias1_v[0:F // 128, :] = b1_v[...].astype(f32)
    bias2_v[0:S // 128, :] = 2.0 * b2_v[...].astype(f32)

    def activate(j):
        g, made = {}, set()

        def emit(r, n, u):
            g[r, 3 - n] = _gelu2(u + bias1_v[pl.ds(4 * j + n, 1), :])
            for i in range(7):
                for k in range(7):
                    need = [_block(o, c) for o, _ in _LHS[i] for c, _ in _LHS[k]]
                    if (i, k) not in made and all(e in g for e in need):
                        made.add((i, k))
                        act_v[i, k, j] = _combine(_LHS[k], lambda c: _combine(
                            _LHS[i], lambda o: g[_block(o, c)])).astype(bf16)
        return emit

    start_w1(8)
    u0 = u_v[...] + first_columns(3)
    emit0 = activate(0)
    for r in range(4):
        for n in range(4):
            emit0(r, n, u0[QD * r:QD * (r + 1), 128 * n:128 * (n + 1)])

    def mlp1(j, carry):
        wait_all(w1_v.at[pl.ds(4 * j, 4)], sem_w1.at[j])
        start_w2(j - 1)
        weights = lambda k, n, t: w1_v[4 * j + n, 512 * k + 128 * t:512 * k + 128 * (t + 1), :]
        lhs = lambda i, k: jnp.concatenate([hs_v[i, k, t] for t in range(4)], 1)
        _strassen2(lhs, weights, 4, stage_v, activate(j))
        return carry

    lax.fori_loop(1, n1, mlp1, None)

    def mlp2(j, carry):
        wait_all(w2_v.at[pl.ds(4 * j, 4)], sem_w2.at[j])

        def weights(k, n, t):
            tile = 4 * t + 3 - k
            return w2_v[4 * j + n, 128 * tile:128 * (tile + 1), :]

        def emit(r, n, y):
            rows = slice(QD * r, QD * (r + 1))
            y = y + bias2_v[pl.ds(4 * j + n, 1), :]
            o_v[j, n, rows, :] = (x1_v[j, n, rows, :] + mod_tile(5, QD * r, QD) * y).astype(bf16)
            pltpu.make_async_copy(o_v.at[j, n, rows, :], o_hbm.at[rows, column(4 * j + n)],
                                  sem_out.at[0]).start()

        lhs = lambda i, k: jnp.concatenate([act_v[i, k, t] for t in range(n1)], 1)
        _strassen2(lhs, weights, n1, stage_v, emit)
        return carry

    lax.fori_loop(0, n2, mlp2, None)
    wait_all(o_v, sem_out.at[0])


@jax.jit
def pallas_adaLN_cond__spectral_gfnet__mixer_token_mlp__prompt_kernel(
    A_x: jax.Array,
    A_w_r: jax.Array,
    A_w_i: jax.Array,
    B_x: jax.Array,
    B_w1: jax.Array,
    B_b1: jax.Array,
    B_w2: jax.Array,
    B_b2: jax.Array,
    c: jax.Array,
    w_mod: jax.Array,
):
    del B_x
    assert A_x.shape == (1, S, D)
    channel_table, token_table = _tables()
    n1, n2 = F // 512, S // 512
    vmem = pltpu.VMEM
    out_t = pl.pallas_call(
        _kernel,
        in_specs=[pl.BlockSpec(memory_space=pltpu.HBM)] * 11,
        out_specs=pl.BlockSpec(memory_space=pltpu.HBM),
        out_shape=jax.ShapeDtypeStruct((D, S), bf16),
        scratch_shapes=[
            vmem((4, 4, D, 128), bf16),
            vmem((2, 288, S), bf16),
            vmem((D, 6 * D), bf16),
            vmem((2, 128, 128), f32),
            vmem((6 * D, 128), f32),
            vmem((NB, 3, 64, 128), jnp.int32),
            vmem((4, D, 512), f32),
            vmem((4, 4, 2, KR, 128), f32),
            vmem((1, 4, 4, 2, KR, 128), f32),
            vmem((1, 2, NB, KR, 128), f32),
            vmem((4, 4, D, 128), f32),
            vmem((4, D, 128), f32),
            vmem((D, 512), f32),
            vmem((4, 4, D, 128), bf16),
            vmem((7, 7, 4, QD, 128), bf16),
            vmem((F // 128, S, 128), bf16),
            vmem((S // 128, F, 128), bf16),
            vmem((SLOTS, 4, F // 4, 128), f32),
            vmem((64, 128), f32),
            vmem((32, 128), f32),
            vmem((4, 4, D, 128), bf16),
            vmem((7, 7, n1, QD, 128), bf16),
            vmem((_DROWS, 128), bf16),
            vmem((_SROWS, 128), f32),
            vmem((2, KR, 128), f32),
            vmem((2, 1, S), bf16),
            vmem((8, 1, D), bf16),
            vmem((2, F // 128, 128), bf16),
            vmem((S // 128, 128), bf16),
            pltpu.SMEM((1,), jnp.int32),
            pltpu.SemaphoreType.DMA((24,)),
            pltpu.SemaphoreType.DMA((n1,)),
            pltpu.SemaphoreType.DMA((n2,)),
            pltpu.SemaphoreType.DMA((1,)),
        ],
        compiler_params=pltpu.CompilerParams(vmem_limit_bytes=124 * 1024 * 1024),
    )(
        A_x.reshape(S, D).T, A_w_r.T, A_w_i.T, B_w1, B_b1.reshape(F // 128, 128),
        B_w2, B_b2.reshape(S // 128, 128), c, w_mod, channel_table, token_table,
    )
    return out_t.T.reshape(1, S, D)
```
